```python
import jax
import jax.numpy as jnp

def _softmax(x, axis=-1):
    return jax.nn.softmax(x, axis=axis)
def _gelu(x):
    return jax.nn.gelu(x, approximate=True)
def _silu(x):
    return jax.nn.silu(x)
def _sigmoid(x):
    return jax.nn.sigmoid(x)
def _layernorm(x, axis=-1, eps=1e-5):
    m = jnp.mean(x, axis=axis, keepdims=True)
    v = jnp.var(x, axis=axis, keepdims=True)
    return (x - m) / jnp.sqrt(v + eps)
def _scatter_add(tgt, idx, src, axis=0):
    return tgt.at[idx].add(src)
def _segment_sum(src, seg, n):
    return jax.ops.segment_sum(src, seg, n)
class _Rng:
    def __init__(self, key):
        self._k = key
    def _next(self):
        self._k, sub = jax.random.split(self._k)
        return sub
    def normal(self, shape):
        return jax.random.normal(self._next(), shape, dtype=jnp.bfloat16)
    def randint(self, lo, hi, shape):
        return jax.random.randint(self._next(), shape, lo, hi, dtype=jnp.int32)
    def uniform(self, shape, lo=0.0, hi=1.0):
        return jax.random.uniform(self._next(), shape, jnp.bfloat16, lo, hi)
    def permutation(self, n):
        return jax.random.permutation(self._next(), n)


kernel_name = 'gated_mix__ssm_conv_h3__sliding_local_dilated__prompt'

def setup_inputs():
    _rng = _Rng(jax.random.key(int.from_bytes(__import__("os").urandom(4), "little")))
    _w = (lambda a: (lambda t: t.astype(jnp.bfloat16) if jnp.issubdtype(t.dtype, jnp.floating) else t)(jnp.asarray(a)))
    def _A_setup():
        B, S, D = 1, 2048, 640
        ks = 4
        return {
            "q": _w((lambda *s: _rng.normal(s) * 0.05)(B, S, D)),
            "k": _w((lambda *s: _rng.normal(s) * 0.05)(B, S, D)),
            "v": _w((lambda *s: _rng.normal(s) * 0.05)(B, S, D)),
            "shift_k": _w((lambda *s: _rng.normal(s) * 0.05)(D, ks) * 0.5),
            "ssm_k": _w((lambda *s: _rng.normal(s) * 0.05)(D, S) * (1.0 / S ** 0.5)),
            "ssm_D": _w((lambda *s: _rng.normal(s) * 0.05)(D)),
        }
    _A_in = _A_setup()

    def _B_setup():
        B, S, D = 1, 2048, 640
        return {
            "x": _w((lambda *s: _rng.normal(s) * 0.05)(B, S, D)),
            "wqkv": _w((lambda *s: _rng.normal(s) * 0.05)(D, 3 * D)),
            "wo": _w((lambda *s: _rng.normal(s) * 0.05)(D, D)),
        }
    _B_in = _B_setup()

    return {
        "A_q": _A_in["q"],
        "A_k": _A_in["k"],
        "A_v": _A_in["v"],
        "A_shift_k": _A_in["shift_k"],
        "A_ssm_k": _A_in["ssm_k"],
        "A_ssm_D": _A_in["ssm_D"],
        "B_x": _B_in["x"],
        "B_wqkv": _B_in["wqkv"],
        "B_wo": _B_in["wo"],
        "gate_w": _w((lambda *s: _rng.normal(s) * 0.05)(640)),
    }

def reference(A_q, A_k, A_v, A_shift_k, A_ssm_k, A_ssm_D, B_x, B_wqkv, B_wo, gate_w):
    def _A_ref(q, k, v, shift_k, ssm_k, ssm_D):
        B, S, D = q.shape
        ks = shift_k.shape[-1]
        k_pad = jnp.pad(k, ((0, 0), (ks - 1, 0), (0, 0)))
        k_shift = jnp.zeros_like(k)
        for t in range(ks):
            k_shift = k_shift + k_pad[:, t:t + S, :] * shift_k[:, ks - 1 - t][None, None, :]
        kv = k_shift * v
        L = 2 * S
        kv_pad = jnp.pad(kv, ((0, 0), (0, S), (0, 0)))
        kf_pad = jnp.pad(ssm_k, ((0, 0), (0, S)))
        kv_f = (lambda x, axes=(-2,-1): jnp.fft.rfft2(x.astype(jnp.float32), axes=axes))(kv_pad[:, None, :, :], axes=(1, 2))
        kf_f = (lambda x, axes=(-2,-1): jnp.fft.rfft2(x.astype(jnp.float32), axes=axes))(kf_pad[:, None, :], axes=(1, 2))
        kf_f = (lambda x, *d: x.transpose(*d))(kf_f, 1, 2, 0)
        y_f = kv_f * kf_f[None, :, :, :]
        y = (lambda x, s, axes=(-2,-1): jnp.fft.irfft2(x, s=s, axes=axes).astype(jnp.bfloat16))(y_f, (1, L), axes=(1, 2))[:, 0, :S, :]
        y = y + kv * ssm_D[None, None, :]
        return q * y

    def _B_ref(x, wqkv, wo):
        B, S, D = x.shape
        H = 32; Dh = D // H
        W, dil = 8, 2
        qkv = (lambda x, *d: x.transpose(*d))((x @ wqkv).reshape(B, S, 3, H, Dh), 2, 0, 3, 1, 4)
        q, k, v = qkv[0], qkv[1], qkv[2]
        scale = Dh ** -0.5
        pos = jnp.arange(S)
        off = jnp.arange(W) * dil
        idx = pos[:, None] - off[None, :]
        mask = idx >= 0
        idx_c = jnp.where(mask, idx, 0).reshape(-1)
        kg = k[:, :, idx_c, :].reshape(B, H, S, W, Dh)
        vg = v[:, :, idx_c, :].reshape(B, H, S, W, Dh)
        logits = jnp.einsum("bhsd,bhswd->bhsw", q, kg) * scale
        logits = jnp.where(mask[None, None, :, :], logits, -1e9)
        attn = _softmax(logits, axis=-1)
        o = jnp.einsum("bhsw,bhswd->bhsd", attn, vg)
        return (lambda x, *d: x.transpose(*d))(o, 0, 2, 1, 3).reshape(B, S, D) @ wo

    x = A_q
    g = _sigmoid((x * gate_w).sum(-1, keepdims=True))
    a = _A_ref(x, A_k, A_v, A_shift_k, A_ssm_k, A_ssm_D)
    b = _B_ref(x, B_wqkv, B_wo)
    return g * a + (1 - g) * b
```

```python
import functools
import math

import numpy as np
import jax
import jax.numpy as jnp
from jax import lax
from jax.experimental import pallas as pl
from jax.experimental.pallas import tpu as pltpu

S, D = 2048, 640
NT = D // 128
BLK = 128
NB = S // BLK
NG = 16
H, DH, WIN, DIL = 32, 20, 8, 2
HALO = 16
F32, BF16, U32 = jnp.float32, jnp.bfloat16, jnp.uint32


def _pack_rows(m):
    b = np.asarray(m, dtype=np.float32).astype(BF16).view(np.uint16).astype(np.uint32)
    return b[0::2] | (b[1::2] << 16)


def _dft_constants():
    g = np.arange(NG)[:, None]
    i = np.arange(8)[None, :]
    k = (2 * (8 * (g % 8) + i) + (g // 8)).reshape(BLK)
    n = np.arange(BLK)
    th = 2.0 * np.pi * (k[:, None] + 0.5) * n[None, :] / (2 * BLK)
    fwd = np.concatenate([np.cos(th), -np.sin(th)], axis=0)
    inv = np.zeros((BLK, NG, 8, 2))
    inv[..., 0] = (np.cos(th).T / BLK).reshape(BLK, NG, 8)
    inv[..., 1] = (-np.sin(th).T / BLK).reshape(BLK, NG, 8)
    return _pack_rows(fwd), _pack_rows(inv.reshape(BLK, 2 * BLK))


def make_kernel(R=256, phases="AWB", ua=4, ug=1, ui=4):
    NRB = S // R

    def kernel(q_hbm, k_hbm, v_hbm, sk_hbm, h_hbm, dd_hbm, wqkv_hbm, wo_hbm, gw_hbm,
               f_hbm, g_hbm, out_hbm,
               qb, kb, vb, hb, wqb, wob, skb, ddb, gwb, fb, gb,
               kf, u3, h3, zs, yy,
               wt, wtp, wof, wop,
               qs, ks, vs, ob, outb,
               sem_a, sem_m, sem_x, sem_o):
        def strip_copies(t):
            return [
                pltpu.make_async_copy(h_hbm.at[pl.ds(t * 128, 128), :], hb.at[pl.ds(t * 128, 128), :], sem_a.at[3 * t]),
                pltpu.make_async_copy(k_hbm.at[0, :, pl.ds(t * 128, 128)], kb.at[t], sem_a.at[3 * t + 1]),
                pltpu.make_async_copy(v_hbm.at[0, :, pl.ds(t * 128, 128)], vb.at[t], sem_a.at[3 * t + 2]),
            ]

        misc = [
            pltpu.make_async_copy(f_hbm, fb, sem_m.at[0]),
            pltpu.make_async_copy(g_hbm, gb, sem_m.at[1]),
            pltpu.make_async_copy(sk_hbm, skb, sem_m.at[2]),
            pltpu.make_async_copy(dd_hbm, ddb, sem_m.at[3]),
            pltpu.make_async_copy(gw_hbm, gwb, sem_m.at[4]),
        ]
        wcp = [
            pltpu.make_async_copy(wqkv_hbm, wqb, sem_m.at[5]),
            pltpu.make_async_copy(wo_hbm, wob, sem_m.at[6]),
        ]

        def row_copies(i):
            return [
                pltpu.make_async_copy(q_hbm.at[0, pl.ds(i * R, R), :], qb.at[pl.ds(i * R, R), :], sem_x.at[i]),
            ]

        for c in misc:
            c.start()
        for t in range(NT):
            for c in strip_copies(t):
                c.start()
            if t == 1:
                for c in wcp:
                    c.start()
        for i in range(NRB):
            for c in row_copies(i):
                c.start()
        for c in misc:
            c.wait()

        fmat = lambda: pltpu.bitcast(fb[...], BF16)
        gmat = lambda: pltpu.bitcast(gb[...], BF16)

        kf[pl.ds(0, 8), :] = jnp.zeros((8, 128), F32)
        skf = skb[...].astype(F32)
        ddf = ddb[...].astype(F32).reshape(1, D)

        for t in range(NT):
            for c in strip_copies(t):
                c.wait()
            if "A" not in phases:
                continue
            taps = [skf[j:j + 1, t * 128:(t + 1) * 128] for j in range(4)]
            dvec = ddf[:, t * 128:(t + 1) * 128]

            def stage_k(a, c, t=t):
                r0 = pl.multiple_of(a * BLK, BLK)
                kf[pl.ds(8 + r0, BLK), :] = kb[t, pl.ds(r0, BLK), :].astype(F32)
                return c
            lax.fori_loop(0, NB, stage_k, 0, unroll=2)

            def fwd(a, c, t=t, taps=taps, dvec=dvec):
                r0 = pl.multiple_of(a * BLK, BLK)
                ksh = kf[pl.ds(8 + r0, BLK), :] * taps[0]
                for j in range(1, 4):
                    ksh = ksh + kf[pl.ds(8 + r0 - j, BLK), :] * taps[j]
                kv = (ksh * vb[t, pl.ds(r0, BLK), :].astype(F32)).astype(BF16)
                uu = jnp.dot(fmat(), kv, preferred_element_type=F32)
                ar, ai = uu[:BLK], uu[BLK:]
                u3[0, a] = ar + ai
                u3[1, a] = ar
                u3[2, a] = ai
                hblk = hb[pl.ds(t * 128, 128), pl.ds(r0, BLK)]
                hh = lax.dot_general(fmat(), hblk, (((1,), (1,)), ((), ())), preferred_element_type=F32)
                br, bi = hh[:BLK], hh[BLK:]
                br = br + jnp.where(a == 0, 1.0, 0.0) * dvec
                h3[0, a] = br
                h3[1, a] = bi - br
                h3[2, a] = br + bi
                return c
            lax.fori_loop(0, NB, fwd, 0, unroll=ua)

            def toep(g, c, sign):
                g0 = pl.multiple_of(g * 8, 8)
                acc = []
                for comp in range(3):
                    uv = [u3[comp, a, pl.ds(g0, 8), :] for a in range(NB)]
                    hv = [h3[comp, a, pl.ds(g0, 8), :] for a in range(NB)]
                    res = []
                    for a in range(NB):
                        s = hv[0] * uv[a]
                        for d in range(1, a + 1):
                            s = s + hv[d] * uv[a - d]
                        res.append(s)
                    acc.append(res)
                cr = [acc[0][a] - acc[2][a] for a in range(NB)]
                ci = [acc[0][a] + acc[1][a] for a in range(NB)]
                for a in range(NB):
                    if a == 0:
                        zr, zi = cr[0], ci[0]
                    elif sign > 0:
                        zr, zi = cr[a] - ci[a - 1], ci[a] + cr[a - 1]
                    else:
                        zr, zi = cr[a] + ci[a - 1], ci[a] - cr[a - 1]
                    zs[a, pl.ds(g0, 8), :] = pltpu.pack_elementwise([zr, zi], packed_dtype=BF16)
                return c
            lax.fori_loop(0, NG // 2, functools.partial(toep, sign=1), 0, unroll=ug)
            lax.fori_loop(NG // 2, NG, functools.partial(toep, sign=-1), 0, unroll=ug)

            def inv(a, c, t=t):
                r0 = pl.multiple_of(a * BLK, BLK)
                z = pltpu.bitcast(zs[a], BF16)
                yy[t, pl.ds(r0, BLK), :] = jnp.dot(gmat(), z, preferred_element_type=F32)
                return c
            lax.fori_loop(0, NB, inv, 0, unroll=ui)

        for c in wcp:
            c.wait()
        if "W" in phases:
            def wtr(j, c):
                c0 = pl.multiple_of(j * 128, 128)
                for i in range(NT):
                    tile = wqb[pl.ds(i * 128, 128), pl.ds(c0, 128)].astype(F32)
                    wt[i, pl.ds(c0, 128), :] = tile.T
                return c
            lax.fori_loop(0, 3 * NT, wtr, 0)

            def wperm(p, c):
                part = p // DH
                j = p - part * DH
                src0 = part * D + j
                dst0 = pl.multiple_of(p * 16, 16)
                for i in range(NT):
                    for m in range(2):
                        a = wt[i, pl.ds(src0 + 320 * m, 8, stride=2 * DH), :]
                        b = wt[i, pl.ds(src0 + 320 * m + DH, 8, stride=2 * DH), :]
                        wtp[pl.ds(dst0 + 8 * m, 8), i * 128:(i + 1) * 128] = pltpu.pack_elementwise([a, b], packed_dtype=BF16)
                return c
            lax.fori_loop(0, 3 * DH, wperm, 0, unroll=2)

            for i in range(NT):
                wof[i] = wob[:, i * 128:(i + 1) * 128].astype(F32)

            def woperm(j, c):
                dst0 = pl.multiple_of(j * 16, 16)
                for i in range(NT):
                    for m in range(2):
                        a = wof[i, pl.ds(j + 320 * m, 8, stride=2 * DH), :]
                        b = wof[i, pl.ds(j + 320 * m + DH, 8, stride=2 * DH), :]
                        wop[pl.ds(dst0 + 8 * m, 8), i * 128:(i + 1) * 128] = pltpu.pack_elementwise([a, b], packed_dtype=BF16)
                return c
            lax.fori_loop(0, DH, woperm, 0, unroll=2)

        gwf = gwb[...].astype(F32).reshape(1, D)
        cexp = (DH ** -0.5) * math.log2(math.e)
        for t in range(NT):
            ks[t, pl.ds(0, HALO), :] = jnp.zeros((HALO, 128), F32)
            vs[t, pl.ds(0, HALO), :] = jnp.zeros((HALO, 128), F32)

        def out_copy(i, slot):
            return pltpu.make_async_copy(outb.at[slot], out_hbm.at[0, pl.ds(i * R, R), :], sem_o.at[slot])

        def bblock(i, c):
            r0 = pl.multiple_of(i * R, R)
            slot = i % 2
            cq = pltpu.make_async_copy(q_hbm.at[0, pl.ds(r0, R), :], qb.at[pl.ds(r0, R), :], sem_x.at[i])
            cq.wait()

            @pl.when(i >= 2)
            def _():
                out_copy(i - 2, slot).wait()

            if "B" in phases:
                wmat = pltpu.bitcast(wtp[...], BF16)
                qkv = lax.dot_general(qb[pl.ds(r0, R), :], wmat, (((1,), (1,)), ((), ())),
                                      preferred_element_type=F32)
                for t in range(NT):
                    qs[t] = qkv[:, t * 128:(t + 1) * 128]
                    ks[t, pl.ds(HALO, R), :] = qkv[:, D + t * 128:D + (t + 1) * 128]
                    vs[t, pl.ds(HALO, R), :] = qkv[:, 2 * D + t * 128:2 * D + (t + 1) * 128]

                def attn(rg, c):
                    b0 = pl.multiple_of(rg * 8, 8)
                    qv = [qs[t, pl.ds(b0, 8), :] for t in range(NT)]
                    pos = r0 + b0 + lax.broadcasted_iota(jnp.int32, (8, 128), 0)
                    lg = []
                    for w in range(WIN):
                        l = qv[0] * ks[0, pl.ds(HALO + b0 - DIL * w, 8), :]
                        for t in range(1, NT):
                            l = l + qv[t] * ks[t, pl.ds(HALO + b0 - DIL * w, 8), :]
                        l = l + pltpu.roll(l, 64, 1)
                        l = l + pltpu.roll(l, 32, 1)
                        if w > 0:
                            l = jnp.where(pos >= DIL * w, l, -1e30)
                        lg.append(l)
                    m = lg[0]
                    for w in range(1, WIN):
                        m = jnp.maximum(m, lg[w])
                    e = [jnp.exp2((lg[w] - m) * cexp) for w in range(WIN)]
                    den = e[0]
                    for w in range(1, WIN):
                        den = den + e[w]
                    rinv = pl.reciprocal(den, approx=True)
                    for t in range(NT):
                        o = e[0] * vs[t, pl.ds(HALO + b0, 8), :]
                        for w in range(1, WIN):
                            o = o + e[w] * vs[t, pl.ds(HALO + b0 - DIL * w, 8), :]
                        ob[pl.ds(b0, 8), t * 128:(t + 1) * 128] = o * rinv
                    return c
                lax.fori_loop(0, R // 8, attn, 0, unroll=2)

                for t in range(NT):
                    ks[t, pl.ds(0, HALO), :] = ks[t, pl.ds(R, HALO), :]
                    vs[t, pl.ds(0, HALO), :] = vs[t, pl.ds(R, HALO), :]

                bo = jnp.dot(ob[...].astype(BF16), pltpu.bitcast(wop[...], BF16), preferred_element_type=F32)
                qa = qb[pl.ds(r0, R), :].astype(F32)
                gate = jax.nn.sigmoid(jnp.sum(qa * gwf, axis=-1, keepdims=True))
                for t in range(NT):
                    sl = slice(t * 128, (t + 1) * 128)
                    a_br = qa[:, sl] * yy[t, pl.ds(r0, R), :]
                    b_br = bo[:, sl]
                    outb[slot, :, sl] = (b_br + gate * (a_br - b_br)).astype(BF16)
            else:
                outb[slot] = qb[pl.ds(r0, R), :]
            out_copy(i, slot).start()
            return c
        lax.fori_loop(0, NRB, bblock, 0)
        out_copy(NRB - 2, NRB % 2).wait()
        out_copy(NRB - 1, (NRB - 1) % 2).wait()

    scratch = [
        pltpu.VMEM((S, D), BF16),
        pltpu.VMEM((NT, S, 128), BF16),
        pltpu.VMEM((NT, S, 128), BF16),
        pltpu.VMEM((D, S), BF16),
        pltpu.VMEM((D, 3 * D), BF16),
        pltpu.VMEM((D, D), BF16),
        pltpu.VMEM((4, D), BF16),
        pltpu.VMEM((D,), BF16),
        pltpu.VMEM((D,), BF16),
        pltpu.VMEM((BLK, BLK), U32),
        pltpu.VMEM((BLK // 2, 2 * BLK), U32),
        pltpu.VMEM((S + 8, 128), F32),
        pltpu.VMEM((3, NB, BLK, 128), F32),
        pltpu.VMEM((3, NB, BLK, 128), F32),
        pltpu.VMEM((NB, BLK, 128), U32),
        pltpu.VMEM((NT, S, 128), F32),
        pltpu.VMEM((NT, 3 * D, 128), F32),
        pltpu.VMEM((3 * D // 2, D), U32),
        pltpu.VMEM((NT, D, 128), F32),
        pltpu.VMEM((D // 2, D), U32),
        pltpu.VMEM((NT, R, 128), F32),
        pltpu.VMEM((NT, R + HALO, 128), F32),
        pltpu.VMEM((NT, R + HALO, 128), F32),
        pltpu.VMEM((R, D), F32),
        pltpu.VMEM((2, R, D), BF16),
        pltpu.SemaphoreType.DMA((3 * NT,)),
        pltpu.SemaphoreType.DMA((7,)),
        pltpu.SemaphoreType.DMA((NRB,)),
        pltpu.SemaphoreType.DMA((2,)),
    ]

    fwd_c, inv_c = _dft_constants()

    @jax.jit
    def run(A_q, A_k, A_v, A_shift_k, A_ssm_k, A_ssm_D, B_x, B_wqkv, B_wo, gate_w):
        return pl.pallas_call(
            kernel,
            out_shape=jax.ShapeDtypeStruct((1, S, D), BF16),
            in_specs=[pl.BlockSpec(memory_space=pl.ANY)] * 11,
            out_specs=pl.BlockSpec(memory_space=pl.ANY),
            scratch_shapes=scratch,
            compiler_params=pltpu.CompilerParams(vmem_limit_bytes=100 * 1024 * 1024),
        )(A_q, A_k, A_v, A_shift_k.T, A_ssm_k, A_ssm_D, B_wqkv, B_wo, gate_w,
          jnp.asarray(fwd_c), jnp.asarray(inv_c))

    return run


pallas_gated_mix__ssm_conv_h3__sliding_local_dilated__prompt_kernel = make_kernel()
```

```python
import functools
import math

import numpy as np
import jax
import jax.numpy as jnp
from jax import lax
from jax.experimental import pallas as pl
from jax.experimental.pallas import tpu as pltpu

S, D = 2048, 640
NT = D // 128
BLK = 128
NB = S // BLK
NG = 16
H, DH, WIN, DIL = 32, 20, 8, 2
PAD = 16
F32, BF16, U32 = jnp.float32, jnp.bfloat16, jnp.uint32
NT_DIMS = (((1,), (1,)), ((), ()))
ONE_LO, ONE_HI = 0x3F80, 0x3F800000


def _pack_rows(m):
    b = np.asarray(m, dtype=np.float32).astype(BF16).view(np.uint16).astype(np.uint32)
    return b[0::2] | (b[1::2] << 16)


def _dft_constants():
    k = np.arange(BLK)
    n = np.arange(BLK)
    th = 2.0 * np.pi * (k[:, None] + 0.5) * n[None, :] / (2 * BLK)
    fwd = np.stack([np.cos(th).reshape(NG, 8, BLK), -np.sin(th).reshape(NG, 8, BLK)], axis=1).reshape(2 * BLK, BLK)
    inv = np.stack([np.cos(th).T / BLK, -np.sin(th).T / BLK], axis=-1).reshape(BLK, 2 * BLK)
    pi = _pack_rows(inv)
    return np.concatenate([_pack_rows(fwd), pi[:, :BLK], pi[:, BLK:]], axis=0)


def _toeplitz(hv, uv):
    res = [None] * NB
    for a in reversed(range(NB)):
        s = hv[0] * uv[a]
        for d in range(1, a + 1):
            s = s + hv[d] * uv[a - d]
        res[a] = s
    return res


def _interleave(streams):
    items = []
    for s in streams:
        for idx, fn in enumerate(s):
            items.append(((idx + 0.5) / len(s), fn))
    items.sort(key=lambda x: x[0])
    return [fn for _, fn in items]


def default_plan():
    plan = {e: dict(P=[], T=[], F=[], TP=[], IV=[], O=[], G=[]) for e in range(1, 17)}
    plan[1]["P"] = [2]
    plan[1]["T"] = [0, 1]
    for e in range(2, 15):
        plan[e]["P"] = [e + 1]
        plan[e]["T"] = [e]
    plan[15]["T"] = [15]
    plan[1]["F"] = [(0, a) for a in range(16)]
    for t in range(1, NT):
        plan[2 * t]["F"] = [(t, a) for a in range(8)]
        plan[2 * t + 1]["F"] = [(t, a) for a in range(8, 16)]
    for t in range(NT):
        plan[2 + 2 * t]["TP"] = [(t, g) for g in range(8)]
        plan[3 + 2 * t]["TP"] = [(t, g) for g in range(8, 16)]
        plan[4 + 2 * t]["IV"] = [(t, a) for a in range(8)]
        plan[5 + 2 * t]["IV"] = [(t, a) for a in range(8, 16)]
    for i in range(NB):
        plan[max(2, i)]["G"].append(i)
    todo = [(i, n) for n in range(NT) for i in range(NB)]
    quota = {6: 2, 7: 2, 8: 3, 9: 3, 10: 10, 11: 10, 12: 10, 13: 12, 14: 12, 15: 11, 16: 99}
    for e in range(6, 17):
        avail = [x for x in todo if 4 + 2 * x[1] + (1 if x[0] >= 8 else 0) < e and max(x[0], 1) < e]
        avail.sort(key=lambda x: (x[0], x[1]) if e >= 13 else (x[1], x[0]))
        take = avail[:quota[e]]
        plan[e]["O"] = take
        for x in take:
            todo.remove(x)
    assert not todo, todo
    return plan


def make_kernel(plan=None, skip="", sepmode="wait"):
    plan = plan or default_plan()

    def kernel(q_hbm, k_hbm, v_hbm, sk_hbm, h_hbm, dd_hbm, wqkv_hbm, wo_hbm, gw_hbm, c_hbm, out_hbm,
               qb, kb, vb, hb, wqb, wob, skb, ddb, gwb, cb,
               fm, gm, em, bc,
               wt, wtp, wof, wop, xs,
               qs, ks, vs, ob, gs,
               kfa, kfb, u3a, u3b, h3a, h3b, zsa, zsb, yy, outb,
               sem_in, sem_o):
        kfs, u3s, h3s, zss = (kfa, kfb), (u3a, u3b), (h3a, h3b), (zsa, zsb)

        def rows(i0, i1):
            return pl.ds(i0 * BLK, (i1 - i0) * BLK)

        copies = {}
        nsem = [0]

        def add_copy(name, src, dst):
            copies.setdefault(name, []).append(pltpu.make_async_copy(src, dst, sem_in.at[nsem[0]]))
            nsem[0] += 1

        for part, nm in enumerate(("Wq", "Wk", "Wv")):
            add_copy(nm, wqkv_hbm.at[:, pl.ds(part * D, D)], wqb.at[:, pl.ds(part * D, D)])
        add_copy("misc", c_hbm, cb)
        add_copy("misc", sk_hbm, skb)
        add_copy("misc", dd_hbm, ddb)
        add_copy("misc", gw_hbm, gwb)
        add_copy("Wo", wo_hbm, wob)
        qgroups = {"q01": (0, 2), "q2": (2, 3), "q34": (3, 5), "q58": (5, 9), "q9f": (9, 16)}
        for nm, (i0, i1) in qgroups.items():
            add_copy(nm, q_hbm.at[0, rows(i0, i1), :], qb.at[rows(i0, i1), :])
        for t in range(NT):
            add_copy("A%d" % t, h_hbm.at[pl.ds(t * 128, 128), :], hb.at[pl.ds(t * 128, 128), :])
            add_copy("A%d" % t, k_hbm.at[0, :, pl.ds(t * 128, 128)], kb.at[t])
            add_copy("A%d" % t, v_hbm.at[0, :, pl.ds(t * 128, 128)], vb.at[t])

        def start(*names):
            for nm in names:
                for c in copies[nm]:
                    c.start()

        def wait(*names):
            for nm in names:
                for c in copies[nm]:
                    c.wait()

        def out_copy(j, i0, i1):
            return pltpu.make_async_copy(outb.at[rows(i0, i1), :], out_hbm.at[0, rows(i0, i1), :], sem_o.at[j])

        def tile16(v):
            return jnp.concatenate([v] * (BLK // 8), axis=0)

        def fmat(a):
            return pltpu.bitcast(fm[a % 2], BF16)

        def gmat(a):
            return pltpu.bitcast(jnp.concatenate([gm[a % 2, 0], gm[a % 2, 1]], axis=1), BF16)

        emat = lambda j: pltpu.bitcast(em[j], BF16)
        cexp = (DH ** -0.5) * math.log2(math.e)

        def setup_masks():
            r = lax.broadcasted_iota(jnp.int32, (64, 128), 0)
            l = lax.broadcasted_iota(jnp.int32, (64, 128), 1)
            lo, hi, zero = jnp.uint32(ONE_LO), jnp.uint32(ONE_HI), jnp.uint32(0)
            em[0] = jnp.where(l == 2 * r, lo, zero) | jnp.where(l == 2 * r + 1, hi, zero)
            em[1] = jnp.where((l & 31) == ((2 * r) & 31), lo, zero) | jnp.where((l & 31) == ((2 * r + 1) & 31), hi, zero)
            em[2] = jnp.full((64, 128), ONE_LO | ONE_HI, U32)
            for t in range(NT):
                ks[t, pl.ds(0, PAD), :] = jnp.zeros((PAD, 128), F32)
                vs[t, pl.ds(0, PAD), :] = jnp.zeros((PAD, 128), F32)
            kfa[pl.ds(0, 8), :] = jnp.zeros((8, 128), F32)
            kfb[pl.ds(0, 8), :] = jnp.zeros((8, 128), F32)

        def setup_misc():
            f = cb[pl.ds(0, 128), :]
            fm[0] = f
            fm[1] = f ^ jnp.uint32(0x80000000)
            l = lax.broadcasted_iota(jnp.int32, (64, 128), 1)
            flip = jnp.where((l & 2) != 0, jnp.uint32(0x80008000), jnp.uint32(0))
            for hf in range(2):
                g = cb[pl.ds(128 + 64 * hf, 64), :]
                gm[0, hf] = g
                gm[1, hf] = g ^ flip
            skf = skb[...].astype(F32)
            ddf = ddb[...].astype(F32).reshape(1, D)
            gwf = gwb[...].astype(F32).reshape(1, D)
            for t in range(NT):
                sl = slice(t * 128, (t + 1) * 128)
                for j in range(4):
                    bc[6 * t + j] = jnp.broadcast_to(skf[j:j + 1, sl], (8, 128))
                bc[6 * t + 4] = jnp.broadcast_to(ddf[:, sl], (8, 128))
                bc[6 * t + 5] = jnp.broadcast_to(gwf[:, sl], (8, 128))

        def WT(c):
            for i in range(NT):
                tile = wqb[pl.ds(i * 128, 128), pl.ds(c * 128, 128)]
                wt[i, pl.ds(c * 128, 128), :] = lax.dot_general(emat(0), tile, NT_DIMS, preferred_element_type=F32)

        def WP(part, t):
            for j in range(4 * t, 4 * t + 4):
                src0 = part * D + j
                dst0 = (part * DH + j) * 16
                for i in range(NT):
                    for m in range(2):
                        a = wt[i, pl.ds(src0 + 320 * m, 8, stride=2 * DH), :]
                        b = wt[i, pl.ds(src0 + 320 * m + DH, 8, stride=2 * DH), :]
                        wtp[pl.ds(dst0 + 8 * m, 8), i * 128:(i + 1) * 128] = pltpu.pack_elementwise([a, b], packed_dtype=BF16)

        def WO(i):
            wof[i] = wob[:, i * 128:(i + 1) * 128].astype(F32)
            for j in range(DH):
                for m in range(2):
                    a = wof[i, pl.ds(j + 320 * m, 8, stride=2 * DH), :]
                    b = wof[i, pl.ds(j + 320 * m + DH, 8, stride=2 * DH), :]
                    wop[pl.ds(j * 16 + 8 * m, 8), i * 128:(i + 1) * 128] = pltpu.pack_elementwise([a, b], packed_dtype=BF16)

        def X(i):
            xs[pl.ds(i * 64, 64), :] = pltpu.bitcast(qb[rows(i, i + 1), :], U32)

        def P(i, n):
            xblk = pltpu.bitcast(xs[pl.ds(i * 64, 64), :], BF16)
            wn = pltpu.bitcast(wtp[pl.ds(n * 64, 64), :], BF16)
            res = lax.dot_general(xblk, wn, NT_DIMS, preferred_element_type=F32)
            part, t = divmod(n, NT)
            if part == 0:
                qs[t, rows(i, i + 1), :] = res
            elif part == 1:
                ks[t, pl.ds(PAD + i * BLK, BLK), :] = res
            else:
                vs[t, pl.ds(PAD + i * BLK, BLK), :] = res

        def T(i, p):
            b0 = i * BLK + 16 * p
            lg = []
            for c in range(2):
                qv = [qs[t, pl.ds(b0 + c, 8, stride=2), :] for t in range(NT)]
                for w in range(WIN):
                    l = qv[0] * ks[0, pl.ds(PAD + b0 + c - DIL * w, 8, stride=2), :]
                    for t in range(1, NT):
                        l = l + qv[t] * ks[t, pl.ds(PAD + b0 + c - DIL * w, 8, stride=2), :]
                    lg.append(l)
            red = jnp.dot(jnp.concatenate(lg, axis=0).astype(BF16), emat(1), preferred_element_type=F32)
            outs = []
            for c in range(2):
                lw = [red[(c * WIN + w) * 8:(c * WIN + w + 1) * 8] for w in range(WIN)]
                if b0 < DIL * (WIN - 1):
                    pos = b0 + c + 2 * lax.broadcasted_iota(jnp.int32, (8, 128), 0)
                    lw = [jnp.where(pos >= DIL * w, lw[w], -1e30) for w in range(WIN)]
                m = lw[0]
                for w in range(1, WIN):
                    m = jnp.maximum(m, lw[w])
                e = [jnp.exp2((lw[w] - m) * cexp) for w in range(WIN)]
                den = e[0]
                for w in range(1, WIN):
                    den = den + e[w]
                rinv = pl.reciprocal(den, approx=True)
                oc = []
                for t in range(NT):
                    o = e[0] * vs[t, pl.ds(PAD + b0 + c, 8, stride=2), :]
                    for w in range(1, WIN):
                        o = o + e[w] * vs[t, pl.ds(PAD + b0 + c - DIL * w, 8, stride=2), :]
                    oc.append(o * rinv)
                outs.append(oc)
            for t in range(NT):
                ob[t, pl.ds(b0 // 2, 8), :] = pltpu.pack_elementwise([outs[0][t], outs[1][t]], packed_dtype=BF16)

        def G(i):
            zp = None
            for t in range(NT):
                term = qb[rows(i, i + 1), t * 128:(t + 1) * 128].astype(F32) * tile16(bc[6 * t + 5])
                zp = term if zp is None else zp + term
            z = jnp.dot(zp.astype(BF16), emat(2), preferred_element_type=F32)
            gs[rows(i, i + 1), :] = 0.5 + 0.5 * jnp.tanh(0.5 * z)

        def O(i, n):
            sl = slice(n * 128, (n + 1) * 128)
            o = pltpu.bitcast(jnp.concatenate([ob[t, pl.ds(i * 64, 64), :] for t in range(NT)], axis=1), BF16)
            bo = jnp.dot(o, pltpu.bitcast(wop[:, sl], BF16), preferred_element_type=F32)
            a_br = qb[rows(i, i + 1), sl].astype(F32) * yy[n, rows(i, i + 1), :]
            outb[rows(i, i + 1), sl] = (bo + gs[rows(i, i + 1), :] * (a_br - bo)).astype(BF16)

        def F(t, a):
            kf, u3, h3 = kfs[t % 2], u3s[t % 2], h3s[t % 2]
            r0 = a * BLK
            kf[pl.ds(8 + r0, BLK), :] = kb[t, pl.ds(r0, BLK), :].astype(F32)
            ksh = kf[pl.ds(8 + r0, BLK), :] * tile16(bc[6 * t])
            for j in range(1, 4):
                ksh = ksh + kf[pl.ds(8 + r0 - j, BLK), :] * tile16(bc[6 * t + j])
            kv = (ksh * vb[t, pl.ds(r0, BLK), :].astype(F32)).astype(BF16)
            uu = jnp.dot(fmat(a), kv, preferred_element_type=F32).reshape(NG, 2, 8, 128)
            ar, ai = uu[:, 0], uu[:, 1]
            u3[0, a] = ar + ai
            u3[1, a] = ar
            u3[2, a] = ai
            hblk = hb[pl.ds(t * 128, 128), pl.ds(r0, BLK)]
            hh = lax.dot_general(fmat(a), hblk, NT_DIMS, preferred_element_type=F32).reshape(NG, 2, 8, 128)
            br, bi = hh[:, 0], hh[:, 1]
            h3[0, a] = br
            h3[1, a] = bi - br
            h3[2, a] = br + bi

        def TP(t, g):
            u3, h3, zs = u3s[t % 2], h3s[t % 2], zss[t % 2]
            dv = bc[6 * t + 4]
            acc = []
            for comp in range(3):
                uv = [u3[comp, a, g] for a in range(NB)]
                hv = [h3[comp, a, g] for a in range(NB)]
                hv[0] = hv[0] - dv if comp == 1 else hv[0] + dv
                acc.append(_toeplitz(hv, uv))
            cr = [acc[0][a] - acc[2][a] for a in range(NB)]
            ci = [acc[0][a] + acc[1][a] for a in range(NB)]
            for a in range(NB):
                if a == 0:
                    zr, zi = cr[0], ci[0]
                else:
                    zr, zi = cr[a] - ci[a - 1], ci[a] + cr[a - 1]
                zs[a, pl.ds(g * 8, 8), :] = pltpu.pack_elementwise([zr, zi], packed_dtype=BF16)

        def IV(t, a):
            z = pltpu.bitcast(zss[t % 2][a], BF16)
            yy[t, rows(a, a + 1), :] = jnp.dot(gmat(a), z, preferred_element_type=F32)

        def run(fns):
            for fn in fns:
                fn()

        pt = functools.partial

        start("Wq", "q01")
        start("Wk")
        setup_masks()
        wait("Wq", "q01")
        start("Wv", "misc", "q2")
        run([pt(WT, c) for c in range(5)])
        run([pt(X, 0), pt(X, 1)])
        run([pt(WP, 0, t) for t in range(NT)])
        run([pt(P, i, n) for i in range(2) for n in range(5)])
        wait("Wk")
        start("A0")
        run([pt(WT, c) for c in range(5, 10)])
        run([pt(WP, 1, t) for t in range(NT)])
        run([pt(P, i, n) for i in range(2) for n in range(5, 10)])
        wait("Wv", "misc", "q2")
        start("q34", "A1")
        setup_misc()
        run([pt(WT, c) for c in range(10, 15)])
        run([pt(WP, 2, t) for t in range(NT)])
        run([pt(P, i, n) for i in range(2) for n in range(10, 15)])

        waits = {1: ("A0",), 2: ("q34", "A1"), 4: ("q58", "A2"), 5: ("Wo",), 6: ("A3",), 8: ("q9f", "A4")}
        starts = {1: ("q58", "A2"), 2: ("Wo", "A3"), 4: ("q9f", "A4")}
        out_groups = []
        done_o = set()
        next_out = 0
        for e in range(1, 17):
            if e in waits:
                wait(*waits[e])
            if e in starts:
                start(*starts[e])
            pe = plan[e]
            streams = []
            for i in pe["P"]:
                streams.append([pt(X, i)] + [pt(P, i, n) for n in range(3 * NT)])
            if pe["T"]:
                streams.append([pt(T, i, p) for i in pe["T"] for p in range(8)])
            for key, fn in (("F", F), ("TP", TP), ("IV", IV), ("O", O)):
                if pe[key] and key not in skip.split(","):
                    streams.append([pt(fn, *x) for x in pe[key]])
            if e == 5:
                streams.append([pt(WO, i) for i in range(NT)])
            if pe["G"]:
                run([pt(G, i) for i in pe["G"]])
            run(_interleave(streams))
            done_o.update(pe["O"])
            i1 = next_out
            while i1 < NB and all((i1, n) in done_o for n in range(NT)):
                i1 += 1
            if i1 > next_out and e >= 13:
                cp = out_copy(len(out_groups), next_out, i1)
                cp.start()
                out_groups.append(cp)
                next_out = i1
        assert next_out == NB
        for cp in out_groups:
            cp.wait()

    scratch = [
        pltpu.VMEM((S, D), BF16),
        pltpu.VMEM((NT, S, 128), BF16),
        pltpu.VMEM((NT, S, 128), BF16),
        pltpu.VMEM((D, S), BF16),
        pltpu.VMEM((D, 3 * D), BF16),
        pltpu.VMEM((D, D), BF16),
        pltpu.VMEM((4, D), BF16),
        pltpu.VMEM((D,), BF16),
        pltpu.VMEM((D,), BF16),
        pltpu.VMEM((256, 128), U32),
        pltpu.VMEM((2, 128, 128), U32),
        pltpu.VMEM((2, 2, 64, 128), U32),
        pltpu.VMEM((3, 64, 128), U32),
        pltpu.VMEM((6 * NT, 8, 128), F32),
        pltpu.VMEM((NT, 3 * D, 128), F32),
        pltpu.VMEM((3 * D // 2, D), U32),
        pltpu.VMEM((NT, D, 128), F32),
        pltpu.VMEM((D // 2, D), U32),
        pltpu.VMEM((S // 2, D), U32),
        pltpu.VMEM((NT, S, 128), F32),
        pltpu.VMEM((NT, S + PAD, 128), F32),
        pltpu.VMEM((NT, S + PAD, 128), F32),
        pltpu.VMEM((NT, S // 2, 128), U32),
        pltpu.VMEM((S, 128), F32),
        pltpu.VMEM((S + 8, 128), F32),
        pltpu.VMEM((S + 8, 128), F32),
        pltpu.VMEM((3, NB, NG, 8, 128), F32),
        pltpu.VMEM((3, NB, NG, 8, 128), F32),
        pltpu.VMEM((3, NB, NG, 8, 128), F32),
        pltpu.VMEM((3, NB, NG, 8, 128), F32),
        pltpu.VMEM((NB, BLK, 128), U32),
        pltpu.VMEM((NB, BLK, 128), U32),
        pltpu.VMEM((NT, S, 128), F32),
        pltpu.VMEM((S, D), BF16),
        pltpu.SemaphoreType.DMA((32,)),
        pltpu.SemaphoreType.DMA((8,)),
    ]

    consts = _dft_constants()

    @jax.jit
    def run_kernel(A_q, A_k, A_v, A_shift_k, A_ssm_k, A_ssm_D, B_x, B_wqkv, B_wo, gate_w):
        return pl.pallas_call(
            kernel,
            out_shape=jax.ShapeDtypeStruct((1, S, D), BF16),
            in_specs=[pl.BlockSpec(memory_space=pl.ANY)] * 10,
            out_specs=pl.BlockSpec(memory_space=pl.ANY),
            scratch_shapes=scratch,
            compiler_params=pltpu.CompilerParams(vmem_limit_bytes=110 * 1024 * 1024),
        )(A_q, A_k, A_v, A_shift_k.T, A_ssm_k, A_ssm_D, B_wqkv, B_wo, gate_w, jnp.asarray(consts))

    return run_kernel


pallas_gated_mix__ssm_conv_h3__sliding_local_dilated__prompt_kernel = make_kernel()
```

```python
import contextlib
import functools
import math

import numpy as np
import jax
import jax.numpy as jnp
from jax import lax
from jax.experimental import pallas as pl
from jax.experimental.pallas import tpu as pltpu

S, D = 2048, 640
NT = D // 128
BLK = 128
NB = S // BLK
NG = 16
H, DH, WIN, DIL = 32, 20, 8, 2
PAD = 16
F32, BF16, U32 = jnp.float32, jnp.bfloat16, jnp.uint32
NT_DIMS = (((1,), (1,)), ((), ()))
ONE_LO, ONE_HI = 0x3F80, 0x3F800000
pt = functools.partial


def _pack_rows(m):
    b = np.asarray(m, dtype=np.float32).astype(BF16).view(np.uint16).astype(np.uint32)
    return b[0::2] | (b[1::2] << 16)


def _dft_constants():
    k = np.arange(BLK)
    n = np.arange(BLK)
    th = 2.0 * np.pi * (k[:, None] + 0.5) * n[None, :] / (2 * BLK)
    fwd = np.stack([np.cos(th).reshape(NG, 8, BLK), -np.sin(th).reshape(NG, 8, BLK)], axis=1).reshape(2 * BLK, BLK)
    inv = np.stack([np.cos(th).T / BLK, -np.sin(th).T / BLK], axis=-1).reshape(BLK, 2 * BLK)
    pi = _pack_rows(inv)
    return np.concatenate([_pack_rows(fwd), pi[:, :BLK], pi[:, BLK:]], axis=0)


def _interleave(streams):
    items = []
    for si, s in enumerate(streams):
        if not s:
            continue
        tot = float(sum(w for w, _ in s))
        acc = 0.0
        for w, fn in s:
            items.append(((acc + 0.5 * w) / tot, si, fn))
            acc += w
    items.sort(key=lambda x: (x[0], x[1]))
    return [fn for _, _, fn in items]


COST = dict(X=(0, 40), P=(2400, 960), TL=(0, 1216), TR=(256, 1960), GB=(160, 120), KV=(0, 170), FU=(64, 16), FH=(64, 40),
            TPA=(0, 775), TPB=(0, 80), IV=(64, 16), O=(160, 150), WO=(0, 130))
KEYS = ("X", "P", "TL", "TR", "GB", "KV", "FU", "FH", "TPA", "TPB", "IV", "O", "WO")


def make_plan(tl_ep=(1, 1, 2, 4, 6, 8, 10, 11, 12, 13, 13, 14, 14, 15, 15, 16), tp0=3, rate=8.0, wo_epoch=5, m_target=4600, a_ready=(1, 2, 3, 4, 6), nep=None, p_ep=None, o_rows_from=None):
    p_ep = p_ep or [0, 0] + list(range(1, 15))
    nep = nep or max(tl_ep) + 2
    plan = {e: {k: [] for k in KEYS} for e in range(1, nep + 1)}
    for i in range(3, NB):
        plan[max(1, p_ep[i] - 1)]["X"].append(i)
    for i in range(2, NB):
        plan[p_ep[i]]["P"].append(i)
    for i in range(NB):
        assert tl_ep[i] > p_ep[i], i
        plan[tl_ep[i]]["TL"].append(i)
        plan[tl_ep[i] + 1]["TR"].append(i)
        plan[max(3, tl_ep[i] + 1)]["GB"].append(i)
    ep_tp = [tp0 + int(v / rate) for v in range(80)]
    for v in range(80):
        plan[ep_tp[v]]["TPA"].append(divmod(v, 16))
        plan[ep_tp[v] + 1]["TPB"].append(divmod(v, 16))
    plan[1]["KV"] = [(0, a) for a in range(16)]
    plan[1]["FH"] = [(0, a) for a in range(16)]
    plan[tp0 - 1]["FU"] += [(0, a) for a in range(16)]
    kv_done = {0: tp0 - 1}
    for t in range(1, NT):
        last = ep_tp[16 * t] - 1
        first = max(3, ep_tp[16 * (t - 1)], a_ready[t] + 1)
        if t >= 3:
            first = max(first, ep_tp[16 * (t - 3) + 15] + 1)
        if t >= 2:
            first = max(first, kv_done[t - 2] + 2)
        eps = list(range(first, last + 1))
        assert eps, (t, first, last)
        for a in range(16):
            e = eps[a * len(eps) // 16]
            plan[e]["FU"].append((t, a))
            plan[e]["FH"].append((t, a))
            plan[e - 1]["KV"].append((t, a))
        kv_done[t] = last
    iv_ep = {}
    for t in range(NT):
        e0 = ep_tp[16 * t + 15] + 2
        for a in range(16):
            e = e0 + (a >= 8 and t < NT - 1)
            plan[e]["IV"].append((t, a))
            iv_ep[(t, a)] = e
    plan[wo_epoch]["WO"] = list(range(NT))

    def mxu(e):
        return sum(COST[k][0] * len(v) for k, v in plan[e].items())
    todo = [(i, n) for n in range(NT) for i in range(NB)]
    o_rows_from = o_rows_from or (iv_ep[(NT - 1, 0)] + 1)
    for e in range(wo_epoch + 1, nep + 1):
        avail = [x for x in todo if iv_ep[(x[1], x[0])] < e and tl_ep[x[0]] + 1 < e and max(3, tl_ep[x[0]] + 1) < e]
        avail.sort(key=lambda x: (x[0], x[1]))
        for x in avail:
            if e < nep and mxu(e) + 160 > m_target:
                break
            plan[e]["O"].append(x)
            todo.remove(x)
    assert not todo, todo
    return plan


def make_kernel(plan=None, skip="", scopes=False, barriers=(10, 12, 14, 16), out_chunk=8, out_mode="rows",
                tp_parts=((15, 14), (13, 12, 11), (10, 9, 8, 7), (6, 5, 4, 3, 2, 1, 0)), plan_kw=None, pin="", pace="TL,KV,TPA,TPB", lag=0, waitfirst=False):
    plan = plan or make_plan(**(plan_kw or {}))
    nep = max(plan)

    def kernel(q_hbm, k_hbm, v_hbm, sk_hbm, h_hbm, dd_hbm, wqkv_hbm, wo_hbm, gw_hbm, c_hbm, z_hbm, out_hbm,
               qb, kb, vb, hb, wqb, wob, skb, ddb, gwb, cb,
               fm, gm, em, bc,
               wt, wtp, wof, wop, xs,
               qs, ks, vs, lgs, ob, gwm, gs,
               kfa, kfb, kva, kvb, u3a, u3b, u3c, h3a, h3b, h3c, aca, acb, zsa, zsb, zsc, yy, outb,
               dumf, dumu, sem_in, sem_o, sem_b, sem_d, zsm):
        kfs, kvs, u3s, h3s = (kfa, kfb), (kva, kvb), (u3a, u3b, u3c), (h3a, h3b, h3c)
        acs, zss = (aca, acb), (zsa, zsb, zsc)

        def rows(i0, i1=None):
            i1 = i0 + 1 if i1 is None else i1
            return pl.ds(i0 * BLK, (i1 - i0) * BLK)

        copies = {}
        nsem = [0]

        def add_copy(name, src, dst):
            copies.setdefault(name, []).append(pltpu.make_async_copy(src, dst, sem_in.at[nsem[0]]))
            nsem[0] += 1

        add_copy("Wq0", wqkv_hbm.at[:, pl.ds(0, 256)], wqb.at[:, pl.ds(0, 256)])
        add_copy("Wq1", wqkv_hbm.at[:, pl.ds(256, 384)], wqb.at[:, pl.ds(256, 384)])
        for part, nm in ((1, "Wk"), (2, "Wv")):
            add_copy(nm, wqkv_hbm.at[:, pl.ds(part * D, D)], wqb.at[:, pl.ds(part * D, D)])
        add_copy("z", z_hbm, zsm)
        add_copy("misc", c_hbm, cb)
        add_copy("misc", sk_hbm, skb)
        add_copy("misc", dd_hbm, ddb)
        add_copy("misc", gw_hbm, gwb)
        add_copy("Wo", wo_hbm, wob)
        qgroups = {"q01": (0, 2), "q23": (2, 4), "q47": (4, 8), "q8f": (8, 16)}
        for nm, (i0, i1) in qgroups.items():
            add_copy(nm, q_hbm.at[0, rows(i0, i1), :], qb.at[rows(i0, i1), :])
        for t in range(NT):
            add_copy("A%d" % t, h_hbm.at[pl.ds(t * 128, 128), :], hb.at[pl.ds(t * 128, 128), pl.ds(0, S)])
            add_copy("A%d" % t, k_hbm.at[0, :, pl.ds(t * 128, 128)], kb.at[t, pl.ds(16, S), :])
            add_copy("A%d" % t, v_hbm.at[0, :, pl.ds(t * 128, 128)], vb.at[t])

        def start(*names):
            for nm in names:
                for c in copies[nm]:
                    c.start()

        def wait(*names):
            for nm in names:
                for c in copies[nm]:
                    c.wait()

        def barrier():
            pl.semaphore_signal(sem_b, 1)
            pl.semaphore_wait(sem_b, 1)

        def pin_buffers():
            names = pin.split(",")
            f32 = {"qs": [qs.at[0, pl.ds(S, 8), :]], "u3": [r.at[0, 0, NG] for r in u3s], "h3": [r.at[0, 0, NG] for r in h3s],
                   "ac": [r.at[0, 0, NG] for r in acs], "yy": [yy.at[0, pl.ds(0, 8), :]], "gs": [gs.at[pl.ds(0, 8), :]],
                   "bc": [bc.at[0]]}
            u32 = {"zs": [r.at[0, pl.ds(0, 8), :] for r in zss], "xs": [xs.at[pl.ds(0, 8), pl.ds(0, 128)]],
                   "wtp": [wtp.at[pl.ds(0, 8), pl.ds(0, 128)]], "wop": [wop.at[pl.ds(0, 8), pl.ds(0, 128)]],
                   "fm": [fm.at[0, pl.ds(0, 8), :]], "gm": [gm.at[0, 0, pl.ds(0, 8), :]], "em": [em.at[0, pl.ds(0, 8), :]]}
            cps = []
            for table, dum, dt in ((f32, dumf, F32), (u32, dumu, U32)):
                k = 0
                for nm in names:
                    for r in table.get(nm, []):
                        r[...] = jnp.zeros((8, 128), dt)
                        cps.append(pltpu.make_async_copy(r, dum.at[k], sem_d.at[len(cps)]))
                        k += 1
            for c in cps:
                c.start()
            for c in cps:
                c.wait()

        state = {"marks": [], "use": None}

        def dep(x):
            mk = state["use"]
            if mk is None:
                return x
            mask = lax.broadcasted_iota(jnp.int32, (8, 128), 0) < zsm[0]
            return jnp.where(mask, mk, x)

        def mark(res):
            state["marks"] += [res[8 * j:8 * j + 8] for j in range(res.shape[0] // 8)]

        def rep(v, n):
            return jnp.concatenate([v] * n, axis=0)

        def words(ref, *idx):
            return pltpu.bitcast(ref.bitcast(U32)[idx], BF16)

        def fmat(a):
            return pltpu.bitcast(fm[a % 2], BF16)

        def gmat(a):
            return pltpu.bitcast(jnp.concatenate([gm[a % 2, 0], gm[a % 2, 1]], axis=1), BF16)

        emat = lambda j: pltpu.bitcast(em[j], BF16)
        cexp = (DH ** -0.5) * math.log2(math.e)

        def setup_masks():
            r = lax.broadcasted_iota(jnp.int32, (64, 128), 0)
            l = lax.broadcasted_iota(jnp.int32, (64, 128), 1)
            lo, hi, zero = jnp.uint32(ONE_LO), jnp.uint32(ONE_HI), jnp.uint32(0)
            em[0] = jnp.where(l == 2 * r, lo, zero) | jnp.where(l == 2 * r + 1, hi, zero)
            em[1] = jnp.where((l & 31) == ((2 * r) & 31), lo, zero) | jnp.where((l & 31) == ((2 * r + 1) & 31), hi, zero)
            em[2] = jnp.full((64, 128), ONE_LO | ONE_HI, U32)
            for t in range(NT):
                ks[t, pl.ds(0, PAD), :] = jnp.zeros((PAD, 128), F32)
                vs[t, pl.ds(0, PAD), :] = jnp.zeros((PAD, 128), F32)
            for t in range(NT):
                kb[t, pl.ds(0, 16), :] = jnp.zeros((16, 128), BF16)

        def setup_misc():
            f = cb[pl.ds(0, 128), :]
            fm[0] = f
            fm[1] = f ^ jnp.uint32(0x80000000)
            l = lax.broadcasted_iota(jnp.int32, (64, 128), 1)
            flip = jnp.where((l & 2) != 0, jnp.uint32(0x80008000), jnp.uint32(0))
            for hf in range(2):
                g = cb[pl.ds(128 + 64 * hf, 64), :]
                gm[0, hf] = g
                gm[1, hf] = g ^ flip
            skf = skb[...].astype(F32)
            ddf = ddb[...].astype(F32).reshape(1, D)
            gwf = gwb[...].astype(F32).reshape(1, D)
            for t in range(NT):
                sl = slice(t * 128, (t + 1) * 128)
                for j in range(4):
                    bc[6 * t + j] = jnp.broadcast_to(skf[j:j + 1, sl], (8, 128))
                bc[6 * t + 4] = jnp.broadcast_to(ddf[:, sl], (8, 128))
                g8 = jnp.broadcast_to(gwf[:, sl], (8, 128))
                gwm[:, sl] = jnp.concatenate([pltpu.pack_elementwise([g8, g8], packed_dtype=BF16)] * 8, axis=0)

        def WT(c):
            for i in range(NT):
                tile = wqb[pl.ds(i * 128, 128), pl.ds(c * 128, 128)]
                wt[i, pl.ds(c * 128, 128), :] = lax.dot_general(emat(0), tile, NT_DIMS, preferred_element_type=F32)

        def WP(part, t):
            for j in range(4 * t, 4 * t + 4):
                src0 = part * D + j
                dst0 = (part * DH + j) * 16
                for i in range(NT):
                    for m in range(2):
                        a = wt[i, pl.ds(src0 + 320 * m, 8, stride=2 * DH), :]
                        b = wt[i, pl.ds(src0 + 320 * m + DH, 8, stride=2 * DH), :]
                        if part == 0:
                            a, b = a * cexp, b * cexp
                        wtp[pl.ds(dst0 + 8 * m, 8), i * 128:(i + 1) * 128] = pltpu.pack_elementwise([a, b], packed_dtype=BF16)

        def WO(i):
            wof[i] = wob[:, i * 128:(i + 1) * 128].astype(F32)
            for j in range(DH):
                for m in range(2):
                    a = wof[i, pl.ds(j + 320 * m, 8, stride=2 * DH), :]
                    b = wof[i, pl.ds(j + 320 * m + DH, 8, stride=2 * DH), :]
                    wop[pl.ds(j * 16 + 8 * m, 8), i * 128:(i + 1) * 128] = pltpu.pack_elementwise([a, b], packed_dtype=BF16)

        def X(i):
            xs[pl.ds(i * 64, 64), :] = pltpu.bitcast(qb[rows(i), :], U32)

        def P(i, n):
            xblk = pltpu.bitcast(xs[pl.ds(i * 64, 64), :], BF16)
            wn = pltpu.bitcast(wtp[pl.ds(n * 64, 64), :], BF16)
            res = lax.dot_general(xblk, wn, NT_DIMS, preferred_element_type=F32)
            mark(res)
            part, t = divmod(n, NT)
            if part == 0:
                qs[t, rows(i), :] = res
            elif part == 1:
                ks[t, pl.ds(PAD + i * BLK, BLK), :] = res
            else:
                vs[t, pl.ds(PAD + i * BLK, BLK), :] = res

        def TL(i, p, c):
            r = i * BLK + 16 * p + 8 * c
            qv = [qs[t, pl.ds(r, 8), :] for t in range(NT)]
            qv[0] = dep(qv[0])
            ls = []
            for w in range(WIN):
                l = qv[0] * ks[0, pl.ds(PAD + r - DIL * w, 8), :]
                for t in range(1, NT):
                    l = l + qv[t] * ks[t, pl.ds(PAD + r - DIL * w, 8), :]
                ls.append(l)
            lgs[i % 4, p, pl.ds(64 * c, 64), :] = jnp.concatenate(ls, axis=0).astype(BF16)

        def TR(i, p):
            b0 = i * BLK + 16 * p
            red = jnp.dot(words(lgs, i % 4, p), emat(1), preferred_element_type=F32)
            outs = []
            for c in range(2):
                r = b0 + 8 * c
                lw = [red[(c * WIN + w) * 8:(c * WIN + w + 1) * 8] for w in range(WIN)]
                if r < DIL * (WIN - 1):
                    pos = r + lax.broadcasted_iota(jnp.int32, (8, 128), 0)
                    lw = [jnp.where(pos >= DIL * w, lw[w], -1e30) for w in range(WIN)]
                m = lw[0]
                for w in range(1, WIN):
                    m = jnp.maximum(m, lw[w])
                e = [jnp.exp2(lw[w] - m) for w in range(WIN)]
                den = e[0]
                for w in range(1, WIN):
                    den = den + e[w]
                rinv = pl.reciprocal(den, approx=True)
                oc = [e[0] * vs[t, pl.ds(PAD + r, 8), :] for t in range(NT)]
                for w in range(1, WIN):
                    oc = [oc[t] + e[w] * vs[t, pl.ds(PAD + r - DIL * w, 8), :] for t in range(NT)]
                oc = [oc[t] * rinv for t in range(NT)]
                outs.append(oc)
            for t in range(NT):
                ob[t, pl.ds(b0, 16), :] = jnp.concatenate([outs[0][t], outs[1][t]], axis=0).astype(BF16)

        def GB(i):
            xblk = pltpu.bitcast(xs[pl.ds(i * 64, 64), :], BF16)
            z = lax.dot_general(xblk, pltpu.bitcast(gwm[...], BF16), NT_DIMS, preferred_element_type=F32)
            mark(z)
            gs[rows(i), :] = 0.5 + 0.5 * jnp.tanh(0.5 * z)

        def O(i, n):
            sl = slice(n * 128, (n + 1) * 128)
            obw = ob.bitcast(U32)
            o = pltpu.bitcast(jnp.concatenate([obw[t, pl.ds(i * 64, 64), :] for t in range(NT)], axis=1), BF16)
            bo = jnp.dot(o, pltpu.bitcast(wop[:, sl], BF16), preferred_element_type=F32)
            mark(bo)
            a_br = qb[rows(i), sl].astype(F32) * yy[n, rows(i), :]
            outb[rows(i), sl] = (bo + gs[rows(i), :] * (a_br - bo)).astype(BF16)

        def KV(t, a):
            kw, vw = kb.bitcast(U32), vb.bitcast(U32)
            lo = lambda x: pltpu.unpack_elementwise(x, index=0, packed_dtype=BF16, unpacked_dtype=F32)
            hi = lambda x: pltpu.unpack_elementwise(x, index=1, packed_dtype=BF16, unpacked_dtype=F32)
            c = [dep(bc[6 * t])] + [bc[6 * t + j] for j in range(1, 4)]
            for m in range(8):
                base = 8 + 64 * a + 8 * m
                p0, p1, p2 = kw[t, pl.ds(base, 8), :], kw[t, pl.ds(base - 1, 8), :], kw[t, pl.ds(base - 2, 8), :]
                l0, h0, l1, h1, h2 = lo(p0), hi(p0), lo(p1), hi(p1), hi(p2)
                ev = c[0] * l0 + c[1] * h1 + c[2] * l1 + c[3] * h2
                od = c[0] * h0 + c[1] * l0 + c[2] * h1 + c[3] * l1
                vv = vw[t, pl.ds(64 * a + 8 * m, 8), :]
                kvs[t % 2][a, pl.ds(8 * m, 8), :] = pltpu.pack_elementwise([ev * lo(vv), od * hi(vv)], packed_dtype=BF16)

        def FU(t, a):
            u3 = u3s[t % 3]
            uu = jnp.dot(fmat(a), pltpu.bitcast(kvs[t % 2][a], BF16), preferred_element_type=F32)
            mark(uu[:64])
            uu = uu.reshape(NG, 2, 8, 128)
            ar, ai = uu[:, 0], uu[:, 1]
            u3[0, a, pl.ds(0, NG)] = ar + ai
            u3[1, a, pl.ds(0, NG)] = ar
            u3[2, a, pl.ds(0, NG)] = ai

        def FH(t, a):
            h3 = h3s[t % 3]
            hblk = hb[pl.ds(t * 128, 128), pl.ds(a * BLK, BLK)]
            hh = lax.dot_general(fmat(a), hblk, NT_DIMS, preferred_element_type=F32)
            mark(hh[:64])
            hh = hh.reshape(NG, 2, 8, 128)
            br, bi = hh[:, 0], hh[:, 1]
            h3[0, a, pl.ds(0, NG)] = br
            h3[1, a, pl.ds(0, NG)] = bi - br
            h3[2, a, pl.ds(0, NG)] = br + bi

        def TPA(t, g, comp, part, cache):
            u3, h3, ac = u3s[t % 3], h3s[t % 3], acs[t % 2]
            if part == 0:
                dv = bc[6 * t + 4]
                cache["u"] = [u3[comp, a, g] for a in range(NB)]
                hv = [h3[comp, a, g] for a in range(NB)]
                hv[0] = hv[0] - dv if comp == 1 else hv[0] + dv
                cache["h"] = hv
            uv, hv = cache["u"], cache["h"]
            h0 = dep(hv[0])
            for a in tp_parts[part]:
                s = h0 * uv[a]
                for d in range(1, a + 1):
                    s = s + hv[d] * uv[a - d]
                ac[comp, a, g] = s

        def TPB(t, g):
            ac, zs = acs[t % 2], zss[t % 3]
            prev = None
            for a in range(NB):
                a1 = ac[0, a, g]
                if a == 0:
                    a1 = dep(a1)
                cr, ci = a1 - ac[2, a, g], a1 + ac[1, a, g]
                zr, zi = (cr, ci) if prev is None else (cr - prev[1], ci + prev[0])
                prev = (cr, ci)
                zs[a, pl.ds(g * 8, 8), :] = pltpu.pack_elementwise([zr, zi], packed_dtype=BF16)

        def IV(t, a):
            z = pltpu.bitcast(zss[t % 3][a], BF16)
            y = jnp.dot(gmat(a), z, preferred_element_type=F32)
            mark(y[:64])
            yy[t, rows(a), :] = y

        def step_of(order, fn):
            names = [f.func.__name__ for f in order]
            per = {"P": 16, "O": 16, "GB": 16, "FU": 8, "FH": 8, "IV": 8}
            nm = sum(per.get(n, 0) for n in names)
            npaced = sum(n in pace.split(",") for n in names)
            return max(1, nm // max(1, npaced))

        def run(fns):
            for fn in fns:
                fn()

        scope = (lambda n: jax.named_scope(n)) if scopes else (lambda n: contextlib.nullcontext())
        with scope("ep00a"):
            start("Wq0", "Wq1", "q01", "z", "Wk", "Wv", "misc", "q23", "A0", "A1", "q47", "A2", "Wo", "A3", "q8f", "A4")
            if pin:
                pin_buffers()
            setup_masks()
            if waitfirst:
                allc = list(copies)
                wait(*allc)
                copies.update({k: [] for k in allc})
            wait("Wq0")
            run([pt(WT, c) for c in range(2)])
            wait("Wq1", "q01", "z")
            run([pt(WT, c) for c in range(2, 5)])
            run([pt(X, 0), pt(X, 1)])
            run([pt(WP, 0, t) for t in range(NT)])
            run([pt(P, i, n) for n in range(5) for i in range(2)])
        with scope("ep00b"):
            wait("Wk")
            run([pt(WT, c) for c in range(5, 10)])
            run([pt(WP, 1, t) for t in range(NT)])
            run([pt(P, i, n) for n in range(5, 10) for i in range(2)])
        with scope("ep00c"):
            wait("Wv", "misc", "q23")
            setup_misc()
            run([pt(X, 2)])
            run([pt(WT, c) for c in range(10, 15)])
            run([pt(WP, 2, t) for t in range(NT)])
            run([pt(P, i, n) for n in range(10, 15) for i in range(2)])

        def first_epoch(pred):
            return min(e for e in plan if pred(plan[e]))
        waits = {}
        for nm in ("q47", "q8f"):
            i0 = qgroups[nm][0]
            waits.setdefault(first_epoch(lambda pe: any(i >= i0 for i in pe["X"])), []).append(nm)
        for t in range(NT):
            waits.setdefault(first_epoch(lambda pe: any(x[0] == t for x in pe["KV"] + pe["FH"])), []).append("A%d" % t)
        waits.setdefault(first_epoch(lambda pe: pe["WO"]), []).append("Wo")
        starts = {}
        out_groups = []
        done_o = set()
        sent = {n: 0 for n in range(NT)}
        sent_rows = [0]
        sk = skip.split(",")
        for e in range(1, nep + 1):
            with scope("ep%02d" % e):
                if e in waits:
                    wait(*waits[e])
                elif e in barriers and e not in starts:
                    barrier()
                if e in starts:
                    start(*starts[e])
                pe = {k: (v if k not in sk else []) for k, v in plan[e].items()}
                streams = [
                    [(160, pt(P, i, n)) for i in pe["P"] for n in range(3 * NT)],
                    [(160, pt(O, *x)) for x in pe["O"]],
                    [(64, pt(FH, *x)) for x in pe["FH"]] ,
                    [(64, pt(FU, *x)) for x in pe["FU"]],
                    [(64, pt(IV, *x)) for x in pe["IV"]],
                    [(160, pt(GB, i)) for i in pe["GB"]],
                    [(55, pt(TR, i, p)) for i in pe["TR"] for p in range(8)],
                    [(10, pt(X, i)) for i in pe["X"]] + [(20, pt(TL, i, p, c)) for i in pe["TL"] for p in range(8) for c in range(2)],
                    [(42, pt(KV, *x)) for x in pe["KV"]],
                    [(20, pt(TPB, *x)) for x in pe["TPB"]],
                    [(30, pt(WO, i)) for i in pe["WO"]],
                ]
                lst = []
                for (t, g) in pe["TPA"]:
                    for c in range(3):
                        cache = {}
                        lst += [(16, pt(TPA, t, g, c, part, cache)) for part in range(len(tp_parts))]
                streams.append(lst)
                order = _interleave(streams)
                state["marks"] = []
                paced = set(pace.split(",")) if pace else set()
                seen = 0
                for fn in order:
                    if fn.func.__name__ in paced and state["marks"]:
                        marks = state["marks"]
                        idx = max(0, min(len(marks) - 1, seen - lag))
                        state["use"] = marks[idx]
                        seen = min(len(marks), seen + step_of(order, fn))
                    else:
                        state["use"] = None
                    fn()
                state["use"] = None
                done_o.update(plan[e]["O"])
                if out_mode == "strip":
                    for n in range(NT):
                        i1 = sent[n]
                        while i1 < NB and (i1, n) in done_o:
                            i1 += 1
                        if i1 - sent[n] >= out_chunk or (i1 > sent[n] and (i1 == NB or e >= nep - 1)):
                            cols = pl.ds(n * 128, 128)
                            cp = pltpu.make_async_copy(outb.at[rows(sent[n], i1), cols], out_hbm.at[0, rows(sent[n], i1), cols],
                                                       sem_o.at[len(out_groups)])
                            cp.start()
                            out_groups.append(cp)
                            sent[n] = i1
                else:
                    i1 = sent_rows[0]
                    while i1 < NB and all((i1, n) in done_o for n in range(NT)):
                        i1 += 1
                    if i1 > sent_rows[0]:
                        cp = pltpu.make_async_copy(outb.at[rows(sent_rows[0], i1), :], out_hbm.at[0, rows(sent_rows[0], i1), :],
                                                   sem_o.at[len(out_groups)])
                        cp.start()
                        out_groups.append(cp)
                        sent_rows[0] = i1
        for cp in out_groups:
            cp.wait()

    scratch = [
        pltpu.VMEM((S, D), BF16),
        pltpu.VMEM((NT, S + 16, 128), BF16),
        pltpu.VMEM((NT, S, 128), BF16),
        pltpu.VMEM((D, S + 128), BF16),
        pltpu.VMEM((D, 3 * D), BF16),
        pltpu.VMEM((D, D), BF16),
        pltpu.VMEM((4, D), BF16),
        pltpu.VMEM((D,), BF16),
        pltpu.VMEM((D,), BF16),
        pltpu.VMEM((256, 128), U32),
        pltpu.VMEM((2, 128, 128), U32),
        pltpu.VMEM((2, 2, 64, 128), U32),
        pltpu.VMEM((3, 64, 128), U32),
        pltpu.VMEM((6 * NT, 8, 128), F32),
        pltpu.VMEM((NT, 3 * D, 128), F32),
        pltpu.VMEM((3 * D // 2, D), U32),
        pltpu.VMEM((NT, D, 128), F32),
        pltpu.VMEM((D // 2, D), U32),
        pltpu.VMEM((S // 2, D), U32),
        pltpu.VMEM((NT, S + 8, 128), F32),
        pltpu.VMEM((NT, S + PAD + 8, 128), F32),
        pltpu.VMEM((NT, S + PAD + 8, 128), F32),
        pltpu.VMEM((4, 8, 128, 128), BF16),
        pltpu.VMEM((NT, S, 128), BF16),
        pltpu.VMEM((64, D), U32),
        pltpu.VMEM((S, 128), F32),
        pltpu.VMEM((S + 8, 128), F32),
        pltpu.VMEM((S + 8, 128), F32),
        pltpu.VMEM((NB, 64, 128), U32),
        pltpu.VMEM((NB, 64, 128), U32),
        pltpu.VMEM((3, NB, NG + 1, 8, 128), F32),
        pltpu.VMEM((3, NB, NG + 1, 8, 128), F32),
        pltpu.VMEM((3, NB, NG + 1, 8, 128), F32),
        pltpu.VMEM((3, NB, NG + 1, 8, 128), F32),
        pltpu.VMEM((3, NB, NG + 1, 8, 128), F32),
        pltpu.VMEM((3, NB, NG + 1, 8, 128), F32),
        pltpu.VMEM((3, NB, NG + 1, 8, 128), F32),
        pltpu.VMEM((3, NB, NG + 1, 8, 128), F32),
        pltpu.VMEM((NB, BLK, 128), U32),
        pltpu.VMEM((NB, BLK, 128), U32),
        pltpu.VMEM((NB, BLK, 128), U32),
        pltpu.VMEM((NT, S, 128), F32),
        pltpu.VMEM((S, D), BF16),
        pltpu.VMEM((24, 8, 128), F32),
        pltpu.VMEM((24, 8, 128), U32),
        pltpu.SemaphoreType.DMA((40,)),
        pltpu.SemaphoreType.DMA((32,)),
        pltpu.SemaphoreType.REGULAR,
        pltpu.SemaphoreType.DMA((48,)),
        pltpu.SMEM((8,), jnp.int32),
    ]

    consts = _dft_constants()

    @jax.jit
    def run_kernel(A_q, A_k, A_v, A_shift_k, A_ssm_k, A_ssm_D, B_x, B_wqkv, B_wo, gate_w):
        return pl.pallas_call(
            kernel,
            out_shape=jax.ShapeDtypeStruct((1, S, D), BF16),
            in_specs=[pl.BlockSpec(memory_space=pl.ANY)] * 11,
            out_specs=pl.BlockSpec(memory_space=pl.ANY),
            scratch_shapes=scratch,
            compiler_params=pltpu.CompilerParams(vmem_limit_bytes=110 * 1024 * 1024),
        )(A_q, A_k, A_v, A_shift_k.T, A_ssm_k, A_ssm_D, B_wqkv, B_wo, gate_w, jnp.asarray(consts), jnp.asarray(np.zeros((8,), np.int32)))

    return run_kernel


pallas_gated_mix__ssm_conv_h3__sliding_local_dilated__prompt_kernel = make_kernel()
```

```python
import contextlib
import functools
import math

import numpy as np
import jax
import jax.numpy as jnp
from jax import lax
from jax.experimental import pallas as pl
from jax.experimental.pallas import tpu as pltpu

S, D = 2048, 640
NT = D // 128
BLK = 128
NB = S // BLK
NG = 16
H, DH, WIN, DIL = 32, 20, 8, 2
PAD = 16
F32, BF16, U32 = jnp.float32, jnp.bfloat16, jnp.uint32
NT_DIMS = (((1,), (1,)), ((), ()))
ONE_LO, ONE_HI = 0x3F80, 0x3F800000
pt = functools.partial


def _pack_rows(m):
    b = np.asarray(m, dtype=np.float32).astype(BF16).view(np.uint16).astype(np.uint32)
    return b[0::2] | (b[1::2] << 16)


def _dft_constants():
    k = np.arange(BLK)
    n = np.arange(BLK)
    th = 2.0 * np.pi * (k[:, None] + 0.5) * n[None, :] / (2 * BLK)
    fwd = np.stack([np.cos(th).reshape(NG, 8, BLK), -np.sin(th).reshape(NG, 8, BLK)], axis=1).reshape(2 * BLK, BLK)
    inv = np.stack([np.cos(th).T / BLK, -np.sin(th).T / BLK], axis=-1).reshape(BLK, 2 * BLK)
    pi = _pack_rows(inv)
    return np.concatenate([_pack_rows(fwd), pi[:, :BLK], pi[:, BLK:]], axis=0)


def _interleave(streams, shifts=None):
    items = []
    for si, s in enumerate(streams):
        if not s:
            continue
        tot = float(sum(w for w, _ in s))
        acc = 0.0
        for w, fn in s:
            items.append(((acc + 0.5 * w) / tot - (shifts[si] if shifts else 0.0), si, fn))
            acc += w
    items.sort(key=lambda x: (x[0], x[1]))
    return [fn for _, _, fn in items]


COST = dict(X=(0, 40), P=(2400, 960), TL=(0, 1216), TR=(256, 1960), GB=(160, 120), KV=(0, 170), FU=(64, 16), FH=(64, 40),
            TPA=(0, 775), TPB=(0, 80), IV=(64, 16), O=(160, 150), WO=(0, 130))
KEYS = ("X", "P", "TL", "TR", "GB", "KV", "FU", "FH", "TPA", "TPB", "IV", "O", "WO")


def make_plan(tl_ep=(1, 2, 2, 3, 5, 7, 9, 11, 12, 13, 14, 14, 15, 15, 16, 16), tp0=4, a0=2, rate=8.0, wo_epoch=6, m_target=4600, a_ready=(2, 3, 4, 5, 7), nep=None, p_ep=None, o_rows_from=None):
    p_ep = p_ep or [0, 1, 1] + list(range(2, 15))
    nep = nep or max(tl_ep) + 2
    plan = {e: {k: [] for k in KEYS} for e in range(1, nep + 1)}
    for i in range(3, NB):
        plan[max(1, p_ep[i] - 1)]["X"].append(i)
    for i in range(1, NB):
        plan[p_ep[i]]["P"].append(i)
    for i in range(NB):
        assert tl_ep[i] > p_ep[i], i
        plan[tl_ep[i]]["TL"].append(i)
        plan[tl_ep[i] + 1]["TR"].append(i)
        plan[max(3, tl_ep[i] + 1)]["GB"].append(i)
    ep_tp = [tp0 + int(v / rate) for v in range(80)]
    for v in range(80):
        plan[ep_tp[v]]["TPA"].append(divmod(v, 16))
        plan[ep_tp[v] + 1]["TPB"].append(divmod(v, 16))
    plan[a0]["KV"] = [(0, a) for a in range(16)]
    plan[a0]["FH"] = [(0, a) for a in range(16)]
    plan[tp0 - 1]["FU"] += [(0, a) for a in range(16)]
    kv_done = {0: tp0 - 1}
    for t in range(1, NT):
        last = ep_tp[16 * t] - 1
        first = max(a0 + 2, ep_tp[16 * (t - 1)], a_ready[t] + 1)
        if t >= 3:
            first = max(first, ep_tp[16 * (t - 3) + 15] + 1)
        if t >= 2:
            first = max(first, kv_done[t - 2] + 2)
        eps = list(range(first, last + 1))
        assert eps, (t, first, last)
        for a in range(16):
            e = eps[a * len(eps) // 16]
            plan[e]["FU"].append((t, a))
            plan[e]["FH"].append((t, a))
            plan[e - 1]["KV"].append((t, a))
        kv_done[t] = last
    iv_ep = {}
    for t in range(NT):
        e0 = ep_tp[16 * t + 15] + 2
        for a in range(16):
            e = e0 + (a >= 8 and t < NT - 1)
            plan[e]["IV"].append((t, a))
            iv_ep[(t, a)] = e
    plan[wo_epoch]["WO"] = list(range(NT))

    def mxu(e):
        return sum(COST[k][0] * len(v) for k, v in plan[e].items())
    todo = [(i, n) for n in range(NT) for i in range(NB)]
    o_rows_from = o_rows_from or (iv_ep[(NT - 1, 0)] + 1)
    for e in range(wo_epoch + 1, nep + 1):
        avail = [x for x in todo if iv_ep[(x[1], x[0])] < e and tl_ep[x[0]] + 1 < e and max(3, tl_ep[x[0]] + 1) < e]
        avail.sort(key=lambda x: (x[0], x[1]))
        for x in avail:
            if e < nep and mxu(e) + 160 > m_target:
                break
            plan[e]["O"].append(x)
            todo.remove(x)
    assert not todo, todo
    return plan


def make_kernel(plan=None, skip="", scopes=False, barriers=(10, 12, 15), out_chunk=8, out_mode="rows",
                tp_parts=((15, 14, 13, 12), (11, 10, 9, 8), (7, 6, 5, 4, 3, 2, 1, 0)), plan_kw=None, pin="", pace="TL,KV,TPA,TPB,GA,TRS", lag=0, waitfirst=False, keep=16, mshift=0.0, gate="valu", kvsplit=2, trsplit=False, mscale=1.0, waits_override={1: ["q3"], 2: ["A0", "q45"], 3: ["A1", "q67"], 5: ["A2"], 6: ["Wo", "A3", "q8f"], 8: ["A4"]}, out_eps=None, tp_order="rows"):
    plan = plan or make_plan(**(plan_kw or {}))
    nep = max(plan)

    def kernel(q_hbm, k_hbm, v_hbm, sk_hbm, h_hbm, dd_hbm, wqkv_hbm, wo_hbm, gw_hbm, c_hbm, z_hbm, out_hbm,
               qb, kb, vb, hb, wqb, wob, skb, ddb, gwb, cb,
               fm, gm, em, bc,
               wt, wtp, wof, wop, xs,
               qs, ks, vs, lgs, ob, gwm, gps, gs,
               kfa, kfb, kva, kvb, u3a, u3b, u3c, h3a, h3b, h3c, aca, acb, zsa, zsb, zsc, yy, outb,
               dumf, dumu, sem_in, sem_o, sem_b, sem_d, zsm):
        kfs, kvs, u3s, h3s = (kfa, kfb), (kva, kvb), (u3a, u3b, u3c), (h3a, h3b, h3c)
        acs, zss = (aca, acb), (zsa, zsb, zsc)

        def rows(i0, i1=None):
            i1 = i0 + 1 if i1 is None else i1
            return pl.ds(i0 * BLK, (i1 - i0) * BLK)

        copies = {}
        nsem = [0]

        def add_copy(name, src, dst):
            copies.setdefault(name, []).append(pltpu.make_async_copy(src, dst, sem_in.at[nsem[0]]))
            nsem[0] += 1

        add_copy("Wq0", wqkv_hbm.at[:, pl.ds(0, 256)], wqb.at[:, pl.ds(0, 256)])
        add_copy("Wq1", wqkv_hbm.at[:, pl.ds(256, 384)], wqb.at[:, pl.ds(256, 384)])
        for part, nm in ((1, "Wk"), (2, "Wv")):
            add_copy(nm, wqkv_hbm.at[:, pl.ds(part * D, D)], wqb.at[:, pl.ds(part * D, D)])
        add_copy("z", z_hbm, zsm)
        add_copy("misc", c_hbm, cb)
        add_copy("misc", sk_hbm, skb)
        add_copy("misc", dd_hbm, ddb)
        add_copy("misc", gw_hbm, gwb)
        add_copy("Wo", wo_hbm, wob)
        qgroups = {"q01": (0, 2), "q2": (2, 3), "q3": (3, 4), "q45": (4, 6), "q67": (6, 8), "q8f": (8, 16)}
        for nm, (i0, i1) in qgroups.items():
            add_copy(nm, q_hbm.at[0, rows(i0, i1), :], qb.at[rows(i0, i1), :])
        for t in range(NT):
            add_copy("A%d" % t, h_hbm.at[pl.ds(t * 128, 128), :], hb.at[pl.ds(t * 128, 128), pl.ds(0, S)])
            add_copy("A%d" % t, k_hbm.at[0, :, pl.ds(t * 128, 128)], kb.at[t, pl.ds(16, S), :])
            add_copy("A%d" % t, v_hbm.at[0, :, pl.ds(t * 128, 128)], vb.at[t])

        def start(*names):
            for nm in names:
                for c in copies[nm]:
                    c.start()

        def wait(*names):
            for nm in names:
                for c in copies[nm]:
                    c.wait()

        def barrier():
            pl.semaphore_signal(sem_b, 1)
            pl.semaphore_wait(sem_b, 1)

        def pin_buffers():
            names = pin.split(",")
            f32 = {"qs": [qs.at[0, pl.ds(S, 8), :]], "u3": [r.at[0, 0, NG] for r in u3s], "h3": [r.at[0, 0, NG] for r in h3s],
                   "ac": [r.at[0, 0, NG] for r in acs], "yy": [yy.at[0, pl.ds(0, 8), :]], "gs": [gs.at[pl.ds(0, 8), :]],
                   "bc": [bc.at[0]]}
            u32 = {"zs": [r.at[0, pl.ds(0, 8), :] for r in zss], "xs": [xs.at[pl.ds(0, 8), pl.ds(0, 128)]],
                   "wtp": [wtp.at[pl.ds(0, 8), pl.ds(0, 128)]], "wop": [wop.at[pl.ds(0, 8), pl.ds(0, 128)]],
                   "fm": [fm.at[0, pl.ds(0, 8), :]], "gm": [gm.at[0, 0, pl.ds(0, 8), :]], "em": [em.at[0, pl.ds(0, 8), :]]}
            cps = []
            for table, dum, dt in ((f32, dumf, F32), (u32, dumu, U32)):
                k = 0
                for nm in names:
                    for r in table.get(nm, []):
                        r[...] = jnp.zeros((8, 128), dt)
                        cps.append(pltpu.make_async_copy(r, dum.at[k], sem_d.at[len(cps)]))
                        k += 1
            for c in cps:
                c.start()
            for c in cps:
                c.wait()

        state = {"marks": [], "use": None}

        def dep(x):
            mk = state["use"]
            if mk is None:
                return x
            mask = lax.broadcasted_iota(jnp.int32, (8, 128), 0) < zsm[0]
            return jnp.where(mask, mk, x)

        def mark(res):
            state["marks"] += [res[8 * j:8 * j + 8] for j in range(res.shape[0] // 8)]

        def rep(v, n):
            return jnp.concatenate([v] * n, axis=0)

        def words(ref, *idx):
            return pltpu.bitcast(ref.bitcast(U32)[idx], BF16)

        def fmat(a):
            return pltpu.bitcast(fm[a % 2], BF16)

        def gmat(a):
            return pltpu.bitcast(jnp.concatenate([gm[a % 2, 0], gm[a % 2, 1]], axis=1), BF16)

        emat = lambda j: pltpu.bitcast(em[j], BF16)
        cexp = (DH ** -0.5) * math.log2(math.e)

        def setup_masks():
            r = lax.broadcasted_iota(jnp.int32, (64, 128), 0)
            l = lax.broadcasted_iota(jnp.int32, (64, 128), 1)
            lo, hi, zero = jnp.uint32(ONE_LO), jnp.uint32(ONE_HI), jnp.uint32(0)
            em[0] = jnp.where(l == 2 * r, lo, zero) | jnp.where(l == 2 * r + 1, hi, zero)
            em[1] = jnp.where((l & 31) == ((2 * r) & 31), lo, zero) | jnp.where((l & 31) == ((2 * r + 1) & 31), hi, zero)
            em[2] = jnp.full((64, 128), ONE_LO | ONE_HI, U32)
            for t in range(NT):
                ks[t, pl.ds(0, PAD), :] = jnp.zeros((PAD, 128), F32)
                vs[t, pl.ds(0, PAD), :] = jnp.zeros((PAD, 128), F32)
            for t in range(NT):
                kb[t, pl.ds(0, 16), :] = jnp.zeros((16, 128), BF16)

        def setup_misc():
            f = cb[pl.ds(0, 128), :]
            fm[0] = f
            fm[1] = f ^ jnp.uint32(0x80000000)
            l = lax.broadcasted_iota(jnp.int32, (64, 128), 1)
            flip = jnp.where((l & 2) != 0, jnp.uint32(0x80008000), jnp.uint32(0))
            for hf in range(2):
                g = cb[pl.ds(128 + 64 * hf, 64), :]
                gm[0, hf] = g
                gm[1, hf] = g ^ flip
            skf = skb[...].astype(F32)
            ddf = ddb[...].astype(F32).reshape(1, D)
            gwf = gwb[...].astype(F32).reshape(1, D)
            for t in range(NT):
                sl = slice(t * 128, (t + 1) * 128)
                for j in range(4):
                    bc[6 * t + j] = jnp.broadcast_to(skf[j:j + 1, sl], (8, 128))
                bc[6 * t + 4] = jnp.broadcast_to(ddf[:, sl], (8, 128))
                g8 = jnp.broadcast_to(gwf[:, sl], (8, 128))
                bc[6 * t + 5] = g8
                gwm[:, sl] = jnp.concatenate([pltpu.pack_elementwise([g8, g8], packed_dtype=BF16)] * 8, axis=0)

        def WT(c):
            for i in range(NT):
                tile = wqb[pl.ds(i * 128, 128), pl.ds(c * 128, 128)]
                wt[i, pl.ds(c * 128, 128), :] = lax.dot_general(emat(0), tile, NT_DIMS, preferred_element_type=F32)

        def WP(part, t):
            for j in range(4 * t, 4 * t + 4):
                src0 = part * D + j
                dst0 = (part * DH + j) * 16
                for i in range(NT):
                    for m in range(2):
                        a = wt[i, pl.ds(src0 + 320 * m, 8, stride=2 * DH), :]
                        b = wt[i, pl.ds(src0 + 320 * m + DH, 8, stride=2 * DH), :]
                        if part == 0:
                            a, b = a * cexp, b * cexp
                        wtp[pl.ds(dst0 + 8 * m, 8), i * 128:(i + 1) * 128] = pltpu.pack_elementwise([a, b], packed_dtype=BF16)

        def WO(i):
            wof[i] = wob[:, i * 128:(i + 1) * 128].astype(F32)
            for j in range(DH):
                for m in range(2):
                    a = wof[i, pl.ds(j + 320 * m, 8, stride=2 * DH), :]
                    b = wof[i, pl.ds(j + 320 * m + DH, 8, stride=2 * DH), :]
                    wop[pl.ds(j * 16 + 8 * m, 8), i * 128:(i + 1) * 128] = pltpu.pack_elementwise([a, b], packed_dtype=BF16)

        def X(i):
            xs[pl.ds(i * 64, 64), :] = pltpu.bitcast(qb[rows(i), :], U32)

        def P(i, n):
            xblk = pltpu.bitcast(xs[pl.ds(i * 64, 64), :], BF16)
            wn = pltpu.bitcast(wtp[pl.ds(n * 64, 64), :], BF16)
            res = lax.dot_general(xblk, wn, NT_DIMS, preferred_element_type=F32)
            mark(res)
            part, t = divmod(n, NT)
            if part == 0:
                qs[t, rows(i), :] = res
            elif part == 1:
                ks[t, pl.ds(PAD + i * BLK, BLK), :] = res
            else:
                vs[t, pl.ds(PAD + i * BLK, BLK), :] = res

        def TL(i, p, c):
            r = i * BLK + 16 * p + 8 * c
            qv = [qs[t, pl.ds(r, 8), :] for t in range(NT)]
            qv[0] = dep(qv[0])
            ls = []
            for w in range(WIN):
                l = qv[0] * ks[0, pl.ds(PAD + r - DIL * w, 8), :]
                for t in range(1, NT):
                    l = l + qv[t] * ks[t, pl.ds(PAD + r - DIL * w, 8), :]
                ls.append(l)
            lgs[i % 4, p, pl.ds(64 * c, 64), :] = jnp.concatenate(ls, axis=0).astype(BF16)

        def TRR(i, p, st):
            st["red"] = jnp.dot(words(lgs, i % 4, p), emat(1), preferred_element_type=F32)
            mark(st["red"][:64])
            st["outs"] = []

        def TRS(i, p, c, st):
            b0 = i * BLK + 16 * p
            red = st["red"]
            r = b0 + 8 * c
            lw = [red[(c * WIN + w) * 8:(c * WIN + w + 1) * 8] for w in range(WIN)]
            lw[0] = dep(lw[0]) if trsplit else lw[0]
            if r < DIL * (WIN - 1):
                pos = r + lax.broadcasted_iota(jnp.int32, (8, 128), 0)
                lw = [jnp.where(pos >= DIL * w, lw[w], -1e30) for w in range(WIN)]
            m = lw[0]
            for w in range(1, WIN):
                m = jnp.maximum(m, lw[w])
            e = [jnp.exp2(lw[w] - m) for w in range(WIN)]
            den = e[0]
            for w in range(1, WIN):
                den = den + e[w]
            rinv = pl.reciprocal(den, approx=True)
            oc = [e[0] * vs[t, pl.ds(PAD + r, 8), :] for t in range(NT)]
            for w in range(1, WIN):
                oc = [oc[t] + e[w] * vs[t, pl.ds(PAD + r - DIL * w, 8), :] for t in range(NT)]
            st["outs"].append([oc[t] * rinv for t in range(NT)])
            if c == 1:
                outs = st["outs"]
                for t in range(NT):
                    ob[t, pl.ds(b0, 16), :] = jnp.concatenate([outs[0][t], outs[1][t]], axis=0).astype(BF16)

        def tr_steps(i):
            out = []
            for p in range(8):
                st = {}
                out += [(32, pt(TRR, i, p, st)), (30, pt(TRS, i, p, 0, st)), (30, pt(TRS, i, p, 1, st))]
            return out

        def GA(i):
            zp = None
            for t in range(NT):
                g8 = dep(bc[6 * t + 5]) if t == 0 else bc[6 * t + 5]
                term = qb[rows(i), t * 128:(t + 1) * 128].astype(F32) * rep(g8, 16)
                zp = term if zp is None else zp + term
            gps[i] = zp.astype(BF16)

        def GB(i):
            if gate == "valu":
                z = jnp.dot(words(gps, i), emat(2), preferred_element_type=F32)
            else:
                xblk = pltpu.bitcast(xs[pl.ds(i * 64, 64), :], BF16)
                z = lax.dot_general(xblk, pltpu.bitcast(gwm[...], BF16), NT_DIMS, preferred_element_type=F32)
            mark(z)
            gs[rows(i), :] = 0.5 + 0.5 * jnp.tanh(0.5 * z)

        def O(i, n):
            sl = slice(n * 128, (n + 1) * 128)
            obw = ob.bitcast(U32)
            o = pltpu.bitcast(jnp.concatenate([obw[t, pl.ds(i * 64, 64), :] for t in range(NT)], axis=1), BF16)
            bo = jnp.dot(o, pltpu.bitcast(wop[:, sl], BF16), preferred_element_type=F32)
            mark(bo)
            a_br = qb[rows(i), sl].astype(F32) * yy[n, rows(i), :]
            outb[rows(i), sl] = (bo + gs[rows(i), :] * (a_br - bo)).astype(BF16)

        def KV(t, a, ms):
            kw, vw = kb.bitcast(U32), vb.bitcast(U32)
            lo = lambda x: pltpu.unpack_elementwise(x, index=0, packed_dtype=BF16, unpacked_dtype=F32)
            hi = lambda x: pltpu.unpack_elementwise(x, index=1, packed_dtype=BF16, unpacked_dtype=F32)
            c = [dep(bc[6 * t])] + [bc[6 * t + j] for j in range(1, 4)]
            for m in ms:
                base = 8 + 64 * a + 8 * m
                p0, p1, p2 = kw[t, pl.ds(base, 8), :], kw[t, pl.ds(base - 1, 8), :], kw[t, pl.ds(base - 2, 8), :]
                l0, h0, l1, h1, h2 = lo(p0), hi(p0), lo(p1), hi(p1), hi(p2)
                ev = c[0] * l0 + c[1] * h1 + c[2] * l1 + c[3] * h2
                od = c[0] * h0 + c[1] * l0 + c[2] * h1 + c[3] * l1
                vv = vw[t, pl.ds(64 * a + 8 * m, 8), :]
                kvs[t % 2][a, pl.ds(8 * m, 8), :] = pltpu.pack_elementwise([ev * lo(vv), od * hi(vv)], packed_dtype=BF16)

        def FU(t, a):
            u3 = u3s[t % 3]
            uu = jnp.dot(fmat(a), pltpu.bitcast(kvs[t % 2][a], BF16), preferred_element_type=F32)
            mark(uu[:64])
            uu = uu.reshape(NG, 2, 8, 128)
            ar, ai = uu[:, 0], uu[:, 1]
            u3[0, a, pl.ds(0, NG)] = ar + ai
            u3[1, a, pl.ds(0, NG)] = ar
            u3[2, a, pl.ds(0, NG)] = ai

        def FH(t, a):
            h3 = h3s[t % 3]
            hblk = hb[pl.ds(t * 128, 128), pl.ds(a * BLK, BLK)]
            hh = lax.dot_general(fmat(a), hblk, NT_DIMS, preferred_element_type=F32)
            mark(hh[:64])
            hh = hh.reshape(NG, 2, 8, 128)
            br, bi = hh[:, 0], hh[:, 1]
            h3[0, a, pl.ds(0, NG)] = br
            h3[1, a, pl.ds(0, NG)] = bi - br
            h3[2, a, pl.ds(0, NG)] = br + bi

        def TPA(t, g, comp, part, cache):
            u3, h3, ac = u3s[t % 3], h3s[t % 3], acs[t % 2]
            if part == 0:
                dv = bc[6 * t + 4]
                cache["u"] = [u3[comp, a, g] for a in range(NB)]
                hv = [h3[comp, a, g] for a in range(NB)]
                hv[0] = hv[0] - dv if comp == 1 else hv[0] + dv
                cache["h"] = hv
            uv, hv = cache["u"], cache["h"]
            h0 = dep(hv[0])
            if tp_order == "chain":
                for a in tp_parts[part]:
                    s = h0 * uv[a]
                    for d in range(1, a + 1):
                        s = s + hv[d] * uv[a - d]
                    ac[comp, a, g] = s
            else:
                outs = tp_parts[part]
                s = {a: h0 * uv[a] for a in outs}
                for d in range(1, max(outs) + 1):
                    for a in outs:
                        if a >= d:
                            s[a] = s[a] + hv[d] * uv[a - d]
                for a in outs:
                    ac[comp, a, g] = s[a]

        def TPB(t, g):
            ac, zs = acs[t % 2], zss[t % 3]
            prev = None
            for a in range(NB):
                a1 = ac[0, a, g]
                if a == 0:
                    a1 = dep(a1)
                cr, ci = a1 - ac[2, a, g], a1 + ac[1, a, g]
                zr, zi = (cr, ci) if prev is None else (cr - prev[1], ci + prev[0])
                prev = (cr, ci)
                zs[a, pl.ds(g * 8, 8), :] = pltpu.pack_elementwise([zr, zi], packed_dtype=BF16)

        def IV(t, a):
            z = pltpu.bitcast(zss[t % 3][a], BF16)
            y = jnp.dot(gmat(a), z, preferred_element_type=F32)
            mark(y[:64])
            yy[t, rows(a), :] = y

        def step_of(order, fn):
            names = [f.func.__name__ for f in order]
            per = {"P": 16, "O": 16, "GB": 16, "FU": 8, "FH": 8, "IV": 8, "TRR": 8}
            nm = sum(per.get(n, 0) for n in names)
            npaced = sum(n in pace.split(",") for n in names)
            return max(1, int(mscale * nm) // max(1, npaced))

        def run(fns):
            for fn in fns:
                fn()

        scope = (lambda n: jax.named_scope(n)) if scopes else (lambda n: contextlib.nullcontext())
        with scope("ep00a"):
            start("Wq0", "Wq1", "q01", "z", "Wk", "Wv", "q2", "misc", "q3", "A0", "q45", "A1", "q67", "A2", "Wo", "A3", "q8f", "A4")
            setup_masks()
            wait("Wq0")
            run([pt(WT, c) for c in range(2)])
            wait("Wq1", "q01", "z")
            run([pt(WT, c) for c in range(2, 5)])
            run([pt(X, 0), pt(X, 1)])
            run([pt(WP, 0, t) for t in range(NT)])
            run([pt(P, 0, n) for n in range(5)])
        with scope("ep00b"):
            wait("Wk")
            run([pt(WT, c) for c in range(5, 10)])
            run([pt(P, 1, n) for n in range(2)])
            run([pt(WP, 1, t) for t in range(NT)])
            run([pt(P, 0, n) for n in range(5, 10)])
        with scope("ep00c"):
            wait("Wv", "q2", "misc")
            setup_misc()
            run([pt(X, 2)])
            run([pt(WT, c) for c in range(10, 15)])
            run([pt(P, 1, n) for n in range(2, 4)])
            run([pt(WP, 2, t) for t in range(NT)])
            run([pt(P, 0, n) for n in range(10, 15)])

        def ga_of(e):
            return plan[e + 1]["GB"] if (gate == "valu" and e + 1 in plan) else []

        def first_epoch(pred):
            return min(e for e in plan if pred(plan[e]))
        waits = {}
        for nm in ("q3", "q45", "q67", "q8f"):
            i0 = qgroups[nm][0]
            waits.setdefault(first_epoch(lambda pe: any(i >= i0 for i in pe["X"])), []).append(nm)
        for t in range(NT):
            waits.setdefault(first_epoch(lambda pe: any(x[0] == t for x in pe["KV"] + pe["FH"])), []).append("A%d" % t)
        waits.setdefault(first_epoch(lambda pe: pe["WO"]), []).append("Wo")
        starts = {}
        if waits_override:
            waits = waits_override
        out_groups = []
        done_o = set()
        sent = {n: 0 for n in range(NT)}
        sent_rows = [0]
        sk = skip.split(",")
        for e in range(1, nep + 1):
            with scope("ep%02d" % e):
                if e in waits:
                    wait(*waits[e])
                elif e in barriers and e not in starts:
                    barrier()
                if e in starts:
                    start(*starts[e])
                pe = {k: (v if k not in sk else []) for k, v in plan[e].items()}
                streams = [
                    [(160, pt(P, i, n)) for i in pe["P"] for n in range(4 if i == 1 else 0, 3 * NT)],
                    [(160, pt(O, *x)) for x in pe["O"]],
                    [(64, pt(FH, *x)) for x in pe["FH"]] ,
                    [(64, pt(FU, *x)) for x in pe["FU"]],
                    [(64, pt(IV, *x)) for x in pe["IV"]],
                    [(160 if gate != "valu" else 32, pt(GB, i)) for i in pe["GB"]],
                    [s for i in pe["TR"] for s in tr_steps(i)],
                    [(10, pt(X, i)) for i in pe["X"]] + [(20, pt(TL, i, p, c)) for i in pe["TL"] for p in range(8) for c in range(2)],
                    [(60, pt(GA, i)) for i in ga_of(e)],
                    [(48 // kvsplit, pt(KV, *x, tuple(range(8 * s // kvsplit, 8 * (s + 1) // kvsplit)))) for x in pe["KV"] for s in range(kvsplit)],
                    [(20, pt(TPB, *x)) for x in pe["TPB"]],
                    [(30, pt(WO, i)) for i in pe["WO"]],
                ]
                lst = []
                for (t, g) in pe["TPA"]:
                    for c in range(3):
                        cache = {}
                        lst += [(16, pt(TPA, t, g, c, part, cache)) for part in range(len(tp_parts))]
                streams.append(lst)
                order = _interleave(streams, [mshift if k < 6 else 0.0 for k in range(len(streams))])
                hard = (e in waits) or (e in barriers) or scopes
                state["marks"] = [] if hard else state["marks"][-keep:]
                paced = set(pace.split(",")) if pace else set()
                seen = len(state["marks"])
                for fn in order:
                    if fn.func.__name__ in paced and state["marks"]:
                        marks = state["marks"]
                        idx = max(0, min(len(marks) - 1, seen - lag))
                        state["use"] = marks[idx]
                        seen = min(len(marks), seen + step_of(order, fn))
                    else:
                        state["use"] = None
                    fn()
                state["use"] = None
                done_o.update(plan[e]["O"])
                if out_mode == "strip":
                    for n in range(NT):
                        i1 = sent[n]
                        while i1 < NB and (i1, n) in done_o:
                            i1 += 1
                        if i1 - sent[n] >= out_chunk or (i1 > sent[n] and (i1 == NB or e >= nep - 1)):
                            cols = pl.ds(n * 128, 128)
                            cp = pltpu.make_async_copy(outb.at[rows(sent[n], i1), cols], out_hbm.at[0, rows(sent[n], i1), cols],
                                                       sem_o.at[len(out_groups)])
                            cp.start()
                            out_groups.append(cp)
                            sent[n] = i1
                else:
                    i1 = sent_rows[0]
                    while i1 < NB and all((i1, n) in done_o for n in range(NT)):
                        i1 += 1
                    if i1 > sent_rows[0] and (out_eps is None or e in out_eps or e == nep):
                        cp = pltpu.make_async_copy(outb.at[rows(sent_rows[0], i1), :], out_hbm.at[0, rows(sent_rows[0], i1), :],
                                                   sem_o.at[len(out_groups)])
                        cp.start()
                        out_groups.append(cp)
                        sent_rows[0] = i1
        for cp in out_groups:
            cp.wait()

    scratch = [
        pltpu.VMEM((S, D), BF16),
        pltpu.VMEM((NT, S + 16, 128), BF16),
        pltpu.VMEM((NT, S, 128), BF16),
        pltpu.VMEM((D, S + 128), BF16),
        pltpu.VMEM((D, 3 * D), BF16),
        pltpu.VMEM((D, D), BF16),
        pltpu.VMEM((4, D), BF16),
        pltpu.VMEM((D,), BF16),
        pltpu.VMEM((D,), BF16),
        pltpu.VMEM((256, 128), U32),
        pltpu.VMEM((2, 128, 128), U32),
        pltpu.VMEM((2, 2, 64, 128), U32),
        pltpu.VMEM((3, 64, 128), U32),
        pltpu.VMEM((6 * NT, 8, 128), F32),
        pltpu.VMEM((NT, 3 * D, 128), F32),
        pltpu.VMEM((3 * D // 2, D), U32),
        pltpu.VMEM((NT, D, 128), F32),
        pltpu.VMEM((D // 2, D), U32),
        pltpu.VMEM((S // 2, D), U32),
        pltpu.VMEM((NT, S + 8, 128), F32),
        pltpu.VMEM((NT, S + PAD + 8, 128), F32),
        pltpu.VMEM((NT, S + PAD + 8, 128), F32),
        pltpu.VMEM((4, 8, 128, 128), BF16),
        pltpu.VMEM((NT, S, 128), BF16),
        pltpu.VMEM((64, D), U32),
        pltpu.VMEM((NB, BLK, 128), BF16),
        pltpu.VMEM((S, 128), F32),
        pltpu.VMEM((S + 8, 128), F32),
        pltpu.VMEM((S + 8, 128), F32),
        pltpu.VMEM((NB, 64, 128), U32),
        pltpu.VMEM((NB, 64, 128), U32),
        pltpu.VMEM((3, NB, NG + 1, 8, 128), F32),
        pltpu.VMEM((3, NB, NG + 1, 8, 128), F32),
        pltpu.VMEM((3, NB, NG + 1, 8, 128), F32),
        pltpu.VMEM((3, NB, NG + 1, 8, 128), F32),
        pltpu.VMEM((3, NB, NG + 1, 8, 128), F32),
        pltpu.VMEM((3, NB, NG + 1, 8, 128), F32),
        pltpu.VMEM((3, NB, NG + 1, 8, 128), F32),
        pltpu.VMEM((3, NB, NG + 1, 8, 128), F32),
        pltpu.VMEM((NB, BLK, 128), U32),
        pltpu.VMEM((NB, BLK, 128), U32),
        pltpu.VMEM((NB, BLK, 128), U32),
        pltpu.VMEM((NT, S, 128), F32),
        pltpu.VMEM((S, D), BF16),
        pltpu.VMEM((24, 8, 128), F32),
        pltpu.VMEM((24, 8, 128), U32),
        pltpu.SemaphoreType.DMA((40,)),
        pltpu.SemaphoreType.DMA((32,)),
        pltpu.SemaphoreType.REGULAR,
        pltpu.SemaphoreType.DMA((48,)),
        pltpu.SMEM((8,), jnp.int32),
    ]

    consts = _dft_constants()

    @jax.jit
    def run_kernel(A_q, A_k, A_v, A_shift_k, A_ssm_k, A_ssm_D, B_x, B_wqkv, B_wo, gate_w):
        return pl.pallas_call(
            kernel,
            out_shape=jax.ShapeDtypeStruct((1, S, D), BF16),
            in_specs=[pl.BlockSpec(memory_space=pl.ANY)] * 11,
            out_specs=pl.BlockSpec(memory_space=pl.ANY),
            scratch_shapes=scratch,
            compiler_params=pltpu.CompilerParams(vmem_limit_bytes=110 * 1024 * 1024),
        )(A_q, A_k, A_v, A_shift_k.T, A_ssm_k, A_ssm_D, B_wqkv, B_wo, gate_w, jnp.asarray(consts), jnp.asarray(np.zeros((8,), np.int32)))

    return run_kernel


pallas_gated_mix__ssm_conv_h3__sliding_local_dilated__prompt_kernel = make_kernel()
```

```python
import contextlib
import functools
import math

import numpy as np
import jax
import jax.numpy as jnp
from jax import lax
from jax.experimental import pallas as pl
from jax.experimental.pallas import tpu as pltpu

S, D = 2048, 640
NT = D // 128
BLK = 128
NB = S // BLK
NG = 16
H, DH, WIN, DIL = 32, 20, 8, 2
PAD = 16
F32, BF16, U32 = jnp.float32, jnp.bfloat16, jnp.uint32
NT_DIMS = (((1,), (1,)), ((), ()))
ONE_LO, ONE_HI = 0x3F80, 0x3F800000
pt = functools.partial


def _pack_rows(m):
    b = np.asarray(m, dtype=np.float32).astype(BF16).view(np.uint16).astype(np.uint32)
    return b[0::2] | (b[1::2] << 16)


def _dft_constants():
    k = np.arange(BLK)
    n = np.arange(BLK)
    th = 2.0 * np.pi * (k[:, None] + 0.5) * n[None, :] / (2 * BLK)
    fwd = np.stack([np.cos(th).reshape(NG, 8, BLK), -np.sin(th).reshape(NG, 8, BLK)], axis=1).reshape(2 * BLK, BLK)
    order = np.arange(BLK).reshape(8, 8, 2).transpose(0, 2, 1).reshape(BLK)
    inv = np.stack([(np.cos(th).T / BLK).reshape(BLK, NG, 8), (-np.sin(th).T / BLK).reshape(BLK, NG, 8)], axis=2)
    pi = _pack_rows(inv.reshape(BLK, 2 * BLK))
    return np.concatenate([_pack_rows(fwd), _pack_rows(fwd[:, order]), pi[:, :BLK], pi[:, BLK:]], axis=0)


def _interleave(streams):
    items = []
    for si, s in enumerate(streams):
        tot = float(sum(w for w, _ in s))
        acc = 0.0
        for w, fn in s:
            items.append(((acc + 0.5 * w) / tot, si, fn))
            acc += w
    items.sort(key=lambda x: (x[0], x[1]))
    return [fn for _, _, fn in items]


MXU_COST = dict(P=2400, TR=256, GB=32, FU=64, FH=64, IV=64, O=160)
KEYS = ("P", "TL", "TR", "GA", "GB", "KV", "FU", "FH", "TP", "IV", "O", "WO")


def make_plan(tl_ep=(1, 2, 2, 3, 5, 7, 9, 11, 12, 13, 14, 14, 15, 15, 16, 16), tp0=4, a0=2, rate=8.0, wo_epoch=6,
              m_target=4600, a_ready=(2, 3, 4, 5, 7)):
    p_ep = [0, 1, 1] + list(range(2, 15))
    nep = max(tl_ep) + 2
    plan = {e: {k: [] for k in KEYS} for e in range(1, nep + 1)}
    for i in range(1, NB):
        plan[p_ep[i]]["P"].append(i)
    gb_ep = {}
    for i in range(NB):
        assert tl_ep[i] > p_ep[i], i
        plan[tl_ep[i]]["TL"].append(i)
        plan[tl_ep[i] + 1]["TR"].append(i)
        gb_ep[i] = max(3, tl_ep[i] + 1)
        plan[gb_ep[i]]["GB"].append(i)
        plan[gb_ep[i] - 1]["GA"].append(i)
    ep_tp = [tp0 + int(v / rate) for v in range(NT * NG)]
    for v, e in enumerate(ep_tp):
        plan[e]["TP"].append(divmod(v, NG))
    plan[a0]["KV"] = [(0, a) for a in range(NB)]
    plan[a0]["FH"] = [(0, a) for a in range(NB)]
    plan[tp0 - 1]["FU"] += [(0, a) for a in range(NB)]
    fu_done = {0: tp0 - 1}
    for t in range(1, NT):
        last = ep_tp[NG * t] - 1
        first = max(a0 + 2, ep_tp[NG * (t - 1)], a_ready[t] + 1)
        if t >= 3:
            first = max(first, ep_tp[NG * (t - 3) + NG - 1] + 1)
        if t >= 2:
            first = max(first, fu_done[t - 2] + 2)
        eps = list(range(first, last + 1))
        assert eps, (t, first, last)
        for a in range(NB):
            e = eps[a * len(eps) // NB]
            plan[e]["FU"].append((t, a))
            plan[e]["FH"].append((t, a))
            plan[e - 1]["KV"].append((t, a))
        fu_done[t] = last
    iv_ep = {}
    for t in range(NT):
        e0 = ep_tp[NG * t + NG - 1] + 1
        for a in range(NB):
            iv_ep[(t, a)] = e0 + (a >= NB // 2 and t < NT - 1)
            plan[iv_ep[(t, a)]]["IV"].append((t, a))
        if t >= 3:
            assert max(iv_ep[(t - 3, a)] for a in range(NB)) < ep_tp[NG * t]
    plan[wo_epoch]["WO"] = list(range(NT))

    def mxu(e):
        return sum(MXU_COST.get(k, 0) * len(v) for k, v in plan[e].items())
    todo = [(i, n) for n in range(NT) for i in range(NB)]
    for e in range(wo_epoch + 1, nep + 1):
        avail = [x for x in todo if iv_ep[(x[1], x[0])] < e and tl_ep[x[0]] + 1 < e and gb_ep[x[0]] < e]
        avail.sort()
        for x in avail:
            if e < nep and mxu(e) + MXU_COST["O"] > m_target:
                break
            plan[e]["O"].append(x)
            todo.remove(x)
    assert not todo, todo
    return plan


Q_GROUPS = {"q0": (0, 1), "q1": (1, 2), "q2": (2, 3), "q3": (3, 4), "q45": (4, 6), "q67": (6, 8), "q8f": (8, 16)}
DMA_ORDER = ("tiny", "z", "Wq0", "Wq1", "q0", "q1", "Wk", "Wv", "q2", "misc", "q3", "A0", "q45", "A1", "q67", "A2", "Wo", "A3",
             "q8f", "A4")
WAITS = {1: ("q3",), 2: ("A0", "q45"), 3: ("A1", "q67"), 5: ("A2",), 6: ("Wo", "A3", "q8f"), 8: ("A4",)}


def make_kernel(plan_kw=None, scopes=False, barriers=(10, 12, 15), waits=WAITS, dma_order=DMA_ORDER,
                tp_blocks=((15, 14, 13, 12), (11, 10, 9, 8), (7, 6, 5, 4, 3, 2, 1, 0)),
                pace=("TL", "KV", "TP", "GA"), keep=16, kvsplit=2):
    plan = make_plan(**(plan_kw or {}))
    nep = max(plan)

    def kernel(q_hbm, k_hbm, v_hbm, sk_hbm, h_hbm, dd_hbm, wqkv_hbm, wo_hbm, gw_hbm, c_hbm, z_hbm, out_hbm,
               qb, kb, vb, hb, wqb, wob, skb, ddb, gwb, cb,
               fm, fp, gm, em, bc,
               wt, wtp, wof, wop,
               qs, ks, vs, lgs, ob, gps, gs,
               kva, kvb, u3a, u3b, u3c, h3a, h3b, h3c, zsa, zsb, zsc, yy, outb,
               sem_in, sem_o, sem_b, zsm):
        kvs, u3s, h3s, zss = (kva, kvb), (u3a, u3b, u3c), (h3a, h3b, h3c), (zsa, zsb, zsc)

        def rows(i0, i1=None):
            i1 = i0 + 1 if i1 is None else i1
            return pl.ds(i0 * BLK, (i1 - i0) * BLK)

        copies = {}
        nsem = [0]

        def add_copy(name, src, dst):
            copies.setdefault(name, []).append(pltpu.make_async_copy(src, dst, sem_in.at[nsem[0]]))
            nsem[0] += 1

        add_copy("Wq0", wqkv_hbm.at[:, pl.ds(0, 256)], wqb.at[:, pl.ds(0, 256)])
        add_copy("Wq1", wqkv_hbm.at[:, pl.ds(256, 384)], wqb.at[:, pl.ds(256, 384)])
        for part, nm in ((1, "Wk"), (2, "Wv")):
            add_copy(nm, wqkv_hbm.at[:, pl.ds(part * D, D)], wqb.at[:, pl.ds(part * D, D)])
        add_copy("z", z_hbm, zsm)
        add_copy("misc", c_hbm, cb)
        add_copy("tiny", sk_hbm, skb)
        add_copy("tiny", dd_hbm, ddb)
        add_copy("tiny", gw_hbm, gwb)
        add_copy("Wo", wo_hbm, wob)
        for nm, (i0, i1) in Q_GROUPS.items():
            for t in range(NT):
                add_copy(nm, q_hbm.at[0, rows(i0, i1), pl.ds(t * 128, 128)], qb.at[t, rows(i0, i1), :])
        for t in range(NT):
            add_copy("A%d" % t, h_hbm.at[pl.ds(t * 128, 128), :], hb.at[pl.ds(t * 128, 128), pl.ds(0, S)])
            add_copy("A%d" % t, k_hbm.at[0, :, pl.ds(t * 128, 128)], kb.at[t, pl.ds(16, S), :])
            add_copy("A%d" % t, v_hbm.at[0, :, pl.ds(t * 128, 128)], vb.at[t])

        def wait(*names):
            for nm in names:
                for c in copies[nm]:
                    c.wait()

        def barrier():
            pl.semaphore_signal(sem_b, 1)
            pl.semaphore_wait(sem_b, 1)

        state = {"marks": [], "use": None}

        def dep(x):
            if state["use"] is None:
                return x
            never = lax.broadcasted_iota(jnp.int32, (8, 128), 0) < zsm[0]
            return jnp.where(never, state["use"], x)

        def mark(res):
            state["marks"] += [res[8 * j:8 * j + 8] for j in range(res.shape[0] // 8)]

        def rep(v, n):
            return jnp.concatenate([v] * n, axis=0)

        def words(ref, *idx):
            return ref.bitcast(U32)[idx]

        def as_bf16(w):
            return pltpu.bitcast(w, BF16)

        def as_f32(w):
            return pltpu.bitcast(w, F32)

        def wide(ref, r0, n):
            return as_bf16(jnp.concatenate([words(ref, t, pl.ds(r0, n)) for t in range(NT)], axis=1))

        emat = lambda j: as_bf16(em[j])
        cexp = (DH ** -0.5) * math.log2(math.e)

        def setup_masks():
            r = lax.broadcasted_iota(jnp.int32, (64, 128), 0)
            l = lax.broadcasted_iota(jnp.int32, (64, 128), 1)
            lo, hi, zero = jnp.uint32(ONE_LO), jnp.uint32(ONE_HI), jnp.uint32(0)
            em[0] = jnp.where(l == 2 * r, lo, zero) | jnp.where(l == 2 * r + 1, hi, zero)
            em[1] = jnp.where((l & 31) == ((2 * r) & 31), lo, zero) | jnp.where((l & 31) == ((2 * r + 1) & 31), hi, zero)
            em[2] = jnp.full((64, 128), ONE_LO | ONE_HI, U32)
            for t in range(NT):
                ks[t, pl.ds(0, PAD), :] = jnp.zeros((PAD, 128), F32)
                vs[t, pl.ds(0, PAD), :] = jnp.zeros((PAD, 128), F32)
                kb[t, pl.ds(0, 16), :] = jnp.zeros((16, 128), BF16)

        def setup_dft():
            for ref, r0 in ((fm, 0), (fp, 128)):
                f = cb[pl.ds(r0, 128), :]
                ref[0] = f
                ref[1] = f ^ jnp.uint32(0x80000000)
            l = lax.broadcasted_iota(jnp.int32, (64, 128), 1)
            flip = jnp.where((l & 1) != 0, jnp.uint32(0x80008000), jnp.uint32(0))
            for hf in range(2):
                g = cb[pl.ds(256 + 64 * hf, 64), :]
                gm[0, hf] = g
                gm[1, hf] = g ^ flip

        def setup_rows():
            skf = skb[...].astype(F32)
            ddf = ddb[...].astype(F32).reshape(1, D)
            gwf = gwb[...].astype(F32).reshape(1, D)
            for t in range(NT):
                sl = slice(t * 128, (t + 1) * 128)
                for j in range(4):
                    bc[6 * t + j] = jnp.broadcast_to(skf[j:j + 1, sl], (8, 128))
                bc[6 * t + 4] = jnp.broadcast_to(ddf[:, sl], (8, 128))
                bc[6 * t + 5] = jnp.broadcast_to(gwf[:, sl], (8, 128))

        def WT(c):
            for i in range(NT):
                tile = wqb[pl.ds(i * 128, 128), pl.ds(c * 128, 128)]
                wt[i, pl.ds(c * 128, 128), :] = lax.dot_general(emat(0), tile, NT_DIMS, preferred_element_type=F32)

        def head_major(src, i, base):
            return jnp.concatenate([src[i, pl.ds(base, 8, stride=DH), :], src[i, pl.ds(base + 8 * DH, 8, stride=DH), :]], axis=0)

        def WP(part, t):
            for j in range(4 * t, 4 * t + 4):
                for i in range(NT):
                    for m in range(2):
                        w = head_major(wt, i, part * D + j + 16 * DH * m)
                        if part == 0:
                            w = w * cexp
                        wtp[i, pl.ds((part * DH + j) * 32 + 16 * m, 16), :] = w.astype(BF16)

        def WO(n):
            wof[n] = wob[:, n * 128:(n + 1) * 128].astype(F32)
            for j in range(DH):
                for m in range(2):
                    wop[n, pl.ds(j * 32 + 16 * m, 16), :] = head_major(wof, n, j + 16 * DH * m).astype(BF16)

        def P(i, n):
            res = lax.dot_general(wide(qb, i * 64, 64), wide(wtp, n * 64, 64), NT_DIMS, preferred_element_type=F32)
            mark(res)
            part, t = divmod(n, NT)
            if part == 0:
                qs[t, rows(i), :] = res
            elif part == 1:
                ks[t, pl.ds(PAD + i * BLK, BLK), :] = res
            else:
                vs[t, pl.ds(PAD + i * BLK, BLK), :] = res

        def TL(i, p, c):
            r = i * BLK + 16 * p + 8 * c
            qv = [qs[t, pl.ds(r, 8), :] for t in range(NT)]
            qv[0] = dep(qv[0])
            ls = []
            for w in range(WIN):
                l = qv[0] * ks[0, pl.ds(PAD + r - DIL * w, 8), :]
                for t in range(1, NT):
                    l = l + qv[t] * ks[t, pl.ds(PAD + r - DIL * w, 8), :]
                ls.append(l)
            lgs[i % 4, p, pl.ds(64 * c, 64), :] = jnp.concatenate(ls, axis=0).astype(BF16)

        def TR(i, p):
            b0 = i * BLK + 16 * p
            red = jnp.dot(as_bf16(words(lgs, i % 4, p)), emat(1), preferred_element_type=F32)
            mark(red[:64])
            outs = []
            for c in range(2):
                r = b0 + 8 * c
                lw = [red[(c * WIN + w) * 8:(c * WIN + w + 1) * 8] for w in range(WIN)]
                if r < DIL * (WIN - 1):
                    pos = r + lax.broadcasted_iota(jnp.int32, (8, 128), 0)
                    lw = [jnp.where(pos >= DIL * w, lw[w], -1e30) for w in range(WIN)]
                m = lw[0]
                for w in range(1, WIN):
                    m = jnp.maximum(m, lw[w])
                e = [jnp.exp2(lw[w] - m) for w in range(WIN)]
                den = e[0]
                for w in range(1, WIN):
                    den = den + e[w]
                rinv = pl.reciprocal(den, approx=True)
                oc = [e[0] * vs[t, pl.ds(PAD + r, 8), :] for t in range(NT)]
                for w in range(1, WIN):
                    oc = [oc[t] + e[w] * vs[t, pl.ds(PAD + r - DIL * w, 8), :] for t in range(NT)]
                outs.append([oc[t] * rinv for t in range(NT)])
            for t in range(NT):
                ob[t, pl.ds(b0, 16), :] = jnp.concatenate([outs[0][t], outs[1][t]], axis=0).astype(BF16)

        def GA(i):
            zp = None
            for t in range(NT):
                g8 = dep(bc[6 * t + 5]) if t == 0 else bc[6 * t + 5]
                term = qb[t, rows(i), :].astype(F32) * rep(g8, 16)
                zp = term if zp is None else zp + term
            gps[i] = zp.astype(BF16)

        def GB(i):
            z = jnp.dot(as_bf16(words(gps, i)), emat(2), preferred_element_type=F32)
            mark(z)
            gs[rows(i), :] = 0.5 + 0.5 * jnp.tanh(0.5 * z)

        def O(i, n):
            bo = jnp.dot(wide(ob, i * 64, 64), as_bf16(words(wop, n)), preferred_element_type=F32)
            mark(bo)
            a_br = qb[n, rows(i), :].astype(F32) * yy[n, rows(i), :]
            outb[rows(i), n * 128:(n + 1) * 128] = (bo + gs[rows(i), :] * (a_br - bo)).astype(BF16)

        def KV(t, a, ms):
            lo = lambda x: as_f32(x << 16)
            hi = lambda x: as_f32(x & jnp.uint32(0xFFFF0000))
            c = [dep(bc[6 * t])] + [bc[6 * t + j] for j in range(1, 4)]
            for m in ms:
                base = 8 + 64 * a + 8 * m
                p0, p1, p2 = (words(kb, t, pl.ds(base - j, 8)) for j in range(3))
                l0, h0, l1, h1, h2 = lo(p0), hi(p0), lo(p1), hi(p1), hi(p2)
                ev = c[0] * l0 + c[1] * h1 + c[2] * l1 + c[3] * h2
                od = c[0] * h0 + c[1] * l0 + c[2] * h1 + c[3] * l1
                vv = words(vb, t, pl.ds(64 * a + 8 * m, 8))
                kvs[t % 2][a, pl.ds(16 * m, 16), :] = jnp.concatenate([ev * lo(vv), od * hi(vv)], axis=0).astype(BF16)

        def FU(t, a):
            u3 = u3s[t % 3]
            uu = jnp.dot(as_bf16(fp[a % 2]), as_bf16(words(kvs[t % 2], a)), preferred_element_type=F32)
            mark(uu[:64])
            uu = uu.reshape(NG, 2, 8, 128)
            ar, ai = uu[:, 0], uu[:, 1]
            u3[0, a, pl.ds(0, NG)] = ar + ai
            u3[1, a, pl.ds(0, NG)] = ar
            u3[2, a, pl.ds(0, NG)] = ai

        def FH(t, a):
            h3 = h3s[t % 3]
            hblk = hb[pl.ds(t * 128, 128), pl.ds(a * BLK, BLK)]
            hh = lax.dot_general(as_bf16(fm[a % 2]), hblk, NT_DIMS, preferred_element_type=F32)
            mark(hh[:64])
            hh = hh.reshape(NG, 2, 8, 128)
            br, bi = hh[:, 0], hh[:, 1]
            h3[0, a, pl.ds(0, NG)] = br
            h3[1, a, pl.ds(0, NG)] = bi - br
            h3[2, a, pl.ds(0, NG)] = br + bi

        def TP(t, g, part, comp, cache):
            u3, h3, zs = u3s[t % 3], h3s[t % 3], zss[t % 3]
            outs = tp_blocks[part]
            top = max(outs)
            dv = bc[6 * t + 4]
            hv = [h3[comp, d, g] for d in range(top + 1)]
            hv[0] = dep(hv[0] - dv if comp == 1 else hv[0] + dv)
            uv = [u3[comp, b, g] for b in range(top + 1)]
            s = {a: hv[0] * uv[a] for a in outs}
            for d in range(1, top + 1):
                for a in outs:
                    if a >= d:
                        s[a] = s[a] + hv[d] * uv[a - d]
            if comp == 0:
                cache["a1"] = s
            elif comp == 2:
                for a in outs:
                    cache["re", a] = cache["a1"][a] - s[a]
            else:
                for a in outs:
                    cache["im", a] = cache["a1"][a] + s[a]
                for a in sorted(set(outs) | {top + 1}):
                    if a == 0:
                        zr, zi = cache["re", 0], cache["im", 0]
                    elif ("im", a) in cache and ("im", a - 1) in cache:
                        zr = cache["re", a] - cache["im", a - 1]
                        zi = cache["im", a] + cache["re", a - 1]
                    else:
                        continue
                    zs[a, pl.ds(16 * g, 16), :] = jnp.concatenate([zr, zi], axis=0).astype(BF16)

        def IV(t, a):
            gmat = as_bf16(jnp.concatenate([gm[a % 2, 0], gm[a % 2, 1]], axis=1))
            y = jnp.dot(gmat, as_bf16(words(zss[t % 3], a)), preferred_element_type=F32)
            mark(y[:64])
            yy[t, rows(a), :] = y

        def run(fns):
            for fn in fns:
                fn()

        scope = (lambda n: jax.named_scope(n)) if scopes else (lambda n: contextlib.nullcontext())
        with scope("ep00a"):
            for nm in dma_order:
                for c in copies[nm]:
                    c.start()
            setup_masks()
            wait("tiny", "z")
            setup_rows()
            wait("Wq0")
            run([pt(WT, c) for c in range(2)])
            wait("Wq1", "q0", "q1")
            run([pt(WT, c) for c in range(2, 5)])
            run([pt(WP, 0, t) for t in range(NT)])
            run([pt(P, 0, n) for n in range(5)])
        with scope("ep00b"):
            wait("Wk")
            run([pt(WT, c) for c in range(5, 10)])
            run([pt(P, 1, n) for n in range(2)])
            run([pt(WP, 1, t) for t in range(NT)])
            run([pt(P, 0, n) for n in range(5, 10)])
        with scope("ep00c"):
            wait("Wv", "q2", "misc")
            setup_dft()
            run([pt(WT, c) for c in range(10, 15)])
            run([pt(P, 1, n) for n in range(2, 4)])
            run([pt(WP, 2, t) for t in range(NT)])
            run([pt(P, 0, n) for n in range(10, 15)])

        marks_per = {"P": 16, "O": 16, "GB": 16, "FU": 8, "FH": 8, "IV": 8, "TR": 8}
        out_copies = []
        done_o = set()
        sent = 0
        for e in range(1, nep + 1):
            with scope("ep%02d" % e):
                if e in waits:
                    wait(*waits[e])
                elif e in barriers:
                    barrier()
                pe = plan[e]
                streams = [
                    [(160, pt(P, i, n)) for i in pe["P"] for n in range(4 if i == 1 else 0, 3 * NT)],
                    [(160, pt(O, *x)) for x in pe["O"]],
                    [(64, pt(FH, *x)) for x in pe["FH"]],
                    [(64, pt(FU, *x)) for x in pe["FU"]],
                    [(64, pt(IV, *x)) for x in pe["IV"]],
                    [(32, pt(GB, i)) for i in pe["GB"]],
                    [(55, pt(TR, i, p)) for i in pe["TR"] for p in range(8)],
                    [(20, pt(TL, i, p, c)) for i in pe["TL"] for p in range(8) for c in range(2)],
                    [(60, pt(GA, i)) for i in pe["GA"]],
                    [(48 // kvsplit, pt(KV, *x, tuple(range(8 * s // kvsplit, 8 * (s + 1) // kvsplit))))
                     for x in pe["KV"] for s in range(kvsplit)],
                    [(30, pt(WO, i)) for i in pe["WO"]],
                ]
                tps = []
                for (t, g) in pe["TP"]:
                    cache = {}
                    for part, outs in enumerate(tp_blocks):
                        tps += [(sum(a + 1 for a in outs) // 2, pt(TP, t, g, part, c, cache)) for c in (0, 2, 1)]
                streams.append(tps)
                order = _interleave([s for s in streams if s])
                names = [fn.func.__name__ for fn in order]
                step = max(1, sum(marks_per.get(n, 0) for n in names) // max(1, sum(n in pace for n in names)))
                hard = (e in waits) or (e in barriers) or scopes
                state["marks"] = [] if hard else state["marks"][-keep:]
                seen = len(state["marks"])
                for fn, nm in zip(order, names):
                    marks = state["marks"]
                    if nm in pace and marks:
                        state["use"] = marks[min(len(marks) - 1, seen)]
                        seen = min(len(marks), seen + step)
                    else:
                        state["use"] = None
                    fn()
                state["use"] = None
                done_o.update(pe["O"])
                upto = sent
                while upto < NB and all((upto, n) in done_o for n in range(NT)):
                    upto += 1
                if upto > sent:
                    cp = pltpu.make_async_copy(outb.at[rows(sent, upto), :], out_hbm.at[0, rows(sent, upto), :],
                                               sem_o.at[len(out_copies)])
                    cp.start()
                    out_copies.append(cp)
                    sent = upto
        for cp in out_copies:
            cp.wait()

    comp_shape = (3, NB, NG + 1, 8, 128)
    scratch = [
        pltpu.VMEM((NT, S, 128), BF16),
        pltpu.VMEM((NT, S + 16, 128), BF16),
        pltpu.VMEM((NT, S, 128), BF16),
        pltpu.VMEM((D, S + 128), BF16),
        pltpu.VMEM((D, 3 * D), BF16),
        pltpu.VMEM((D, D), BF16),
        pltpu.VMEM((4, D), BF16),
        pltpu.VMEM((D,), BF16),
        pltpu.VMEM((D,), BF16),
        pltpu.VMEM((384, 128), U32),
        pltpu.VMEM((2, 128, 128), U32),
        pltpu.VMEM((2, 128, 128), U32),
        pltpu.VMEM((2, 2, 64, 128), U32),
        pltpu.VMEM((3, 64, 128), U32),
        pltpu.VMEM((6 * NT, 8, 128), F32),
        pltpu.VMEM((NT, 3 * D, 128), F32),
        pltpu.VMEM((NT, 3 * D, 128), BF16),
        pltpu.VMEM((NT, D, 128), F32),
        pltpu.VMEM((NT, D, 128), BF16),
        pltpu.VMEM((NT, S + 8, 128), F32),
        pltpu.VMEM((NT, S + PAD + 8, 128), F32),
        pltpu.VMEM((NT, S + PAD + 8, 128), F32),
        pltpu.VMEM((4, 8, 128, 128), BF16),
        pltpu.VMEM((NT, S, 128), BF16),
        pltpu.VMEM((NB, BLK, 128), BF16),
        pltpu.VMEM((S, 128), F32),
        pltpu.VMEM((NB, BLK, 128), BF16),
        pltpu.VMEM((NB, BLK, 128), BF16),
        pltpu.VMEM(comp_shape, F32),
        pltpu.VMEM(comp_shape, F32),
        pltpu.VMEM(comp_shape, F32),
        pltpu.VMEM(comp_shape, F32),
        pltpu.VMEM(comp_shape, F32),
        pltpu.VMEM(comp_shape, F32),
        pltpu.VMEM((NB, 2 * BLK, 128), BF16),
        pltpu.VMEM((NB, 2 * BLK, 128), BF16),
        pltpu.VMEM((NB, 2 * BLK, 128), BF16),
        pltpu.VMEM((NT, S, 128), F32),
        pltpu.VMEM((S, D), BF16),
        pltpu.SemaphoreType.DMA((64,)),
        pltpu.SemaphoreType.DMA((NB,)),
        pltpu.SemaphoreType.REGULAR,
        pltpu.SMEM((8,), jnp.int32),
    ]

    consts = _dft_constants()
    ramp = np.arange(8, dtype=np.int32)

    @jax.jit
    def run_kernel(A_q, A_k, A_v, A_shift_k, A_ssm_k, A_ssm_D, B_x, B_wqkv, B_wo, gate_w):
        return pl.pallas_call(
            kernel,
            out_shape=jax.ShapeDtypeStruct((1, S, D), BF16),
            in_specs=[pl.BlockSpec(memory_space=pl.ANY)] * 11,
            out_specs=pl.BlockSpec(memory_space=pl.ANY),
            scratch_shapes=scratch,
            compiler_params=pltpu.CompilerParams(vmem_limit_bytes=110 * 1024 * 1024),
        )(A_q, A_k, A_v, A_shift_k.T, A_ssm_k, A_ssm_D, B_wqkv, B_wo, gate_w, jnp.asarray(consts), jnp.asarray(ramp))

    return run_kernel


pallas_gated_mix__ssm_conv_h3__sliding_local_dilated__prompt_kernel = make_kernel()
```

```python
import contextlib
import functools
import math

import numpy as np
import jax
import jax.numpy as jnp
from jax import lax
from jax.experimental import pallas as pl
from jax.experimental.pallas import tpu as pltpu

S, D = 2048, 640
NT = D // 128
BLK = 128
NB = S // BLK
NG = 16
H, DH, WIN, DIL = 32, 20, 8, 2
PAD = 16
F32, BF16, U32 = jnp.float32, jnp.bfloat16, jnp.uint32
NT_DIMS = (((1,), (1,)), ((), ()))
ONE_LO, ONE_HI = 0x3F80, 0x3F800000
pt = functools.partial


def _pack_rows(m):
    b = np.asarray(m, dtype=np.float32).astype(BF16).view(np.uint16).astype(np.uint32)
    return b[0::2] | (b[1::2] << 16)


def _dft_constants():
    k = np.arange(BLK)
    n = np.arange(BLK)
    th = 2.0 * np.pi * (k[:, None] + 0.5) * n[None, :] / (2 * BLK)
    fwd = np.stack([np.cos(th).reshape(NG, 8, BLK), -np.sin(th).reshape(NG, 8, BLK)], axis=1).reshape(2 * BLK, BLK)
    order = np.arange(BLK).reshape(8, 8, 2).transpose(0, 2, 1).reshape(BLK)
    inv = np.stack([(np.cos(th).T / BLK).reshape(BLK, NG, 8), (-np.sin(th).T / BLK).reshape(BLK, NG, 8)], axis=2)
    pi = _pack_rows(inv.reshape(BLK, 2 * BLK))
    return np.concatenate([_pack_rows(fwd), _pack_rows(fwd[:, order]), pi[:, :BLK], pi[:, BLK:]], axis=0)


def _interleave(streams):
    items = []
    for si, s in enumerate(streams):
        tot = float(sum(w for w, _ in s))
        acc = 0.0
        for w, fn in s:
            items.append(((acc + 0.5 * w) / tot, si, fn))
            acc += w
    items.sort(key=lambda x: (x[0], x[1]))
    return [fn for _, _, fn in items]


MXU_COST = dict(P=2400, TR=256, GB=32, FU=64, FH=64, IV=64, O=160)
KEYS = ("P", "TL", "TR", "GA", "GB", "KV", "FU", "FH", "TP", "IV", "O", "WO")


def make_plan(tl_ep=(1, 2, 2, 3, 5, 7, 9, 11, 12, 13, 14, 14, 15, 15, 16, 16), tp0=4, a0=2, rate=8.0, wo_epoch=6,
              m_target=4600, a_ready=(2, 4, 4, 5, 7)):
    p_ep = [0, 1, 1] + list(range(2, 15))
    nep = max(tl_ep) + 2
    plan = {e: {k: [] for k in KEYS} for e in range(1, nep + 1)}
    for i in range(1, NB):
        plan[p_ep[i]]["P"].append(i)
    gb_ep = {}
    for i in range(NB):
        assert tl_ep[i] > p_ep[i], i
        plan[tl_ep[i]]["TL"].append(i)
        plan[tl_ep[i] + 1]["TR"].append(i)
        gb_ep[i] = max(3, tl_ep[i] + 1)
        plan[gb_ep[i]]["GB"].append(i)
        plan[gb_ep[i] - 1]["GA"].append(i)
    ep_tp = [tp0 + int(v / rate) for v in range(NT * NG)]
    for v, e in enumerate(ep_tp):
        plan[e]["TP"].append(divmod(v, NG))
    plan[a0]["KV"] = [(0, a) for a in range(NB)]
    plan[a0]["FH"] = [(0, a) for a in range(NB)]
    plan[tp0 - 1]["FU"] += [(0, a) for a in range(NB)]
    fu_done = {0: tp0 - 1}
    for t in range(1, NT):
        last = ep_tp[NG * t] - 1
        first = max(a0 + 2, ep_tp[NG * (t - 1)], a_ready[t] + 1)
        if t >= 3:
            first = max(first, ep_tp[NG * (t - 3) + NG - 1] + 1)
        if t >= 2:
            first = max(first, fu_done[t - 2] + 2)
        eps = list(range(first, last + 1))
        assert eps, (t, first, last)
        for a in range(NB):
            e = eps[a * len(eps) // NB]
            plan[e]["FU"].append((t, a))
            plan[e]["FH"].append((t, a))
            plan[e - 1]["KV"].append((t, a))
        fu_done[t] = last
    iv_ep = {}
    for t in range(NT):
        e0 = ep_tp[NG * t + NG - 1] + 1
        for a in range(NB):
            iv_ep[(t, a)] = e0 + (a >= NB // 2 and t < NT - 1)
            plan[iv_ep[(t, a)]]["IV"].append((t, a))
        if t >= 3:
            assert max(iv_ep[(t - 3, a)] for a in range(NB)) < ep_tp[NG * t]
    plan[wo_epoch]["WO"] = list(range(NT))

    def mxu(e):
        return sum(MXU_COST.get(k, 0) * len(v) for k, v in plan[e].items())
    todo = [(i, n) for n in range(NT) for i in range(NB)]
    for e in range(wo_epoch + 1, nep + 1):
        avail = [x for x in todo if iv_ep[(x[1], x[0])] < e and tl_ep[x[0]] + 1 < e and gb_ep[x[0]] < e]
        avail.sort()
        for x in avail:
            if e < nep and mxu(e) + MXU_COST["O"] > m_target:
                break
            plan[e]["O"].append(x)
            todo.remove(x)
    assert not todo, todo
    return plan


Q_GROUPS = {"q0": (0, 1), "q1": (1, 2), "q2": (2, 3), "q3": (3, 4), "q45": (4, 6), "q67": (6, 8), "q8f": (8, 16)}
DMA_ORDER = ("tiny", "z", "Wq0", "Wq1", "q0", "q1", "Wk", "Wv", "q2", "misc", "q3", "A0", "q45", "A1", "q67", "A2", "Wo", "A3",
             "q8f", "A4")
WAITS = {2: ("q3", "A0", "q45"), 4: ("A1", "q67", "A2"), 6: ("Wo", "A3", "q8f"), 8: ("A4",)}


def make_kernel(plan_kw=None, scopes=False, barriers=(10, 12, 15), waits=WAITS, dma_order=DMA_ORDER,
                tp_blocks=((15, 14, 13, 12), (11, 10, 9, 8), (7, 6, 5, 4, 3, 2, 1, 0)),
                pace=("TL", "KV", "TP", "GA"), keep=16, kvsplit=2):
    plan = make_plan(**(plan_kw or {}))
    nep = max(plan)
    waited = {nm: e for e, names in waits.items() for nm in names}
    for e, pe in plan.items():
        for i in pe["P"] + pe["GA"] + [x[0] for x in pe["O"]]:
            for nm, (i0, i1) in Q_GROUPS.items():
                assert not (i0 <= i < i1) or waited.get(nm, 0) <= e, (nm, e)
        for t, _ in pe["KV"] + pe["FH"]:
            assert waited["A%d" % t] <= e, (t, e)
        assert not pe["WO"] or waited["Wo"] <= e

    def kernel(q_hbm, k_hbm, v_hbm, sk_hbm, h_hbm, dd_hbm, wqkv_hbm, wo_hbm, gw_hbm, c_hbm, z_hbm, out_hbm,
               qb, kb, vb, hb, wqb, wob, skb, ddb, gwb, cb,
               fm, fp, gm, em, bc,
               wt, wtp, wof, wop,
               qs, ks, vs, lgs, ob, gps, gs,
               kva, kvb, u3a, u3b, u3c, h3a, h3b, h3c, zsa, zsb, zsc, yy, outb,
               sem_in, sem_o, sem_b, zsm):
        kvs, u3s, h3s, zss = (kva, kvb), (u3a, u3b, u3c), (h3a, h3b, h3c), (zsa, zsb, zsc)

        def rows(i0, i1=None):
            i1 = i0 + 1 if i1 is None else i1
            return pl.ds(i0 * BLK, (i1 - i0) * BLK)

        copies = {}
        nsem = [0]

        def add_copy(name, src, dst):
            copies.setdefault(name, []).append(pltpu.make_async_copy(src, dst, sem_in.at[nsem[0]]))
            nsem[0] += 1

        add_copy("Wq0", wqkv_hbm.at[:, pl.ds(0, 256)], wqb.at[:, pl.ds(0, 256)])
        add_copy("Wq1", wqkv_hbm.at[:, pl.ds(256, 384)], wqb.at[:, pl.ds(256, 384)])
        for part, nm in ((1, "Wk"), (2, "Wv")):
            add_copy(nm, wqkv_hbm.at[:, pl.ds(part * D, D)], wqb.at[:, pl.ds(part * D, D)])
        add_copy("z", z_hbm, zsm)
        add_copy("misc", c_hbm, cb)
        add_copy("tiny", sk_hbm, skb)
        add_copy("tiny", dd_hbm, ddb)
        add_copy("tiny", gw_hbm, gwb)
        add_copy("Wo", wo_hbm, wob)
        for nm, (i0, i1) in Q_GROUPS.items():
            for t in range(NT):
                add_copy(nm, q_hbm.at[0, rows(i0, i1), pl.ds(t * 128, 128)], qb.at[t, rows(i0, i1), :])
        for t in range(NT):
            add_copy("A%d" % t, h_hbm.at[pl.ds(t * 128, 128), :], hb.at[pl.ds(t * 128, 128), pl.ds(0, S)])
            add_copy("A%d" % t, k_hbm.at[0, :, pl.ds(t * 128, 128)], kb.at[t, pl.ds(16, S), :])
            add_copy("A%d" % t, v_hbm.at[0, :, pl.ds(t * 128, 128)], vb.at[t])

        def wait(*names):
            for nm in names:
                for c in copies[nm]:
                    c.wait()

        def barrier():
            pl.semaphore_signal(sem_b, 1)
            pl.semaphore_wait(sem_b, 1)

        state = {"marks": [], "use": None}

        def dep(x):
            if state["use"] is None:
                return x
            never = lax.broadcasted_iota(jnp.int32, (8, 128), 0) < zsm[0]
            return jnp.where(never, state["use"], x)

        def mark(res):
            state["marks"] += [res[8 * j:8 * j + 8] for j in range(res.shape[0] // 8)]

        def rep(v, n):
            return jnp.concatenate([v] * n, axis=0)

        def words(ref, *idx):
            return ref.bitcast(U32)[idx]

        def as_bf16(w):
            return pltpu.bitcast(w, BF16)

        def as_f32(w):
            return pltpu.bitcast(w, F32)

        def wide(ref, r0, n):
            return as_bf16(jnp.concatenate([words(ref, t, pl.ds(r0, n)) for t in range(NT)], axis=1))

        emat = lambda j: as_bf16(em[j])
        cexp = (DH ** -0.5) * math.log2(math.e)

        def setup_masks():
            r = lax.broadcasted_iota(jnp.int32, (64, 128), 0)
            l = lax.broadcasted_iota(jnp.int32, (64, 128), 1)
            lo, hi, zero = jnp.uint32(ONE_LO), jnp.uint32(ONE_HI), jnp.uint32(0)
            em[0] = jnp.where(l == 2 * r, lo, zero) | jnp.where(l == 2 * r + 1, hi, zero)
            em[1] = jnp.where((l & 31) == ((2 * r) & 31), lo, zero) | jnp.where((l & 31) == ((2 * r + 1) & 31), hi, zero)
            em[2] = jnp.full((64, 128), ONE_LO | ONE_HI, U32)
            for t in range(NT):
                ks[t, pl.ds(0, PAD), :] = jnp.zeros((PAD, 128), F32)
                vs[t, pl.ds(0, PAD), :] = jnp.zeros((PAD, 128), F32)
                kb[t, pl.ds(0, 16), :] = jnp.zeros((16, 128), BF16)

        def setup_dft():
            for ref, r0 in ((fm, 0), (fp, 128)):
                f = cb[pl.ds(r0, 128), :]
                ref[0] = f
                ref[1] = f ^ jnp.uint32(0x80000000)
            l = lax.broadcasted_iota(jnp.int32, (64, 128), 1)
            flip = jnp.where((l & 1) != 0, jnp.uint32(0x80008000), jnp.uint32(0))
            for hf in range(2):
                g = cb[pl.ds(256 + 64 * hf, 64), :]
                gm[0, hf] = g
                gm[1, hf] = g ^ flip

        def setup_rows():
            skf = skb[...].astype(F32)
            ddf = ddb[...].astype(F32).reshape(1, D)
            gwf = gwb[...].astype(F32).reshape(1, D)
            for t in range(NT):
                sl = slice(t * 128, (t + 1) * 128)
                for j in range(4):
                    bc[6 * t + j] = jnp.broadcast_to(skf[j:j + 1, sl], (8, 128))
                bc[6 * t + 4] = jnp.broadcast_to(ddf[:, sl], (8, 128))
                bc[6 * t + 5] = jnp.broadcast_to(gwf[:, sl], (8, 128))

        def WT(c):
            for i in range(NT):
                tile = wqb[pl.ds(i * 128, 128), pl.ds(c * 128, 128)]
                wt[i, pl.ds(c * 128, 128), :] = lax.dot_general(emat(0), tile, NT_DIMS, preferred_element_type=F32)

        def head_major(src, i, base):
            return jnp.concatenate([src[i, pl.ds(base, 8, stride=DH), :], src[i, pl.ds(base + 8 * DH, 8, stride=DH), :]], axis=0)

        def WP(part, t):
            for j in range(4 * t, 4 * t + 4):
                for i in range(NT):
                    for m in range(2):
                        w = head_major(wt, i, part * D + j + 16 * DH * m)
                        if part == 0:
                            w = w * cexp
                        wtp[i, pl.ds((part * DH + j) * 32 + 16 * m, 16), :] = w.astype(BF16)

        def WO(n):
            wof[n] = wob[:, n * 128:(n + 1) * 128].astype(F32)
            for j in range(DH):
                for m in range(2):
                    wop[n, pl.ds(j * 32 + 16 * m, 16), :] = head_major(wof, n, j + 16 * DH * m).astype(BF16)

        def P(i, n):
            res = lax.dot_general(wide(qb, i * 64, 64), wide(wtp, n * 64, 64), NT_DIMS, preferred_element_type=F32)
            mark(res)
            part, t = divmod(n, NT)
            if part == 0:
                qs[t, rows(i), :] = res
            elif part == 1:
                ks[t, pl.ds(PAD + i * BLK, BLK), :] = res
            else:
                vs[t, pl.ds(PAD + i * BLK, BLK), :] = res

        def TL(i, p, c):
            r = i * BLK + 16 * p + 8 * c
            qv = [qs[t, pl.ds(r, 8), :] for t in range(NT)]
            qv[0] = dep(qv[0])
            ls = []
            for w in range(WIN):
                l = qv[0] * ks[0, pl.ds(PAD + r - DIL * w, 8), :]
                for t in range(1, NT):
                    l = l + qv[t] * ks[t, pl.ds(PAD + r - DIL * w, 8), :]
                ls.append(l)
            lgs[i % 4, p, pl.ds(64 * c, 64), :] = jnp.concatenate(ls, axis=0).astype(BF16)

        def TR(i, p):
            b0 = i * BLK + 16 * p
            red = jnp.dot(as_bf16(words(lgs, i % 4, p)), emat(1), preferred_element_type=F32)
            mark(red[:64])
            outs = []
            for c in range(2):
                r = b0 + 8 * c
                lw = [red[(c * WIN + w) * 8:(c * WIN + w + 1) * 8] for w in range(WIN)]
                if r < DIL * (WIN - 1):
                    pos = r + lax.broadcasted_iota(jnp.int32, (8, 128), 0)
                    lw = [jnp.where(pos >= DIL * w, lw[w], -1e30) for w in range(WIN)]
                m = lw[0]
                for w in range(1, WIN):
                    m = jnp.maximum(m, lw[w])
                e = [jnp.exp2(lw[w] - m) for w in range(WIN)]
                den = e[0]
                for w in range(1, WIN):
                    den = den + e[w]
                rinv = pl.reciprocal(den, approx=True)
                oc = [e[0] * vs[t, pl.ds(PAD + r, 8), :] for t in range(NT)]
                for w in range(1, WIN):
                    oc = [oc[t] + e[w] * vs[t, pl.ds(PAD + r - DIL * w, 8), :] for t in range(NT)]
                outs.append([oc[t] * rinv for t in range(NT)])
            for t in range(NT):
                ob[t, pl.ds(b0, 16), :] = jnp.concatenate([outs[0][t], outs[1][t]], axis=0).astype(BF16)

        def GA(i):
            zp = None
            for t in range(NT):
                g8 = dep(bc[6 * t + 5]) if t == 0 else bc[6 * t + 5]
                term = qb[t, rows(i), :].astype(F32) * rep(g8, 16)
                zp = term if zp is None else zp + term
            gps[i] = zp.astype(BF16)

        def GB(i):
            z = jnp.dot(as_bf16(words(gps, i)), emat(2), preferred_element_type=F32)
            mark(z)
            gs[rows(i), :] = 0.5 + 0.5 * jnp.tanh(0.5 * z)

        def O(i, n):
            bo = jnp.dot(wide(ob, i * 64, 64), as_bf16(words(wop, n)), preferred_element_type=F32)
            mark(bo)
            a_br = qb[n, rows(i), :].astype(F32) * yy[n, rows(i), :]
            outb[rows(i), n * 128:(n + 1) * 128] = (bo + gs[rows(i), :] * (a_br - bo)).astype(BF16)

        def KV(t, a, ms):
            lo = lambda x: as_f32(x << 16)
            hi = lambda x: as_f32(x & jnp.uint32(0xFFFF0000))
            c = [dep(bc[6 * t])] + [bc[6 * t + j] for j in range(1, 4)]
            for m in ms:
                base = 8 + 64 * a + 8 * m
                p0, p1, p2 = (words(kb, t, pl.ds(base - j, 8)) for j in range(3))
                l0, h0, l1, h1, h2 = lo(p0), hi(p0), lo(p1), hi(p1), hi(p2)
                ev = c[0] * l0 + c[1] * h1 + c[2] * l1 + c[3] * h2
                od = c[0] * h0 + c[1] * l0 + c[2] * h1 + c[3] * l1
                vv = words(vb, t, pl.ds(64 * a + 8 * m, 8))
                kvs[t % 2][a, pl.ds(16 * m, 16), :] = jnp.concatenate([ev * lo(vv), od * hi(vv)], axis=0).astype(BF16)

        def FU(t, a):
            u3 = u3s[t % 3]
            uu = jnp.dot(as_bf16(fp[a % 2]), as_bf16(words(kvs[t % 2], a)), preferred_element_type=F32)
            mark(uu[:64])
            uu = uu.reshape(NG, 2, 8, 128)
            ar, ai = uu[:, 0], uu[:, 1]
            u3[0, a, pl.ds(0, NG)] = ar + ai
            u3[1, a, pl.ds(0, NG)] = ar
            u3[2, a, pl.ds(0, NG)] = ai

        def FH(t, a):
            h3 = h3s[t % 3]
            hblk = hb[pl.ds(t * 128, 128), pl.ds(a * BLK, BLK)]
            hh = lax.dot_general(as_bf16(fm[a % 2]), hblk, NT_DIMS, preferred_element_type=F32)
            mark(hh[:64])
            hh = hh.reshape(NG, 2, 8, 128)
            br, bi = hh[:, 0], hh[:, 1]
            h3[0, a, pl.ds(0, NG)] = br
            h3[1, a, pl.ds(0, NG)] = bi - br
            h3[2, a, pl.ds(0, NG)] = br + bi

        def TP(t, g, part, comp, cache):
            u3, h3, zs = u3s[t % 3], h3s[t % 3], zss[t % 3]
            outs = tp_blocks[part]
            top = max(outs)
            dv = bc[6 * t + 4]
            hv = [h3[comp, d, g] for d in range(top + 1)]
            hv[0] = dep(hv[0] - dv if comp == 1 else hv[0] + dv)
            uv = [u3[comp, b, g] for b in range(top + 1)]
            s = {a: hv[0] * uv[a] for a in outs}
            for d in range(1, top + 1):
                for a in outs:
                    if a >= d:
                        s[a] = s[a] + hv[d] * uv[a - d]
            if comp == 0:
                cache["a1"] = s
            elif comp == 2:
                for a in outs:
                    cache["re", a] = cache["a1"][a] - s[a]
            else:
                for a in outs:
                    cache["im", a] = cache["a1"][a] + s[a]
                for a in sorted(set(outs) | {top + 1}):
                    if a == 0:
                        zr, zi = cache["re", 0], cache["im", 0]
                    elif ("im", a) in cache and ("im", a - 1) in cache:
                        zr = cache["re", a] - cache["im", a - 1]
                        zi = cache["im", a] + cache["re", a - 1]
                    else:
                        continue
                    zs[a, pl.ds(16 * g, 16), :] = jnp.concatenate([zr, zi], axis=0).astype(BF16)

        def IV(t, a):
            gmat = as_bf16(jnp.concatenate([gm[a % 2, 0], gm[a % 2, 1]], axis=1))
            y = jnp.dot(gmat, as_bf16(words(zss[t % 3], a)), preferred_element_type=F32)
            mark(y[:64])
            yy[t, rows(a), :] = y

        def run(fns):
            for fn in fns:
                fn()

        scope = (lambda n: jax.named_scope(n)) if scopes else (lambda n: contextlib.nullcontext())
        with scope("ep00a"):
            for nm in dma_order:
                for c in copies[nm]:
                    c.start()
            setup_masks()
            wait("tiny", "z")
            setup_rows()
            wait("Wq0")
            run([pt(WT, c) for c in range(2)])
            wait("Wq1", "q0", "q1")
            run([pt(WT, c) for c in range(2, 5)])
            run([pt(WP, 0, t) for t in range(NT)])
            run([pt(P, 0, n) for n in range(5)])
        with scope("ep00b"):
            wait("Wk")
            run([pt(WT, c) for c in range(5, 10)])
            run([pt(P, 1, n) for n in range(2)])
            run([pt(WP, 1, t) for t in range(NT)])
            run([pt(P, 0, n) for n in range(5, 10)])
        with scope("ep00c"):
            wait("Wv", "q2", "misc")
            setup_dft()
            run([pt(WT, c) for c in range(10, 15)])
            run([pt(P, 1, n) for n in range(2, 4)])
            run([pt(WP, 2, t) for t in range(NT)])
            run([pt(P, 0, n) for n in range(10, 15)])

        marks_per = {"P": 16, "O": 16, "GB": 16, "FU": 8, "FH": 8, "IV": 8, "TR": 8}
        out_copies = []
        done_o = set()
        sent = 0
        for e in range(1, nep + 1):
            with scope("ep%02d" % e):
                if e in waits:
                    wait(*waits[e])
                elif e in barriers:
                    barrier()
                pe = plan[e]
                streams = [
                    [(160, pt(P, i, n)) for i in pe["P"] for n in range(4 if i == 1 else 0, 3 * NT)],
                    [(160, pt(O, *x)) for x in pe["O"]],
                    [(64, pt(FH, *x)) for x in pe["FH"]],
                    [(64, pt(FU, *x)) for x in pe["FU"]],
                    [(64, pt(IV, *x)) for x in pe["IV"]],
                    [(32, pt(GB, i)) for i in pe["GB"]],
                    [(55, pt(TR, i, p)) for i in pe["TR"] for p in range(8)],
                    [(20, pt(TL, i, p, c)) for i in pe["TL"] for p in range(8) for c in range(2)],
                    [(60, pt(GA, i)) for i in pe["GA"]],
                    [(48 // kvsplit, pt(KV, *x, tuple(range(8 * s // kvsplit, 8 * (s + 1) // kvsplit))))
                     for x in pe["KV"] for s in range(kvsplit)],
                    [(30, pt(WO, i)) for i in pe["WO"]],
                ]
                tps = []
                for (t, g) in pe["TP"]:
                    cache = {}
                    for part, outs in enumerate(tp_blocks):
                        tps += [(sum(a + 1 for a in outs) // 2, pt(TP, t, g, part, c, cache)) for c in (0, 2, 1)]
                streams.append(tps)
                order = _interleave([s for s in streams if s])
                names = [fn.func.__name__ for fn in order]
                step = max(1, sum(marks_per.get(n, 0) for n in names) // max(1, sum(n in pace for n in names)))
                hard = (e in waits) or (e in barriers) or scopes
                state["marks"] = [] if hard else state["marks"][-keep:]
                seen = len(state["marks"])
                for fn, nm in zip(order, names):
                    marks = state["marks"]
                    if nm in pace and marks:
                        state["use"] = marks[min(len(marks) - 1, seen)]
                        seen = min(len(marks), seen + step)
                    else:
                        state["use"] = None
                    fn()
                state["use"] = None
                done_o.update(pe["O"])
                upto = sent
                while upto < NB and all((upto, n) in done_o for n in range(NT)):
                    upto += 1
                if upto > sent:
                    cp = pltpu.make_async_copy(outb.at[rows(sent, upto), :], out_hbm.at[0, rows(sent, upto), :],
                                               sem_o.at[len(out_copies)])
                    cp.start()
                    out_copies.append(cp)
                    sent = upto
        for cp in out_copies:
            cp.wait()

    comp_shape = (3, NB, NG + 1, 8, 128)
    scratch = [
        pltpu.VMEM((NT, S, 128), BF16),
        pltpu.VMEM((NT, S + 16, 128), BF16),
        pltpu.VMEM((NT, S, 128), BF16),
        pltpu.VMEM((D, S + 128), BF16),
        pltpu.VMEM((D, 3 * D), BF16),
        pltpu.VMEM((D, D), BF16),
        pltpu.VMEM((4, D), BF16),
        pltpu.VMEM((D,), BF16),
        pltpu.VMEM((D,), BF16),
        pltpu.VMEM((384, 128), U32),
        pltpu.VMEM((2, 128, 128), U32),
        pltpu.VMEM((2, 128, 128), U32),
        pltpu.VMEM((2, 2, 64, 128), U32),
        pltpu.VMEM((3, 64, 128), U32),
        pltpu.VMEM((6 * NT, 8, 128), F32),
        pltpu.VMEM((NT, 3 * D, 128), F32),
        pltpu.VMEM((NT, 3 * D, 128), BF16),
        pltpu.VMEM((NT, D, 128), F32),
        pltpu.VMEM((NT, D, 128), BF16),
        pltpu.VMEM((NT, S + 8, 128), F32),
        pltpu.VMEM((NT, S + PAD + 8, 128), F32),
        pltpu.VMEM((NT, S + PAD + 8, 128), F32),
        pltpu.VMEM((4, 8, 128, 128), BF16),
        pltpu.VMEM((NT, S, 128), BF16),
        pltpu.VMEM((NB, BLK, 128), BF16),
        pltpu.VMEM((S, 128), F32),
        pltpu.VMEM((NB, BLK, 128), BF16),
        pltpu.VMEM((NB, BLK, 128), BF16),
        pltpu.VMEM(comp_shape, F32),
        pltpu.VMEM(comp_shape, F32),
        pltpu.VMEM(comp_shape, F32),
        pltpu.VMEM(comp_shape, F32),
        pltpu.VMEM(comp_shape, F32),
        pltpu.VMEM(comp_shape, F32),
        pltpu.VMEM((NB, 2 * BLK, 128), BF16),
        pltpu.VMEM((NB, 2 * BLK, 128), BF16),
        pltpu.VMEM((NB, 2 * BLK, 128), BF16),
        pltpu.VMEM((NT, S, 128), F32),
        pltpu.VMEM((S, D), BF16),
        pltpu.SemaphoreType.DMA((64,)),
        pltpu.SemaphoreType.DMA((NB,)),
        pltpu.SemaphoreType.REGULAR,
        pltpu.SMEM((8,), jnp.int32),
    ]

    consts = _dft_constants()
    ramp = np.arange(8, dtype=np.int32)

    @jax.jit
    def run_kernel(A_q, A_k, A_v, A_shift_k, A_ssm_k, A_ssm_D, B_x, B_wqkv, B_wo, gate_w):
        return pl.pallas_call(
            kernel,
            out_shape=jax.ShapeDtypeStruct((1, S, D), BF16),
            in_specs=[pl.BlockSpec(memory_space=pl.ANY)] * 11,
            out_specs=pl.BlockSpec(memory_space=pl.ANY),
            scratch_shapes=scratch,
            compiler_params=pltpu.CompilerParams(vmem_limit_bytes=110 * 1024 * 1024),
        )(A_q, A_k, A_v, A_shift_k.T, A_ssm_k, A_ssm_D, B_wqkv, B_wo, gate_w, jnp.asarray(consts), jnp.asarray(ramp))

    return run_kernel


pallas_gated_mix__ssm_conv_h3__sliding_local_dilated__prompt_kernel = make_kernel()
```

```python
import contextlib
import functools
import math

import numpy as np
import jax
import jax.numpy as jnp
from jax import lax
from jax.experimental import pallas as pl
from jax.experimental.pallas import tpu as pltpu

S, D = 2048, 640
NT = D // 128
BLK = 128
NB = S // BLK
NG = 16
H, DH, WIN, DIL = 32, 20, 8, 2
PAD = 16
F32, BF16, U32 = jnp.float32, jnp.bfloat16, jnp.uint32
NT_DIMS = (((1,), (1,)), ((), ()))
ONE_LO, ONE_HI = 0x3F80, 0x3F800000
pt = functools.partial


def _pack_rows(m):
    b = np.asarray(m, dtype=np.float32).astype(BF16).view(np.uint16).astype(np.uint32)
    return b[0::2] | (b[1::2] << 16)


def _dft_constants():
    k = np.arange(BLK)
    n = np.arange(BLK)
    th = 2.0 * np.pi * (k[:, None] + 0.5) * n[None, :] / (2 * BLK)
    fwd = np.stack([np.cos(th).reshape(NG, 8, BLK), -np.sin(th).reshape(NG, 8, BLK)], axis=1).reshape(2 * BLK, BLK)
    order = np.arange(BLK).reshape(8, 8, 2).transpose(0, 2, 1).reshape(BLK)
    inv = np.stack([(np.cos(th).T / BLK).reshape(BLK, NG, 8), (-np.sin(th).T / BLK).reshape(BLK, NG, 8)], axis=2)
    pi = _pack_rows(inv.reshape(BLK, 2 * BLK))
    return np.concatenate([_pack_rows(fwd), _pack_rows(fwd[:, order]), pi[:, :BLK], pi[:, BLK:]], axis=0)


def _interleave(streams):
    items = []
    for si, s in enumerate(streams):
        tot = float(sum(w for w, _ in s))
        acc = 0.0
        for w, fn in s:
            items.append(((acc + 0.5 * w) / tot, si, fn))
            acc += w
    items.sort(key=lambda x: (x[0], x[1]))
    return [fn for _, _, fn in items]


MXU_COST = dict(P=2400, TR=256, GB=32, FU=64, FH=64, IV=64, O=160)
KEYS = ("P", "TL", "TR", "GA", "GB", "KV", "FU", "FH", "TP", "IV", "O", "WO")


def make_plan(tl_ep=(1, 2, 2, 3, 6, 8, 10, 12, 12, 13, 13, 14, 14, 15, 15, 16), tp0=4, a0=2, rate=8.0, wo_epoch=6,
              m_target=4600, a_ready=(2, 4, 4, 5, 7), f_span=1, p_ep=None):
    p_ep = p_ep or [0, 1, 1] + list(range(2, 15))
    nep = max(tl_ep) + 2
    plan = {e: {k: [] for k in KEYS} for e in range(1, nep + 1)}
    for i in range(1, NB):
        plan[p_ep[i]]["P"].append(i)
    gb_ep = {}
    for i in range(NB):
        assert tl_ep[i] > p_ep[i], i
        assert i < 4 or tl_ep[i - 4] + 1 < tl_ep[i], i
        plan[tl_ep[i]]["TL"].append(i)
        plan[tl_ep[i] + 1]["TR"].append(i)
        gb_ep[i] = max(3, tl_ep[i] + 1)
        plan[gb_ep[i]]["GB"].append(i)
        plan[gb_ep[i] - 1]["GA"].append(i)
    ep_tp = [tp0 + int(v / rate) for v in range(NT * NG)]
    for v, e in enumerate(ep_tp):
        plan[e]["TP"].append(divmod(v, NG))
    plan[a0]["KV"] = [(0, a) for a in range(NB)]
    plan[a0]["FH"] = [(0, a) for a in range(NB)]
    plan[tp0 - 1]["FU"] += [(0, a) for a in range(NB)]
    fu_done = {0: tp0 - 1}
    for t in range(1, NT):
        last = ep_tp[NG * t] - 1
        first = max(a0 + 2, ep_tp[NG * (t - 1)], a_ready[t] + 1)
        if t >= 3:
            first = max(first, ep_tp[NG * (t - 3) + NG - 1] + 1)
        if t >= 2:
            first = max(first, fu_done[t - 2] + 2)
        eps = list(range(first, last + 1))[-f_span:]
        assert eps, (t, first, last)
        for a in range(NB):
            e = eps[a * len(eps) // NB]
            plan[e]["FU"].append((t, a))
            plan[e]["FH"].append((t, a))
            plan[e - 1]["KV"].append((t, a))
        fu_done[t] = last
    iv_ep = {}
    for t in range(NT):
        e0 = ep_tp[NG * t + NG - 1] + 1
        for a in range(NB):
            iv_ep[(t, a)] = e0 + (a >= NB // 2 and t < NT - 1)
            plan[iv_ep[(t, a)]]["IV"].append((t, a))
        if t >= 3:
            assert max(iv_ep[(t - 3, a)] for a in range(NB)) < ep_tp[NG * t]
    plan[wo_epoch]["WO"] = list(range(NT))

    def mxu(e):
        return sum(MXU_COST.get(k, 0) * len(v) for k, v in plan[e].items())
    todo = [(i, n) for n in range(NT) for i in range(NB)]
    for e in range(wo_epoch + 1, nep + 1):
        avail = [x for x in todo if iv_ep[(x[1], x[0])] < e and tl_ep[x[0]] + 1 < e and gb_ep[x[0]] < e]
        avail.sort()
        for x in avail:
            if e < nep and mxu(e) + MXU_COST["O"] > m_target:
                break
            plan[e]["O"].append(x)
            todo.remove(x)
    assert not todo, todo
    return plan


Q_GROUPS = {"q0": (0, 1), "q1": (1, 2), "q2": (2, 3), "q3": (3, 4), "q45": (4, 6), "q67": (6, 8), "q8f": (8, 16)}
DMA_ORDER = ("tiny", "z", "Wq0", "Wq1", "q0", "q1", "Wk", "Wv", "q2", "misc", "q3", "A0", "q45", "A1", "q67", "A2", "Wo", "A3",
             "q8f", "A4")
WAITS = {2: ("q3", "A0", "q45"), 4: ("A1", "q67", "A2"), 6: ("Wo", "A3", "q8f"), 8: ("A4",)}


def make_kernel(plan_kw=None, scopes=False, barriers=(10, 12, 15), waits=WAITS, dma_order=DMA_ORDER,
                tp_blocks=((15, 14, 13, 12), (11, 10, 9, 8), (7, 6, 5, 4, 3, 2, 1, 0)),
                pace=("TL", "KV", "TP", "GA"), keep=16, kvsplit=2):
    plan = make_plan(**(plan_kw or {}))
    nep = max(plan)
    waited = {nm: e for e, names in waits.items() for nm in names}
    for e, pe in plan.items():
        for i in pe["P"] + pe["GA"] + [x[0] for x in pe["O"]]:
            for nm, (i0, i1) in Q_GROUPS.items():
                assert not (i0 <= i < i1) or waited.get(nm, 0) <= e, (nm, e)
        for t, _ in pe["KV"] + pe["FH"]:
            assert waited["A%d" % t] <= e, (t, e)
        assert not pe["WO"] or waited["Wo"] <= e

    def kernel(q_hbm, k_hbm, v_hbm, sk_hbm, h_hbm, dd_hbm, wqkv_hbm, wo_hbm, gw_hbm, c_hbm, z_hbm, out_hbm,
               qb, kb, vb, hb, wqb, wob, skb, ddb, gwb, cb,
               fm, fp, gm, em, bc,
               wt, wtp, wof, wop,
               qs, ks, vs, lgs, ob, gps, gs,
               kva, kvb, u3a, u3b, u3c, h3a, h3b, h3c, zsa, zsb, zsc, yy, outb,
               sem_in, sem_o, sem_b, zsm):
        kvs, u3s, h3s, zss = (kva, kvb), (u3a, u3b, u3c), (h3a, h3b, h3c), (zsa, zsb, zsc)

        def rows(i0, i1=None):
            i1 = i0 + 1 if i1 is None else i1
            return pl.ds(i0 * BLK, (i1 - i0) * BLK)

        copies = {}
        nsem = [0]

        def add_copy(name, src, dst):
            copies.setdefault(name, []).append(pltpu.make_async_copy(src, dst, sem_in.at[nsem[0]]))
            nsem[0] += 1

        add_copy("Wq0", wqkv_hbm.at[:, pl.ds(0, 256)], wqb.at[:, pl.ds(0, 256)])
        add_copy("Wq1", wqkv_hbm.at[:, pl.ds(256, 384)], wqb.at[:, pl.ds(256, 384)])
        for part, nm in ((1, "Wk"), (2, "Wv")):
            add_copy(nm, wqkv_hbm.at[:, pl.ds(part * D, D)], wqb.at[:, pl.ds(part * D, D)])
        add_copy("z", z_hbm, zsm)
        add_copy("misc", c_hbm, cb)
        add_copy("tiny", sk_hbm, skb)
        add_copy("tiny", dd_hbm, ddb)
        add_copy("tiny", gw_hbm, gwb)
        add_copy("Wo", wo_hbm, wob)
        for nm, (i0, i1) in Q_GROUPS.items():
            for t in range(NT):
                add_copy(nm, q_hbm.at[0, rows(i0, i1), pl.ds(t * 128, 128)], qb.at[t, rows(i0, i1), :])
        for t in range(NT):
            add_copy("A%d" % t, h_hbm.at[pl.ds(t * 128, 128), :], hb.at[pl.ds(t * 128, 128), pl.ds(0, S)])
            add_copy("A%d" % t, k_hbm.at[0, :, pl.ds(t * 128, 128)], kb.at[t, pl.ds(16, S), :])
            add_copy("A%d" % t, v_hbm.at[0, :, pl.ds(t * 128, 128)], vb.at[t])

        def wait(*names):
            for nm in names:
                for c in copies[nm]:
                    c.wait()

        def barrier():
            pl.semaphore_signal(sem_b, 1)
            pl.semaphore_wait(sem_b, 1)

        state = {"marks": [], "use": None}

        def dep(x):
            if state["use"] is None:
                return x
            never = lax.broadcasted_iota(jnp.int32, (8, 128), 0) < zsm[0]
            return jnp.where(never, state["use"], x)

        def mark(res):
            state["marks"] += [res[8 * j:8 * j + 8] for j in range(res.shape[0] // 8)]

        def rep(v, n):
            return jnp.concatenate([v] * n, axis=0)

        def words(ref, *idx):
            return ref.bitcast(U32)[idx]

        def as_bf16(w):
            return pltpu.bitcast(w, BF16)

        def as_f32(w):
            return pltpu.bitcast(w, F32)

        def wide(ref, r0, n):
            return as_bf16(jnp.concatenate([words(ref, t, pl.ds(r0, n)) for t in range(NT)], axis=1))

        emat = lambda j: as_bf16(em[j])
        cexp = (DH ** -0.5) * math.log2(math.e)

        def setup_masks():
            r = lax.broadcasted_iota(jnp.int32, (64, 128), 0)
            l = lax.broadcasted_iota(jnp.int32, (64, 128), 1)
            lo, hi, zero = jnp.uint32(ONE_LO), jnp.uint32(ONE_HI), jnp.uint32(0)
            em[0] = jnp.where(l == 2 * r, lo, zero) | jnp.where(l == 2 * r + 1, hi, zero)
            em[1] = jnp.where((l & 31) == ((2 * r) & 31), lo, zero) | jnp.where((l & 31) == ((2 * r + 1) & 31), hi, zero)
            em[2] = jnp.full((64, 128), ONE_LO | ONE_HI, U32)
            for t in range(NT):
                ks[t, pl.ds(0, PAD), :] = jnp.zeros((PAD, 128), F32)
                vs[t, pl.ds(0, PAD), :] = jnp.zeros((PAD, 128), F32)
                kb[t, pl.ds(0, 16), :] = jnp.zeros((16, 128), BF16)

        def setup_dft():
            for ref, r0 in ((fm, 0), (fp, 128)):
                f = cb[pl.ds(r0, 128), :]
                ref[0] = f
                ref[1] = f ^ jnp.uint32(0x80000000)
            l = lax.broadcasted_iota(jnp.int32, (64, 128), 1)
            flip = jnp.where((l & 1) != 0, jnp.uint32(0x80008000), jnp.uint32(0))
            for hf in range(2):
                g = cb[pl.ds(256 + 64 * hf, 64), :]
                gm[0, hf] = g
                gm[1, hf] = g ^ flip

        def setup_rows():
            skf = skb[...].astype(F32)
            ddf = ddb[...].astype(F32).reshape(1, D)
            gwf = gwb[...].astype(F32).reshape(1, D)
            for t in range(NT):
                sl = slice(t * 128, (t + 1) * 128)
                for j in range(4):
                    bc[6 * t + j] = jnp.broadcast_to(skf[j:j + 1, sl], (8, 128))
                bc[6 * t + 4] = jnp.broadcast_to(ddf[:, sl], (8, 128))
                bc[6 * t + 5] = jnp.broadcast_to(gwf[:, sl], (8, 128))

        def WT(c):
            for i in range(NT):
                tile = wqb[pl.ds(i * 128, 128), pl.ds(c * 128, 128)]
                wt[i, pl.ds(c * 128, 128), :] = lax.dot_general(emat(0), tile, NT_DIMS, preferred_element_type=F32)

        def head_major(src, i, base):
            return jnp.concatenate([src[i, pl.ds(base, 8, stride=DH), :], src[i, pl.ds(base + 8 * DH, 8, stride=DH), :]], axis=0)

        def WP(part, t):
            for j in range(4 * t, 4 * t + 4):
                for i in range(NT):
                    for m in range(2):
                        w = head_major(wt, i, part * D + j + 16 * DH * m)
                        if part == 0:
                            w = w * cexp
                        wtp[i, pl.ds((part * DH + j) * 32 + 16 * m, 16), :] = w.astype(BF16)

        def WO(n):
            wof[n] = wob[:, n * 128:(n + 1) * 128].astype(F32)
            for j in range(DH):
                for m in range(2):
                    wop[n, pl.ds(j * 32 + 16 * m, 16), :] = head_major(wof, n, j + 16 * DH * m).astype(BF16)

        def P(i, n):
            res = lax.dot_general(wide(qb, i * 64, 64), wide(wtp, n * 64, 64), NT_DIMS, preferred_element_type=F32)
            mark(res)
            part, t = divmod(n, NT)
            if part == 0:
                qs[t, rows(i), :] = res
            elif part == 1:
                ks[t, pl.ds(PAD + i * BLK, BLK), :] = res
            else:
                vs[t, pl.ds(PAD + i * BLK, BLK), :] = res

        def TL(i, p, c):
            r = i * BLK + 16 * p + 8 * c
            qv = [qs[t, pl.ds(r, 8), :] for t in range(NT)]
            qv[0] = dep(qv[0])
            ls = []
            for w in range(WIN):
                l = qv[0] * ks[0, pl.ds(PAD + r - DIL * w, 8), :]
                for t in range(1, NT):
                    l = l + qv[t] * ks[t, pl.ds(PAD + r - DIL * w, 8), :]
                ls.append(l)
            lgs[i % 4, p, pl.ds(64 * c, 64), :] = jnp.concatenate(ls, axis=0).astype(BF16)

        def TR(i, p):
            b0 = i * BLK + 16 * p
            red = jnp.dot(as_bf16(words(lgs, i % 4, p)), emat(1), preferred_element_type=F32)
            mark(red[:64])
            outs = []
            for c in range(2):
                r = b0 + 8 * c
                lw = [red[(c * WIN + w) * 8:(c * WIN + w + 1) * 8] for w in range(WIN)]
                if r < DIL * (WIN - 1):
                    pos = r + lax.broadcasted_iota(jnp.int32, (8, 128), 0)
                    lw = [jnp.where(pos >= DIL * w, lw[w], -1e30) for w in range(WIN)]
                m = lw[0]
                for w in range(1, WIN):
                    m = jnp.maximum(m, lw[w])
                e = [jnp.exp2(lw[w] - m) for w in range(WIN)]
                den = e[0]
                for w in range(1, WIN):
                    den = den + e[w]
                rinv = pl.reciprocal(den, approx=True)
                oc = [e[0] * vs[t, pl.ds(PAD + r, 8), :] for t in range(NT)]
                for w in range(1, WIN):
                    oc = [oc[t] + e[w] * vs[t, pl.ds(PAD + r - DIL * w, 8), :] for t in range(NT)]
                outs.append([oc[t] * rinv for t in range(NT)])
            for t in range(NT):
                ob[t, pl.ds(b0, 16), :] = jnp.concatenate([outs[0][t], outs[1][t]], axis=0).astype(BF16)

        def GA(i):
            zp = None
            for t in range(NT):
                g8 = dep(bc[6 * t + 5]) if t == 0 else bc[6 * t + 5]
                term = qb[t, rows(i), :].astype(F32) * rep(g8, 16)
                zp = term if zp is None else zp + term
            gps[i] = zp.astype(BF16)

        def GB(i):
            z = jnp.dot(as_bf16(words(gps, i)), emat(2), preferred_element_type=F32)
            mark(z)
            gs[rows(i), :] = 0.5 + 0.5 * jnp.tanh(0.5 * z)

        def O(i, n):
            bo = jnp.dot(wide(ob, i * 64, 64), as_bf16(words(wop, n)), preferred_element_type=F32)
            mark(bo)
            a_br = qb[n, rows(i), :].astype(F32) * yy[n, rows(i), :]
            outb[rows(i), n * 128:(n + 1) * 128] = (bo + gs[rows(i), :] * (a_br - bo)).astype(BF16)

        def KV(t, a, ms):
            lo = lambda x: as_f32(x << 16)
            hi = lambda x: as_f32(x & jnp.uint32(0xFFFF0000))
            c = [dep(bc[6 * t])] + [bc[6 * t + j] for j in range(1, 4)]
            for m in ms:
                base = 8 + 64 * a + 8 * m
                p0, p1, p2 = (words(kb, t, pl.ds(base - j, 8)) for j in range(3))
                l0, h0, l1, h1, h2 = lo(p0), hi(p0), lo(p1), hi(p1), hi(p2)
                ev = c[0] * l0 + c[1] * h1 + c[2] * l1 + c[3] * h2
                od = c[0] * h0 + c[1] * l0 + c[2] * h1 + c[3] * l1
                vv = words(vb, t, pl.ds(64 * a + 8 * m, 8))
                kvs[t % 2][a, pl.ds(16 * m, 16), :] = jnp.concatenate([ev * lo(vv), od * hi(vv)], axis=0).astype(BF16)

        def FU(t, a):
            u3 = u3s[t % 3]
            uu = jnp.dot(as_bf16(fp[a % 2]), as_bf16(words(kvs[t % 2], a)), preferred_element_type=F32)
            mark(uu[:64])
            uu = uu.reshape(NG, 2, 8, 128)
            ar, ai = uu[:, 0], uu[:, 1]
            u3[0, a, pl.ds(0, NG)] = ar + ai
            u3[1, a, pl.ds(0, NG)] = ar
            u3[2, a, pl.ds(0, NG)] = ai

        def FH(t, a):
            h3 = h3s[t % 3]
            hblk = hb[pl.ds(t * 128, 128), pl.ds(a * BLK, BLK)]
            hh = lax.dot_general(as_bf16(fm[a % 2]), hblk, NT_DIMS, preferred_element_type=F32)
            mark(hh[:64])
            hh = hh.reshape(NG, 2, 8, 128)
            br, bi = hh[:, 0], hh[:, 1]
            h3[0, a, pl.ds(0, NG)] = br
            h3[1, a, pl.ds(0, NG)] = bi - br
            h3[2, a, pl.ds(0, NG)] = br + bi

        def TP(t, g, part, comp, cache):
            u3, h3, zs = u3s[t % 3], h3s[t % 3], zss[t % 3]
            outs = tp_blocks[part]
            top = max(outs)
            dv = bc[6 * t + 4]
            hv = [h3[comp, d, g] for d in range(top + 1)]
            hv[0] = dep(hv[0] - dv if comp == 1 else hv[0] + dv)
            uv = [u3[comp, b, g] for b in range(top + 1)]
            s = {a: hv[0] * uv[a] for a in outs}
            for d in range(1, top + 1):
                for a in outs:
                    if a >= d:
                        s[a] = s[a] + hv[d] * uv[a - d]
            if comp == 0:
                cache["a1"] = s
            elif comp == 2:
                for a in outs:
                    cache["re", a] = cache["a1"][a] - s[a]
            else:
                for a in outs:
                    cache["im", a] = cache["a1"][a] + s[a]
                for a in sorted(set(outs) | {top + 1}):
                    if a == 0:
                        zr, zi = cache["re", 0], cache["im", 0]
                    elif ("im", a) in cache and ("im", a - 1) in cache:
                        zr = cache["re", a] - cache["im", a - 1]
                        zi = cache["im", a] + cache["re", a - 1]
                    else:
                        continue
                    zs[a, pl.ds(16 * g, 16), :] = jnp.concatenate([zr, zi], axis=0).astype(BF16)

        def IV(t, a):
            gmat = as_bf16(jnp.concatenate([gm[a % 2, 0], gm[a % 2, 1]], axis=1))
            y = jnp.dot(gmat, as_bf16(words(zss[t % 3], a)), preferred_element_type=F32)
            mark(y[:64])
            yy[t, rows(a), :] = y

        def run(fns):
            for fn in fns:
                fn()

        scope = (lambda n: jax.named_scope(n)) if scopes else (lambda n: contextlib.nullcontext())
        with scope("ep00a"):
            for nm in dma_order:
                for c in copies[nm]:
                    c.start()
            setup_masks()
            wait("tiny", "z")
            setup_rows()
            wait("Wq0")
            run([pt(WT, c) for c in range(2)])
            wait("Wq1", "q0", "q1")
            run([pt(WT, c) for c in range(2, 5)])
            run([pt(WP, 0, t) for t in range(NT)])
            run([pt(P, 0, n) for n in range(5)])
        with scope("ep00b"):
            wait("Wk")
            run([pt(WT, c) for c in range(5, 10)])
            run([pt(P, 1, n) for n in range(2)])
            run([pt(WP, 1, t) for t in range(NT)])
            run([pt(P, 0, n) for n in range(5, 10)])
        with scope("ep00c"):
            wait("Wv", "q2", "misc")
            setup_dft()
            run([pt(WT, c) for c in range(10, 15)])
            run([pt(P, 1, n) for n in range(2, 4)])
            run([pt(WP, 2, t) for t in range(NT)])
            run([pt(P, 0, n) for n in range(10, 15)])

        marks_per = {"P": 16, "O": 16, "GB": 16, "FU": 8, "FH": 8, "IV": 8, "TR": 8}
        out_copies = []
        done_o = set()
        sent = 0
        for e in range(1, nep + 1):
            with scope("ep%02d" % e):
                if e in waits:
                    wait(*waits[e])
                elif e in barriers:
                    barrier()
                pe = plan[e]
                streams = [
                    [(160, pt(P, i, n)) for i in pe["P"] for n in range(4 if i == 1 else 0, 3 * NT)],
                    [(160, pt(O, *x)) for x in pe["O"]],
                    [(64, pt(FH, *x)) for x in pe["FH"]],
                    [(64, pt(FU, *x)) for x in pe["FU"]],
                    [(64, pt(IV, *x)) for x in pe["IV"]],
                    [(32, pt(GB, i)) for i in pe["GB"]],
                    [(55, pt(TR, i, p)) for i in pe["TR"] for p in range(8)],
                    [(20, pt(TL, i, p, c)) for i in pe["TL"] for p in range(8) for c in range(2)],
                    [(60, pt(GA, i)) for i in pe["GA"]],
                    [(48 // kvsplit, pt(KV, *x, tuple(range(8 * s // kvsplit, 8 * (s + 1) // kvsplit))))
                     for x in pe["KV"] for s in range(kvsplit)],
                    [(30, pt(WO, i)) for i in pe["WO"]],
                ]
                tps = []
                for (t, g) in pe["TP"]:
                    cache = {}
                    for part, outs in enumerate(tp_blocks):
                        tps += [(sum(a + 1 for a in outs) // 2, pt(TP, t, g, part, c, cache)) for c in (0, 2, 1)]
                streams.append(tps)
                order = _interleave([s for s in streams if s])
                names = [fn.func.__name__ for fn in order]
                step = max(1, sum(marks_per.get(n, 0) for n in names) // max(1, sum(n in pace for n in names)))
                hard = (e in waits) or (e in barriers) or scopes
                state["marks"] = [] if hard else state["marks"][-keep:]
                seen = len(state["marks"])
                for fn, nm in zip(order, names):
                    marks = state["marks"]
                    if nm in pace and marks:
                        state["use"] = marks[min(len(marks) - 1, seen)]
                        seen = min(len(marks), seen + step)
                    else:
                        state["use"] = None
                    fn()
                state["use"] = None
                done_o.update(pe["O"])
                upto = sent
                while upto < NB and all((upto, n) in done_o for n in range(NT)):
                    upto += 1
                if upto > sent:
                    cp = pltpu.make_async_copy(outb.at[rows(sent, upto), :], out_hbm.at[0, rows(sent, upto), :],
                                               sem_o.at[len(out_copies)])
                    cp.start()
                    out_copies.append(cp)
                    sent = upto
        for cp in out_copies:
            cp.wait()

    comp_shape = (3, NB, NG + 1, 8, 128)
    scratch = [
        pltpu.VMEM((NT, S, 128), BF16),
        pltpu.VMEM((NT, S + 16, 128), BF16),
        pltpu.VMEM((NT, S, 128), BF16),
        pltpu.VMEM((D, S + 128), BF16),
        pltpu.VMEM((D, 3 * D), BF16),
        pltpu.VMEM((D, D), BF16),
        pltpu.VMEM((4, D), BF16),
        pltpu.VMEM((D,), BF16),
        pltpu.VMEM((D,), BF16),
        pltpu.VMEM((384, 128), U32),
        pltpu.VMEM((2, 128, 128), U32),
        pltpu.VMEM((2, 128, 128), U32),
        pltpu.VMEM((2, 2, 64, 128), U32),
        pltpu.VMEM((3, 64, 128), U32),
        pltpu.VMEM((6 * NT, 8, 128), F32),
        pltpu.VMEM((NT, 3 * D, 128), F32),
        pltpu.VMEM((NT, 3 * D, 128), BF16),
        pltpu.VMEM((NT, D, 128), F32),
        pltpu.VMEM((NT, D, 128), BF16),
        pltpu.VMEM((NT, S + 8, 128), F32),
        pltpu.VMEM((NT, S + PAD + 8, 128), F32),
        pltpu.VMEM((NT, S + PAD + 8, 128), F32),
        pltpu.VMEM((4, 8, 128, 128), BF16),
        pltpu.VMEM((NT, S, 128), BF16),
        pltpu.VMEM((NB, BLK, 128), BF16),
        pltpu.VMEM((S, 128), F32),
        pltpu.VMEM((NB, BLK, 128), BF16),
        pltpu.VMEM((NB, BLK, 128), BF16),
        pltpu.VMEM(comp_shape, F32),
        pltpu.VMEM(comp_shape, F32),
        pltpu.VMEM(comp_shape, F32),
        pltpu.VMEM(comp_shape, F32),
        pltpu.VMEM(comp_shape, F32),
        pltpu.VMEM(comp_shape, F32),
        pltpu.VMEM((NB, 2 * BLK, 128), BF16),
        pltpu.VMEM((NB, 2 * BLK, 128), BF16),
        pltpu.VMEM((NB, 2 * BLK, 128), BF16),
        pltpu.VMEM((NT, S, 128), F32),
        pltpu.VMEM((S, D), BF16),
        pltpu.SemaphoreType.DMA((64,)),
        pltpu.SemaphoreType.DMA((NB,)),
        pltpu.SemaphoreType.REGULAR,
        pltpu.SMEM((8,), jnp.int32),
    ]

    consts = _dft_constants()
    ramp = np.array([0, 5, 3, 9, 2, 7, 1, 4], np.int32)

    @jax.jit
    def run_kernel(A_q, A_k, A_v, A_shift_k, A_ssm_k, A_ssm_D, B_x, B_wqkv, B_wo, gate_w):
        return pl.pallas_call(
            kernel,
            out_shape=jax.ShapeDtypeStruct((1, S, D), BF16),
            in_specs=[pl.BlockSpec(memory_space=pl.ANY)] * 11,
            out_specs=pl.BlockSpec(memory_space=pl.ANY),
            scratch_shapes=scratch,
            compiler_params=pltpu.CompilerParams(vmem_limit_bytes=110 * 1024 * 1024),
        )(A_q, A_k, A_v, A_shift_k.T, A_ssm_k, A_ssm_D, B_wqkv, B_wo, gate_w, jnp.asarray(consts), jnp.asarray(ramp))

    return run_kernel


pallas_gated_mix__ssm_conv_h3__sliding_local_dilated__prompt_kernel = make_kernel()
```

```python
import contextlib
import functools
import math

import numpy as np
import jax
import jax.numpy as jnp
from jax import lax
from jax.experimental import pallas as pl
from jax.experimental.pallas import tpu as pltpu

S, D = 2048, 640
NT = D // 128
BLK = 128
NB = S // BLK
NG = 16
H, DH, WIN, DIL = 32, 20, 8, 2
PAD = 16
F32, BF16, U32 = jnp.float32, jnp.bfloat16, jnp.uint32
NT_DIMS = (((1,), (1,)), ((), ()))
ONE_LO, ONE_HI = 0x3F80, 0x3F800000
pt = functools.partial


def _pack_rows(m):
    b = np.asarray(m, dtype=np.float32).astype(BF16).view(np.uint16).astype(np.uint32)
    return b[0::2] | (b[1::2] << 16)


def _dft_constants():
    k = np.arange(BLK)
    n = np.arange(BLK)
    th = 2.0 * np.pi * (k[:, None] + 0.5) * n[None, :] / (2 * BLK)
    fwd = np.stack([np.cos(th).reshape(NG, 8, BLK), -np.sin(th).reshape(NG, 8, BLK)], axis=1).reshape(2 * BLK, BLK)
    order = np.arange(BLK).reshape(8, 8, 2).transpose(0, 2, 1).reshape(BLK)
    inv = np.stack([(np.cos(th).T / BLK).reshape(BLK, NG, 8), (-np.sin(th).T / BLK).reshape(BLK, NG, 8)], axis=2)
    pi = _pack_rows(inv.reshape(BLK, 2 * BLK))
    return np.concatenate([_pack_rows(fwd), _pack_rows(fwd[:, order]), pi[:, :BLK], pi[:, BLK:]], axis=0)


def _interleave(streams):
    items = []
    for si, s in enumerate(streams):
        tot = float(sum(w for w, _ in s))
        acc = 0.0
        for w, fn in s:
            items.append(((acc + 0.5 * w) / tot, si, fn))
            acc += w
    items.sort(key=lambda x: (x[0], x[1]))
    return [fn for _, _, fn in items]


MXU_COST = dict(P=2400, TR=256, GB=32, FU=64, FH=64, IV=64, O=160)
KEYS = ("P", "TL", "TR", "GA", "GB", "KV", "FU", "FH", "TP", "IV", "O", "WO")


def make_plan(tl_ep=(1, 2, 2, 3, 5, 7, 9, 11, 12, 13, 13, 14, 14, 15, 15, 16), tp0=4, a0=2, rate=8.0, wo_epoch=6,
              m_target=5200, a_ready=(2, 4, 4, 5, 7), f_span=1, p_ep=None):
    p_ep = p_ep or [0, 1, 1] + list(range(2, 15))
    nep = max(tl_ep) + 2
    plan = {e: {k: [] for k in KEYS} for e in range(1, nep + 1)}
    for i in range(1, NB):
        plan[p_ep[i]]["P"].append(i)
    gb_ep = {}
    for i in range(NB):
        assert tl_ep[i] > p_ep[i], i
        assert i < 4 or tl_ep[i - 4] + 1 < tl_ep[i], i
        plan[tl_ep[i]]["TL"].append(i)
        plan[tl_ep[i] + 1]["TR"].append(i)
        gb_ep[i] = max(3, tl_ep[i] + 1)
        plan[gb_ep[i]]["GB"].append(i)
        plan[gb_ep[i] - 1]["GA"].append(i)
    ep_tp = [tp0 + int(v / rate) for v in range(NT * NG)]
    for v, e in enumerate(ep_tp):
        plan[e]["TP"].append(divmod(v, NG))
    plan[a0]["KV"] = [(0, a) for a in range(NB)]
    plan[a0]["FH"] = [(0, a) for a in range(NB)]
    plan[tp0 - 1]["FU"] += [(0, a) for a in range(NB)]
    fu_done = {0: tp0 - 1}
    for t in range(1, NT):
        last = ep_tp[NG * t] - 1
        first = max(a0 + 2, ep_tp[NG * (t - 1)], a_ready[t] + 1)
        if t >= 3:
            first = max(first, ep_tp[NG * (t - 3) + NG - 1] + 1)
        if t >= 2:
            first = max(first, fu_done[t - 2] + 2)
        eps = list(range(first, last + 1))[-f_span:]
        assert eps, (t, first, last)
        for a in range(NB):
            e = eps[a * len(eps) // NB]
            plan[e]["FU"].append((t, a))
            plan[e]["FH"].append((t, a))
            plan[e - 1]["KV"].append((t, a))
        fu_done[t] = last
    iv_ep = {}
    for t in range(NT):
        e0 = ep_tp[NG * t + NG - 1] + 1
        for a in range(NB):
            iv_ep[(t, a)] = e0 + (a >= NB // 2 and t < NT - 1)
            plan[iv_ep[(t, a)]]["IV"].append((t, a))
        if t >= 3:
            assert max(iv_ep[(t - 3, a)] for a in range(NB)) < ep_tp[NG * t]
    plan[wo_epoch]["WO"] = list(range(NT))

    def mxu(e):
        return sum(MXU_COST.get(k, 0) * len(v) for k, v in plan[e].items())
    todo = [(i, n) for n in range(NT) for i in range(NB)]
    for e in range(wo_epoch + 1, nep + 1):
        avail = [x for x in todo if iv_ep[(x[1], x[0])] < e and tl_ep[x[0]] + 1 < e and gb_ep[x[0]] < e]
        avail.sort()
        for x in avail:
            if e < nep and mxu(e) + MXU_COST["O"] > m_target:
                break
            plan[e]["O"].append(x)
            todo.remove(x)
    assert not todo, todo
    return plan


Q_GROUPS = {"q0": (0, 1), "q1": (1, 2), "q2": (2, 3), "q3": (3, 4), "q45": (4, 6), "q67": (6, 8), "q8f": (8, 16)}
DMA_ORDER = ("tiny", "z", "Wq0", "Wq1", "q0", "q1", "Wk", "Wv", "q2", "misc", "q3", "A0", "q45", "A1", "q67", "A2", "Wo", "A3",
             "q8f", "A4")
WAITS = {2: ("q3", "A0", "q45"), 4: ("A1", "q67", "A2"), 6: ("Wo", "A3", "q8f"), 8: ("A4",)}


def make_kernel(plan_kw=None, scopes=False, barriers=(10, 12, 15), waits=WAITS, dma_order=DMA_ORDER,
                tp_blocks=((15, 14, 13), (12, 11, 10), (9, 8, 7, 6), (5, 4, 3, 2, 1, 0)),
                pace=("TL", "KV", "TP", "GA"), keep=16, kvsplit=2):
    plan = make_plan(**(plan_kw or {}))
    nep = max(plan)
    waited = {nm: e for e, names in waits.items() for nm in names}
    for e, pe in plan.items():
        for i in pe["P"] + pe["GA"] + [x[0] for x in pe["O"]]:
            for nm, (i0, i1) in Q_GROUPS.items():
                assert not (i0 <= i < i1) or waited.get(nm, 0) <= e, (nm, e)
        for t, _ in pe["KV"] + pe["FH"]:
            assert waited["A%d" % t] <= e, (t, e)
        assert not pe["WO"] or waited["Wo"] <= e

    def kernel(q_hbm, k_hbm, v_hbm, sk_hbm, h_hbm, dd_hbm, wqkv_hbm, wo_hbm, gw_hbm, c_hbm, z_hbm, out_hbm,
               qb, kb, vb, hb, wqb, wob, skb, ddb, gwb, cb,
               fm, fp, gm, em, bc,
               wt, wtp, wof, wop,
               qs, ks, vs, lgs, ob, gps, gs,
               kva, kvb, u3a, u3b, u3c, h3a, h3b, h3c, zsa, zsb, zsc, yy, outb,
               sem_in, sem_o, sem_b, zsm):
        kvs, u3s, h3s, zss = (kva, kvb), (u3a, u3b, u3c), (h3a, h3b, h3c), (zsa, zsb, zsc)

        def rows(i0, i1=None):
            i1 = i0 + 1 if i1 is None else i1
            return pl.ds(i0 * BLK, (i1 - i0) * BLK)

        copies = {}
        nsem = [0]

        def add_copy(name, src, dst):
            copies.setdefault(name, []).append(pltpu.make_async_copy(src, dst, sem_in.at[nsem[0]]))
            nsem[0] += 1

        add_copy("Wq0", wqkv_hbm.at[:, pl.ds(0, 256)], wqb.at[:, pl.ds(0, 256)])
        add_copy("Wq1", wqkv_hbm.at[:, pl.ds(256, 384)], wqb.at[:, pl.ds(256, 384)])
        for part, nm in ((1, "Wk"), (2, "Wv")):
            add_copy(nm, wqkv_hbm.at[:, pl.ds(part * D, D)], wqb.at[:, pl.ds(part * D, D)])
        add_copy("z", z_hbm, zsm)
        add_copy("misc", c_hbm, cb)
        add_copy("tiny", sk_hbm, skb)
        add_copy("tiny", dd_hbm, ddb)
        add_copy("tiny", gw_hbm, gwb)
        add_copy("Wo", wo_hbm, wob)
        for nm, (i0, i1) in Q_GROUPS.items():
            for t in range(NT):
                add_copy(nm, q_hbm.at[0, rows(i0, i1), pl.ds(t * 128, 128)], qb.at[t, rows(i0, i1), :])
        for t in range(NT):
            add_copy("A%d" % t, h_hbm.at[pl.ds(t * 128, 128), :], hb.at[pl.ds(t * 128, 128), pl.ds(0, S)])
            add_copy("A%d" % t, k_hbm.at[0, :, pl.ds(t * 128, 128)], kb.at[t, pl.ds(16, S), :])
            add_copy("A%d" % t, v_hbm.at[0, :, pl.ds(t * 128, 128)], vb.at[t])

        def wait(*names):
            for nm in names:
                for c in copies[nm]:
                    c.wait()

        def barrier():
            pl.semaphore_signal(sem_b, 1)
            pl.semaphore_wait(sem_b, 1)

        state = {"marks": [], "use": None}

        def dep(x):
            if state["use"] is None:
                return x
            never = lax.broadcasted_iota(jnp.int32, (8, 128), 0) < zsm[0]
            return jnp.where(never, state["use"], x)

        def mark(res):
            state["marks"] += [res[8 * j:8 * j + 8] for j in range(res.shape[0] // 8)]

        def rep(v, n):
            return jnp.concatenate([v] * n, axis=0)

        def words(ref, *idx):
            return ref.bitcast(U32)[idx]

        def as_bf16(w):
            return pltpu.bitcast(w, BF16)

        def as_f32(w):
            return pltpu.bitcast(w, F32)

        def wide(ref, r0, n):
            return as_bf16(jnp.concatenate([words(ref, t, pl.ds(r0, n)) for t in range(NT)], axis=1))

        emat = lambda j: as_bf16(em[j])
        cexp = (DH ** -0.5) * math.log2(math.e)

        def setup_masks():
            r = lax.broadcasted_iota(jnp.int32, (64, 128), 0)
            l = lax.broadcasted_iota(jnp.int32, (64, 128), 1)
            lo, hi, zero = jnp.uint32(ONE_LO), jnp.uint32(ONE_HI), jnp.uint32(0)
            em[0] = jnp.where(l == 2 * r, lo, zero) | jnp.where(l == 2 * r + 1, hi, zero)
            em[1] = jnp.where((l & 31) == ((2 * r) & 31), lo, zero) | jnp.where((l & 31) == ((2 * r + 1) & 31), hi, zero)
            em[2] = jnp.full((64, 128), ONE_LO | ONE_HI, U32)
            for t in range(NT):
                ks[t, pl.ds(0, PAD), :] = jnp.zeros((PAD, 128), F32)
                vs[t, pl.ds(0, PAD), :] = jnp.zeros((PAD, 128), F32)
                kb[t, pl.ds(0, 16), :] = jnp.zeros((16, 128), BF16)

        def setup_dft():
            for ref, r0 in ((fm, 0), (fp, 128)):
                f = cb[pl.ds(r0, 128), :]
                ref[0] = f
                ref[1] = f ^ jnp.uint32(0x80000000)
            l = lax.broadcasted_iota(jnp.int32, (64, 128), 1)
            flip = jnp.where((l & 1) != 0, jnp.uint32(0x80008000), jnp.uint32(0))
            for hf in range(2):
                g = cb[pl.ds(256 + 64 * hf, 64), :]
                gm[0, hf] = g
                gm[1, hf] = g ^ flip

        def setup_rows():
            skf = skb[...].astype(F32)
            ddf = ddb[...].astype(F32).reshape(1, D)
            gwf = gwb[...].astype(F32).reshape(1, D)
            for t in range(NT):
                sl = slice(t * 128, (t + 1) * 128)
                for j in range(4):
                    bc[6 * t + j] = jnp.broadcast_to(skf[j:j + 1, sl], (8, 128))
                bc[6 * t + 4] = jnp.broadcast_to(ddf[:, sl], (8, 128))
                bc[6 * t + 5] = jnp.broadcast_to(gwf[:, sl], (8, 128))

        def WT(c):
            for i in range(NT):
                tile = wqb[pl.ds(i * 128, 128), pl.ds(c * 128, 128)]
                wt[i, pl.ds(c * 128, 128), :] = lax.dot_general(emat(0), tile, NT_DIMS, preferred_element_type=F32)

        def head_major(src, i, base):
            return jnp.concatenate([src[i, pl.ds(base, 8, stride=DH), :], src[i, pl.ds(base + 8 * DH, 8, stride=DH), :]], axis=0)

        def WP(part, t):
            for j in range(4 * t, 4 * t + 4):
                for i in range(NT):
                    for m in range(2):
                        w = head_major(wt, i, part * D + j + 16 * DH * m)
                        if part == 0:
                            w = w * cexp
                        wtp[i, pl.ds((part * DH + j) * 32 + 16 * m, 16), :] = w.astype(BF16)

        def WO(n):
            wof[n] = wob[:, n * 128:(n + 1) * 128].astype(F32)
            for j in range(DH):
                for m in range(2):
                    wop[n, pl.ds(j * 32 + 16 * m, 16), :] = head_major(wof, n, j + 16 * DH * m).astype(BF16)

        def P(i, n):
            res = lax.dot_general(wide(qb, i * 64, 64), wide(wtp, n * 64, 64), NT_DIMS, preferred_element_type=F32)
            mark(res)
            part, t = divmod(n, NT)
            if part == 0:
                qs[t, rows(i), :] = res
            elif part == 1:
                ks[t, pl.ds(PAD + i * BLK, BLK), :] = res
            else:
                vs[t, pl.ds(PAD + i * BLK, BLK), :] = res

        def TL(i, p, c):
            r = i * BLK + 16 * p + 8 * c
            qv = [qs[t, pl.ds(r, 8), :] for t in range(NT)]
            qv[0] = dep(qv[0])
            ls = []
            for w in range(WIN):
                l = qv[0] * ks[0, pl.ds(PAD + r - DIL * w, 8), :]
                for t in range(1, NT):
                    l = l + qv[t] * ks[t, pl.ds(PAD + r - DIL * w, 8), :]
                ls.append(l)
            lgs[i % 4, p, pl.ds(64 * c, 64), :] = jnp.concatenate(ls, axis=0).astype(BF16)

        def TR(i, p):
            b0 = i * BLK + 16 * p
            red = jnp.dot(as_bf16(words(lgs, i % 4, p)), emat(1), preferred_element_type=F32)
            mark(red[:64])
            outs = []
            for c in range(2):
                r = b0 + 8 * c
                lw = [red[(c * WIN + w) * 8:(c * WIN + w + 1) * 8] for w in range(WIN)]
                if r < DIL * (WIN - 1):
                    pos = r + lax.broadcasted_iota(jnp.int32, (8, 128), 0)
                    lw = [jnp.where(pos >= DIL * w, lw[w], -1e30) for w in range(WIN)]
                m = lw[0]
                for w in range(1, WIN):
                    m = jnp.maximum(m, lw[w])
                e = [jnp.exp2(lw[w] - m) for w in range(WIN)]
                den = e[0]
                for w in range(1, WIN):
                    den = den + e[w]
                rinv = pl.reciprocal(den, approx=True)
                oc = [e[0] * vs[t, pl.ds(PAD + r, 8), :] for t in range(NT)]
                for w in range(1, WIN):
                    oc = [oc[t] + e[w] * vs[t, pl.ds(PAD + r - DIL * w, 8), :] for t in range(NT)]
                outs.append([oc[t] * rinv for t in range(NT)])
            for t in range(NT):
                ob[t, pl.ds(b0, 16), :] = jnp.concatenate([outs[0][t], outs[1][t]], axis=0).astype(BF16)

        def GA(i):
            zp = None
            for t in range(NT):
                g8 = dep(bc[6 * t + 5]) if t == 0 else bc[6 * t + 5]
                term = qb[t, rows(i), :].astype(F32) * rep(g8, 16)
                zp = term if zp is None else zp + term
            gps[i] = zp.astype(BF16)

        def GB(i):
            z = jnp.dot(as_bf16(words(gps, i)), emat(2), preferred_element_type=F32)
            mark(z)
            gs[rows(i), :] = 0.5 + 0.5 * jnp.tanh(0.5 * z)

        def O(i, n):
            bo = jnp.dot(wide(ob, i * 64, 64), as_bf16(words(wop, n)), preferred_element_type=F32)
            mark(bo)
            a_br = qb[n, rows(i), :].astype(F32) * yy[n, rows(i), :]
            outb[rows(i), n * 128:(n + 1) * 128] = (bo + gs[rows(i), :] * (a_br - bo)).astype(BF16)

        def KV(t, a, ms):
            lo = lambda x: as_f32(x << 16)
            hi = lambda x: as_f32(x & jnp.uint32(0xFFFF0000))
            c = [dep(bc[6 * t])] + [bc[6 * t + j] for j in range(1, 4)]
            for m in ms:
                base = 8 + 64 * a + 8 * m
                p0, p1, p2 = (words(kb, t, pl.ds(base - j, 8)) for j in range(3))
                l0, h0, l1, h1, h2 = lo(p0), hi(p0), lo(p1), hi(p1), hi(p2)
                ev = c[0] * l0 + c[1] * h1 + c[2] * l1 + c[3] * h2
                od = c[0] * h0 + c[1] * l0 + c[2] * h1 + c[3] * l1
                vv = words(vb, t, pl.ds(64 * a + 8 * m, 8))
                kvs[t % 2][a, pl.ds(16 * m, 16), :] = jnp.concatenate([ev * lo(vv), od * hi(vv)], axis=0).astype(BF16)

        def FU(t, a):
            u3 = u3s[t % 3]
            uu = jnp.dot(as_bf16(fp[a % 2]), as_bf16(words(kvs[t % 2], a)), preferred_element_type=F32)
            mark(uu[:64])
            uu = uu.reshape(NG, 2, 8, 128)
            ar, ai = uu[:, 0], uu[:, 1]
            u3[0, a, pl.ds(0, NG)] = ar + ai
            u3[1, a, pl.ds(0, NG)] = ar
            u3[2, a, pl.ds(0, NG)] = ai

        def FH(t, a):
            h3 = h3s[t % 3]
            hblk = hb[pl.ds(t * 128, 128), pl.ds(a * BLK, BLK)]
            hh = lax.dot_general(as_bf16(fm[a % 2]), hblk, NT_DIMS, preferred_element_type=F32)
            mark(hh[:64])
            hh = hh.reshape(NG, 2, 8, 128)
            br, bi = hh[:, 0], hh[:, 1]
            if a == 0:
                br = br + bc[6 * t + 4]
            h3[0, a, pl.ds(0, NG)] = br
            h3[1, a, pl.ds(0, NG)] = bi - br
            h3[2, a, pl.ds(0, NG)] = br + bi

        def TP(t, g, part, comp, cache):
            u3, h3, zs = u3s[t % 3], h3s[t % 3], zss[t % 3]
            outs = tp_blocks[part]
            top = max(outs)
            hv = [h3[comp, d, g] for d in range(top + 1)]
            hv[0] = dep(hv[0])
            uv = [u3[comp, b, g] for b in range(top + 1)]
            s = {a: hv[0] * uv[a] for a in outs}
            for d in range(1, top + 1):
                for a in outs:
                    if a >= d:
                        s[a] = s[a] + hv[d] * uv[a - d]
            if comp == 0:
                cache["a1"] = s
            elif comp == 2:
                for a in outs:
                    cache["re", a] = cache["a1"][a] - s[a]
            else:
                for a in outs:
                    cache["im", a] = cache["a1"][a] + s[a]
                for a in sorted(set(outs) | {top + 1}):
                    if a == 0:
                        zr, zi = cache["re", 0], cache["im", 0]
                    elif ("im", a) in cache and ("im", a - 1) in cache:
                        zr = cache["re", a] - cache["im", a - 1]
                        zi = cache["im", a] + cache["re", a - 1]
                    else:
                        continue
                    zs[a, pl.ds(16 * g, 16), :] = jnp.concatenate([zr, zi], axis=0).astype(BF16)

        def IV(t, a):
            gmat = as_bf16(jnp.concatenate([gm[a % 2, 0], gm[a % 2, 1]], axis=1))
            y = jnp.dot(gmat, as_bf16(words(zss[t % 3], a)), preferred_element_type=F32)
            mark(y[:64])
            yy[t, rows(a), :] = y

        def run(fns):
            for fn in fns:
                fn()

        scope = (lambda n: jax.named_scope(n)) if scopes else (lambda n: contextlib.nullcontext())
        with scope("ep00a"):
            for nm in dma_order:
                for c in copies[nm]:
                    c.start()
            setup_masks()
            wait("tiny", "z")
            setup_rows()
            wait("Wq0")
            run([pt(WT, c) for c in range(2)])
            wait("Wq1", "q0", "q1")
            run([pt(WT, c) for c in range(2, 5)])
            run([pt(WP, 0, t) for t in range(NT)])
            run([pt(P, 0, n) for n in range(5)])
        with scope("ep00b"):
            wait("Wk")
            run([pt(WT, c) for c in range(5, 10)])
            run([pt(P, 1, n) for n in range(2)])
            run([pt(WP, 1, t) for t in range(NT)])
            run([pt(P, 0, n) for n in range(5, 10)])
        with scope("ep00c"):
            wait("Wv", "q2", "misc")
            setup_dft()
            run([pt(WT, c) for c in range(10, 15)])
            run([pt(P, 1, n) for n in range(2, 4)])
            run([pt(WP, 2, t) for t in range(NT)])
            run([pt(P, 0, n) for n in range(10, 15)])

        marks_per = {"P": 16, "O": 16, "GB": 16, "FU": 8, "FH": 8, "IV": 8, "TR": 8}
        out_copies = []
        done_o = set()
        sent = 0
        for e in range(1, nep + 1):
            with scope("ep%02d" % e):
                if e in waits:
                    wait(*waits[e])
                elif e in barriers:
                    barrier()
                pe = plan[e]
                streams = [
                    [(160, pt(P, i, n)) for i in pe["P"] for n in range(4 if i == 1 else 0, 3 * NT)],
                    [(160, pt(O, *x)) for x in pe["O"]],
                    [(64, pt(FH, *x)) for x in pe["FH"]],
                    [(64, pt(FU, *x)) for x in pe["FU"]],
                    [(64, pt(IV, *x)) for x in pe["IV"]],
                    [(32, pt(GB, i)) for i in pe["GB"]],
                    [(55, pt(TR, i, p)) for i in pe["TR"] for p in range(8)],
                    [(20, pt(TL, i, p, c)) for i in pe["TL"] for p in range(8) for c in range(2)],
                    [(60, pt(GA, i)) for i in pe["GA"]],
                    [(48 // kvsplit, pt(KV, *x, tuple(range(8 * s // kvsplit, 8 * (s + 1) // kvsplit))))
                     for x in pe["KV"] for s in range(kvsplit)],
                    [(30, pt(WO, i)) for i in pe["WO"]],
                ]
                tps = []
                for (t, g) in pe["TP"]:
                    cache = {}
                    for part, outs in enumerate(tp_blocks):
                        tps += [(sum(a + 1 for a in outs) // 2, pt(TP, t, g, part, c, cache)) for c in (0, 2, 1)]
                streams.append(tps)
                order = _interleave([s for s in streams if s])
                names = [fn.func.__name__ for fn in order]
                step = max(1, sum(marks_per.get(n, 0) for n in names) // max(1, sum(n in pace for n in names)))
                hard = (e in waits) or (e in barriers) or scopes
                state["marks"] = [] if hard else state["marks"][-keep:]
                seen = len(state["marks"])
                for fn, nm in zip(order, names):
                    marks = state["marks"]
                    if nm in pace and marks:
                        state["use"] = marks[min(len(marks) - 1, seen)]
                        seen = min(len(marks), seen + step)
                    else:
                        state["use"] = None
                    fn()
                state["use"] = None
                done_o.update(pe["O"])
                upto = sent
                while upto < NB and all((upto, n) in done_o for n in range(NT)):
                    upto += 1
                if upto > sent:
                    cp = pltpu.make_async_copy(outb.at[rows(sent, upto), :], out_hbm.at[0, rows(sent, upto), :],
                                               sem_o.at[len(out_copies)])
                    cp.start()
                    out_copies.append(cp)
                    sent = upto
        for cp in out_copies:
            cp.wait()

    comp_shape = (3, NB, NG + 1, 8, 128)
    scratch = [
        pltpu.VMEM((NT, S, 128), BF16),
        pltpu.VMEM((NT, S + 16, 128), BF16),
        pltpu.VMEM((NT, S, 128), BF16),
        pltpu.VMEM((D, S + 128), BF16),
        pltpu.VMEM((D, 3 * D), BF16),
        pltpu.VMEM((D, D), BF16),
        pltpu.VMEM((4, D), BF16),
        pltpu.VMEM((D,), BF16),
        pltpu.VMEM((D,), BF16),
        pltpu.VMEM((384, 128), U32),
        pltpu.VMEM((2, 128, 128), U32),
        pltpu.VMEM((2, 128, 128), U32),
        pltpu.VMEM((2, 2, 64, 128), U32),
        pltpu.VMEM((3, 64, 128), U32),
        pltpu.VMEM((6 * NT, 8, 128), F32),
        pltpu.VMEM((NT, 3 * D, 128), F32),
        pltpu.VMEM((NT, 3 * D, 128), BF16),
        pltpu.VMEM((NT, D, 128), F32),
        pltpu.VMEM((NT, D, 128), BF16),
        pltpu.VMEM((NT, S + 8, 128), F32),
        pltpu.VMEM((NT, S + PAD + 8, 128), F32),
        pltpu.VMEM((NT, S + PAD + 8, 128), F32),
        pltpu.VMEM((4, 8, 128, 128), BF16),
        pltpu.VMEM((NT, S, 128), BF16),
        pltpu.VMEM((NB, BLK, 128), BF16),
        pltpu.VMEM((S, 128), F32),
        pltpu.VMEM((NB, BLK, 128), BF16),
        pltpu.VMEM((NB, BLK, 128), BF16),
        pltpu.VMEM(comp_shape, F32),
        pltpu.VMEM(comp_shape, F32),
        pltpu.VMEM(comp_shape, F32),
        pltpu.VMEM(comp_shape, F32),
        pltpu.VMEM(comp_shape, F32),
        pltpu.VMEM(comp_shape, F32),
        pltpu.VMEM((NB, 2 * BLK, 128), BF16),
        pltpu.VMEM((NB, 2 * BLK, 128), BF16),
        pltpu.VMEM((NB, 2 * BLK, 128), BF16),
        pltpu.VMEM((NT, S, 128), F32),
        pltpu.VMEM((S, D), BF16),
        pltpu.SemaphoreType.DMA((64,)),
        pltpu.SemaphoreType.DMA((NB,)),
        pltpu.SemaphoreType.REGULAR,
        pltpu.SMEM((8,), jnp.int32),
    ]

    consts = _dft_constants()
    ramp = np.array([0, 5, 3, 9, 2, 7, 1, 4], np.int32)

    @jax.jit
    def run_kernel(A_q, A_k, A_v, A_shift_k, A_ssm_k, A_ssm_D, B_x, B_wqkv, B_wo, gate_w):
        return pl.pallas_call(
            kernel,
            out_shape=jax.ShapeDtypeStruct((1, S, D), BF16),
            in_specs=[pl.BlockSpec(memory_space=pl.ANY)] * 11,
            out_specs=pl.BlockSpec(memory_space=pl.ANY),
            scratch_shapes=scratch,
            compiler_params=pltpu.CompilerParams(vmem_limit_bytes=110 * 1024 * 1024),
        )(A_q, A_k, A_v, A_shift_k.T, A_ssm_k, A_ssm_D, B_wqkv, B_wo, gate_w, jnp.asarray(consts), jnp.asarray(ramp))

    return run_kernel


pallas_gated_mix__ssm_conv_h3__sliding_local_dilated__prompt_kernel = make_kernel()
```
